```python
import jax
import jax.numpy as jnp

def _softmax(x, axis=-1):
    return jax.nn.softmax(x, axis=axis)
def _gelu(x):
    return jax.nn.gelu(x, approximate=True)
def _silu(x):
    return jax.nn.silu(x)
def _sigmoid(x):
    return jax.nn.sigmoid(x)
def _layernorm(x, axis=-1, eps=1e-5):
    m = jnp.mean(x, axis=axis, keepdims=True)
    v = jnp.var(x, axis=axis, keepdims=True)
    return (x - m) / jnp.sqrt(v + eps)
def _scatter_add(tgt, idx, src, axis=0):
    return tgt.at[idx].add(src)
def _segment_sum(src, seg, n):
    return jax.ops.segment_sum(src, seg, n)
class _Rng:
    def __init__(self, key):
        self._k = key
    def _next(self):
        self._k, sub = jax.random.split(self._k)
        return sub
    def normal(self, shape):
        return jax.random.normal(self._next(), shape, dtype=jnp.bfloat16)
    def randint(self, lo, hi, shape):
        return jax.random.randint(self._next(), shape, lo, hi, dtype=jnp.int32)
    def uniform(self, shape, lo=0.0, hi=1.0):
        return jax.random.uniform(self._next(), shape, jnp.bfloat16, lo, hi)
    def permutation(self, n):
        return jax.random.permutation(self._next(), n)


kernel_name = 'recurrent_scan__sliding_local_dilated__mixer_token_mlp__prompt'

def setup_inputs():
    _rng = _Rng(jax.random.key(int.from_bytes(__import__("os").urandom(4), "little")))
    _w = (lambda a: (lambda t: t.astype(jnp.bfloat16) if jnp.issubdtype(t.dtype, jnp.floating) else t)(jnp.asarray(a)))
    def _A_setup():
        B, S, D = 1, 2048, 448
        return {
            "x": _w((lambda *s: _rng.normal(s) * 0.05)(B, S, D)),
            "wqkv": _w((lambda *s: _rng.normal(s) * 0.05)(D, 3 * D)),
            "wo": _w((lambda *s: _rng.normal(s) * 0.05)(D, D)),
        }
    _A_in = _A_setup()

    def _B_setup():
        B, S, D, F = 1, 2048, 448, 1792
        return {
            "x": _w((lambda *s: _rng.normal(s) * 0.05)(B, S, D)),
            "w1": _w((lambda *s: _rng.normal(s) * 0.05)(S, F) * (S ** -0.5)),
            "b1": _w((lambda *s: _rng.normal(s) * 0.05)(F) * 0.02),
            "w2": _w((lambda *s: _rng.normal(s) * 0.05)(F, S) * (F ** -0.5)),
            "b2": _w((lambda *s: _rng.normal(s) * 0.05)(S) * 0.02),
        }
    _B_in = _B_setup()

    return {
        "A_x": _A_in["x"],
        "A_wqkv": _A_in["wqkv"],
        "A_wo": _A_in["wo"],
        "B_x": _B_in["x"],
        "B_w1": _B_in["w1"],
        "B_b1": _B_in["b1"],
        "B_w2": _B_in["w2"],
        "B_b2": _B_in["b2"],
    }

def reference(A_x, A_wqkv, A_wo, B_x, B_w1, B_b1, B_w2, B_b2):
    def _A_ref(x, wqkv, wo):
        B, S, D = x.shape
        H = 16; Dh = D // H
        W, dil = 8, 2
        qkv = (lambda x, *d: x.transpose(*d))((x @ wqkv).reshape(B, S, 3, H, Dh), 2, 0, 3, 1, 4)
        q, k, v = qkv[0], qkv[1], qkv[2]
        scale = Dh ** -0.5
        pos = jnp.arange(S)
        off = jnp.arange(W) * dil
        idx = pos[:, None] - off[None, :]
        mask = idx >= 0
        idx_c = jnp.where(mask, idx, 0).reshape(-1)
        kg = k[:, :, idx_c, :].reshape(B, H, S, W, Dh)
        vg = v[:, :, idx_c, :].reshape(B, H, S, W, Dh)
        logits = jnp.einsum("bhsd,bhswd->bhsw", q, kg) * scale
        logits = jnp.where(mask[None, None, :, :], logits, -1e9)
        attn = _softmax(logits, axis=-1)
        o = jnp.einsum("bhsw,bhswd->bhsd", attn, vg)
        return (lambda x, *d: x.transpose(*d))(o, 0, 2, 1, 3).reshape(B, S, D) @ wo

    def _B_ref(x, w1, b1, w2, b2):
        B, S, D = x.shape
        h = _layernorm(x, axis=-1)
        u = jnp.einsum("bsd,sf->bdf", h, w1) + b1
        u = _gelu(u)
        y = jnp.einsum("bdf,fs->bds", u, w2) + b2
        return (lambda x, *d: x.transpose(*d))(y, 0, 2, 1)

    x = A_x
    xn = _layernorm(x, axis=-1)
    s = _A_ref(xn, A_wqkv, A_wo)
    g = _silu(_B_ref(xn, B_w1, B_b1, B_w2, B_b2))
    return x + s * g
```

```python
import functools

import jax
import jax.numpy as jnp
import jax.experimental.pallas as pl
import jax.experimental.pallas.tpu as pltpu

S = 2048
D = 448
H = 16
DH = D // H
F = 1792
W = 8
EPS = 1e-5
TC = 256
NC = S // TC
LANES = 128
NCOL = S // LANES
SLAB = 32

f32 = jnp.float32
bf16 = jnp.bfloat16


def _ln_cols(x):
    m = jnp.sum(x, axis=0, keepdims=True) * (1.0 / D)
    xc = x - m
    v = jnp.sum(xc * xc, axis=0, keepdims=True) * (1.0 / D)
    return xc * jax.lax.rsqrt(v + EPS)


def _gelu(x):
    c = 0.7978845608028654
    t = jnp.tanh(x * (c + (c * 0.044715) * (x * x)))
    hx = 0.5 * x
    return hx + hx * t


def _silu(y):
    hy = 0.5 * y
    return hy + hy * jnp.tanh(hy)


def _kernel(x_hbm, wqkv_hbm, wo_hbm, w1_hbm, b1_hbm, w2_hbm, b2_hbm, out_hbm,
            x_s, wqkv_s, wo_s, w1_s, w2_s, b1_s, b2_s,
            xn_s, acc_s, u_s, wt32_s, wqkvt_s, wo32_s, wot_s,
            qkv_s, rk_s, rv_s, o_s, out_s, b1f_s, b2f_s,
            sem_x, sem_w1, sem_w2, sem_misc, sem_out):
    def x_cp(c):
        return pltpu.make_async_copy(x_hbm.at[0, :, c * TC:(c + 1) * TC],
                                     x_s.at[:, c * TC:(c + 1) * TC], sem_x.at[c])

    def w1_cp(c):
        return pltpu.make_async_copy(w1_hbm.at[c * TC:(c + 1) * TC, :],
                                     w1_s.at[c * TC:(c + 1) * TC, :], sem_w1.at[c])

    def w2_cp(c):
        return pltpu.make_async_copy(w2_hbm.at[:, c * TC:(c + 1) * TC],
                                     w2_s.at[:, c * TC:(c + 1) * TC], sem_w2.at[c])

    def out_cp(c):
        return pltpu.make_async_copy(out_s.at[:, c * TC:(c + 1) * TC],
                                     out_hbm.at[0, :, c * TC:(c + 1) * TC], sem_out.at[c])

    wqkv_cp = pltpu.make_async_copy(wqkv_hbm, wqkv_s, sem_misc.at[0])
    wo_cp = pltpu.make_async_copy(wo_hbm, wo_s, sem_misc.at[1])
    b1_cp = pltpu.make_async_copy(b1_hbm, b1_s, sem_misc.at[2])
    b2_cp = pltpu.make_async_copy(b2_hbm, b2_s, sem_misc.at[3])

    for c in range(NC):
        x_cp(c).start()
        w1_cp(c).start()
        if c == 0:
            b1_cp.start()
            b2_cp.start()
        if c == 4:
            wqkv_cp.start()
            wo_cp.start()
    for c in range(NC):
        w2_cp(c).start()

    def prep_wqkv_t():
        for c in range(11):
            wd = min(LANES, 3 * D - c * LANES)
            blk = wqkv_s[:, c * LANES:c * LANES + wd].astype(f32).T
            for kt in range(4):
                kw = min(LANES, D - kt * LANES)
                wt32_s[kt, c * LANES:c * LANES + wd, 0:kw] = blk[:, kt * LANES:kt * LANES + kw]

    def prep_wqkv_perm():
        for sec in range(3):
            for d in range(DH):
                for kt in range(4):
                    kw = min(LANES, D - kt * LANES)
                    rows = wt32_s[kt, pl.ds(sec * D + d, H, stride=DH), :]
                    wqkvt_s[sec * D + d * H:sec * D + (d + 1) * H, kt * LANES:kt * LANES + kw] = (
                        rows[:, 0:kw].astype(bf16))

    def prep_wo():
        for nt in range(4):
            nw = min(LANES, D - nt * LANES)
            wo32_s[nt, :, 0:nw] = wo_s[:, nt * LANES:nt * LANES + nw].astype(f32)
        for nt in range(4):
            nw = min(LANES, D - nt * LANES)
            rows = [wo32_s[nt, pl.ds(d, H, stride=DH), :][:, 0:nw] for d in range(DH)]
            blk = jnp.concatenate(rows, axis=0)
            wot_s[nt * LANES:nt * LANES + nw, :] = blk.T.astype(bf16)

    for c in range(NC):
        x_cp(c).wait()
        hs = []
        for j in range(TC // LANES):
            col = pl.ds(c * TC + j * LANES, LANES)
            xn = _ln_cols(x_s[:, col].astype(f32))
            xn_s[:, col] = xn.astype(bf16)
            hs.append(_ln_cols(xn).astype(bf16))
        h = jnp.concatenate(hs, axis=1)
        w1_cp(c).wait()
        part = jnp.dot(h, w1_s[c * TC:(c + 1) * TC, :], preferred_element_type=f32)
        if c == 0:
            acc_s[...] = part
        else:
            acc_s[...] += part
        if c == 5:
            wqkv_cp.wait()
            wo_cp.wait()
            prep_wqkv_t()
        if c == 6:
            prep_wqkv_perm()
            prep_wo()

    b1_cp.wait()
    b2_cp.wait()
    b1f_s[...] = b1_s[...].astype(f32)
    b2f_s[...] = b2_s[...].astype(f32)

    def gelu_cols(n):
        col = pl.ds(n * LANES, LANES)
        u_s[:, col] = _gelu(acc_s[:, col] + b1f_s[n:n + 1, :]).astype(bf16)

    def qkv(c):
        r = jnp.dot(wqkvt_s[...], xn_s[:, c * TC:(c + 1) * TC], preferred_element_type=f32)
        for j in range(TC // LANES):
            qkv_s[c * (TC // LANES) + j + 1] = r[:, j * LANES:(j + 1) * LANES]

    scale = DH ** -0.5

    def attn_col(jj):
        lane = jax.lax.broadcasted_iota(jnp.int32, (SLAB, LANES), 1)
        m0 = [None] + [lane < LANES - 2 * a for a in range(1, 4)]
        m1 = [(lane >= 8) & (lane < LANES - 2 * a) for a in range(4)]
        nd = SLAB // H
        acc = [[None, None] for _ in range(4)]
        for sl in range(D // SLAB):
            r0 = sl * SLAB
            q = qkv_s[jj + 1, r0:r0 + SLAB, :]
            k = qkv_s[jj + 1, D + r0:D + r0 + SLAB, :]
            kp = qkv_s[jj, D + r0:D + r0 + SLAB, :]
            rkp = rk_s[jj % 2, r0:r0 + SLAB, :]
            rk = pltpu.roll(k, 8, 1)
            rk_s[(jj + 1) % 2, r0:r0 + SLAB, :] = rk
            for a in range(4):
                rq = q if a == 0 else pltpu.roll(q, LANES - 2 * a, 1)
                for b in range(2):
                    if b == 0:
                        mix = k if a == 0 else jnp.where(m0[a], k, kp)
                    else:
                        mix = jnp.where(m1[a], rk, rkp)
                    p = rq * mix
                    for i in range(nd):
                        pi = p[i * H:(i + 1) * H]
                        acc[a][b] = pi if acc[a][b] is None else acc[a][b] + pi
        lane16 = jax.lax.broadcasted_iota(jnp.int32, (H, LANES), 1)
        logit = []
        for w in range(W):
            a, b = w % 4, w // 4
            lw = acc[a][b] if a == 0 else pltpu.roll(acc[a][b], 2 * a, 1)
            lw = lw * scale
            if jj == 0 and w > 0:
                lw = jnp.where(lane16 >= 2 * w, lw, -1e9)
            logit.append(lw)
        mx = functools.reduce(jnp.maximum, logit)
        ex = [jnp.exp(l - mx) for l in logit]
        inv = 1.0 / functools.reduce(jnp.add, ex)
        ra = [[None, None] for _ in range(4)]
        for w in range(W):
            a, b = w % 4, w // 4
            aw = ex[w] * inv
            aw = aw if a == 0 else pltpu.roll(aw, LANES - 2 * a, 1)
            ra[a][b] = jnp.concatenate([aw] * nd, axis=0)
        for sl in range(D // SLAB):
            r0 = sl * SLAB
            v = qkv_s[jj + 1, 2 * D + r0:2 * D + r0 + SLAB, :]
            vp = qkv_s[jj, 2 * D + r0:2 * D + r0 + SLAB, :]
            rvp = rv_s[jj % 2, r0:r0 + SLAB, :]
            rv = pltpu.roll(v, 8, 1)
            rv_s[(jj + 1) % 2, r0:r0 + SLAB, :] = rv
            o = None
            for a in range(4):
                mix0 = v if a == 0 else jnp.where(m0[a], v, vp)
                mix1 = jnp.where(m1[a], rv, rvp)
                t = ra[a][0] * mix0 + ra[a][1] * mix1
                o = t if a == 0 else o + pltpu.roll(t, 2 * a, 1)
            o_s[r0:r0 + SLAB, jj * LANES:(jj + 1) * LANES] = o.astype(bf16)

    def attn(c):
        for j in range(TC // LANES):
            attn_col(c * (TC // LANES) + j)

    def final(c):
        cs = slice(c * TC, (c + 1) * TC)
        y = jnp.dot(u_s[...], w2_s[:, cs], preferred_element_type=f32)
        s = jnp.dot(wot_s[...], o_s[:, cs], preferred_element_type=f32)
        for j in range(TC // LANES):
            jj = c * (TC // LANES) + j
            col = pl.ds(jj * LANES, LANES)
            g = _silu(y[:, j * LANES:(j + 1) * LANES] + b2f_s[jj:jj + 1, :])
            r = x_s[:, col].astype(f32) + s[:, j * LANES:(j + 1) * LANES] * g
            out_s[:, col] = r.astype(bf16)
        out_cp(c).start()

    zeros = jnp.zeros((D, LANES), f32)
    qkv_s[0, D:2 * D, :] = zeros
    qkv_s[0, 2 * D:3 * D, :] = zeros
    rk_s[0] = zeros
    rv_s[0] = zeros

    qkv(0)
    for n in range(F // LANES):
        gelu_cols(n)
    for c in range(NC):
        if c + 1 < NC:
            qkv(c + 1)
        attn(c)
        if c >= 1:
            w2_cp(c - 1).wait()
            final(c - 1)
    w2_cp(NC - 1).wait()
    final(NC - 1)
    for c in range(NC):
        out_cp(c).wait()


@jax.jit
def pallas_recurrent_scan__sliding_local_dilated__mixer_token_mlp__prompt_kernel(
    A_x: jax.Array,
    A_wqkv: jax.Array,
    A_wo: jax.Array,
    B_x: jax.Array,
    B_w1: jax.Array,
    B_b1: jax.Array,
    B_w2: jax.Array,
    B_b2: jax.Array,
):
    del B_x
    xt = jnp.swapaxes(A_x, 1, 2)
    b1 = B_b1.reshape(F // LANES, LANES)
    b2 = B_b2.reshape(S // LANES, LANES)
    any_spec = pl.BlockSpec(memory_space=pl.ANY)
    out_t = pl.pallas_call(
        _kernel,
        out_shape=jax.ShapeDtypeStruct((1, D, S), bf16),
        in_specs=[any_spec] * 7,
        out_specs=any_spec,
        scratch_shapes=[
            pltpu.VMEM((D, S), bf16),
            pltpu.VMEM((D, 3 * D), bf16),
            pltpu.VMEM((D, D), bf16),
            pltpu.VMEM((S, F), bf16),
            pltpu.VMEM((F, S), bf16),
            pltpu.VMEM((F // LANES, LANES), bf16),
            pltpu.VMEM((S // LANES, LANES), bf16),
            pltpu.VMEM((D, S), bf16),
            pltpu.VMEM((D, F), f32),
            pltpu.VMEM((D, F), bf16),
            pltpu.VMEM((4, 11 * LANES, LANES), f32),
            pltpu.VMEM((3 * D, D), bf16),
            pltpu.VMEM((4, D, LANES), f32),
            pltpu.VMEM((D, D), bf16),
            pltpu.VMEM((NCOL + 1, 3 * D, LANES), f32),
            pltpu.VMEM((2, D, LANES), f32),
            pltpu.VMEM((2, D, LANES), f32),
            pltpu.VMEM((D, S), bf16),
            pltpu.VMEM((D, S), bf16),
            pltpu.VMEM((F // LANES, LANES), f32),
            pltpu.VMEM((S // LANES, LANES), f32),
            pltpu.SemaphoreType.DMA((NC,)),
            pltpu.SemaphoreType.DMA((NC,)),
            pltpu.SemaphoreType.DMA((NC,)),
            pltpu.SemaphoreType.DMA((4,)),
            pltpu.SemaphoreType.DMA((NC,)),
        ],
        compiler_params=pltpu.CompilerParams(vmem_limit_bytes=100 * 1024 * 1024),
        name="fused_mixer_attn",
    )(xt, A_wqkv, A_wo, B_w1, b1, B_w2, b2)
    return jnp.swapaxes(out_t, 1, 2)
```

```python
import functools

import jax
import jax.numpy as jnp
import jax.experimental.pallas as pl
import jax.experimental.pallas.tpu as pltpu

S = 2048
D = 448
H = 16
DH = D // H
F = 1792
W = 8
EPS = 1e-5
TC = 256
NC = S // TC
LANES = 128
NCOL = S // LANES
SLAB = 32

f32 = jnp.float32
bf16 = jnp.bfloat16


_SCOPES = False


def _scope(name, fn):
    if _SCOPES:
        with jax.named_scope(name):
            fn()
    else:
        fn()


def _ln_cols(x):
    m = jnp.sum(x, axis=0, keepdims=True) * (1.0 / D)
    xc = x - m
    v = jnp.sum(xc * xc, axis=0, keepdims=True) * (1.0 / D)
    return xc * jax.lax.rsqrt(v + EPS)


def _gelu(x):
    c = 0.7978845608028654
    t = jnp.tanh(x * (c + (c * 0.044715) * (x * x)))
    hx = 0.5 * x
    return hx + hx * t


def _silu(y):
    hy = 0.5 * y
    return hy + hy * jnp.tanh(hy)


PIECES = (128, 128, 256, 256, 384, 384, 512)
POFF = tuple(sum(PIECES[:i]) for i in range(len(PIECES) + 1))
NP = len(PIECES)
NB = 256
QKV_AHEAD = 4
OUT_PIECES = (256,) * 7 + (128, 128)
OOFF = tuple(sum(OUT_PIECES[:i]) for i in range(len(OUT_PIECES) + 1))
NO = len(OUT_PIECES)
SEM_X, SEM_W1, SEM_MISC, SEM_OUT = 0, NP, 2 * NP, 2 * NP + 5
NSEM = SEM_OUT + NO


def _kernel(x_hbm, wqkv_hbm, wo_hbm, w1_hbm, b1_hbm, w2_hbm, b2_hbm, out_hbm,
            x_s, wqkv_s, wo_s, w1_s, w2_s, b1_s, b2_s,
            xn_s, h_s, acc_s, u_s, wt32_s, wqkvt_s, wo32_s, wot_s,
            qkv_s, rk_s, rv_s, o_s, out_s, b1f_s, b2f_s, sem):
    def x_cp(p):
        sl = slice(POFF[p], POFF[p + 1])
        return pltpu.make_async_copy(x_hbm.at[0, :, sl], x_s.at[:, sl], sem.at[SEM_X + p])

    def w1_cp(p):
        sl = slice(POFF[p], POFF[p + 1])
        return pltpu.make_async_copy(w1_hbm.at[sl, :], w1_s.at[sl, :], sem.at[SEM_W1 + p])

    def out_cp(i):
        sl = slice(OOFF[i], OOFF[i + 1])
        return pltpu.make_async_copy(out_s.at[:, sl], out_hbm.at[0, :, sl], sem.at[SEM_OUT + i])

    wqkv_cp = pltpu.make_async_copy(wqkv_hbm, wqkv_s, sem.at[SEM_MISC + 0])
    wo_cp = pltpu.make_async_copy(wo_hbm, wo_s, sem.at[SEM_MISC + 1])
    b1_cp = pltpu.make_async_copy(b1_hbm, b1_s, sem.at[SEM_MISC + 2])
    b2_cp = pltpu.make_async_copy(b2_hbm, b2_s, sem.at[SEM_MISC + 3])
    w2_cp = pltpu.make_async_copy(w2_hbm, w2_s, sem.at[SEM_MISC + 4])

    x_cp(0).start()
    for p in range(NP):
        if p == NP - 1:
            wqkv_cp.start()
            wo_cp.start()
            b1_cp.start()
            b2_cp.start()
        w1_cp(p).start()
        if p + 1 < NP:
            x_cp(p + 1).start()
    w2_cp.start()

    def prep_wqkv_t():
        for c in range(11):
            wd = min(LANES, 3 * D - c * LANES)
            blk = wqkv_s[:, c * LANES:c * LANES + wd].astype(f32).T
            for kt in range(4):
                kw = min(LANES, D - kt * LANES)
                wt32_s[kt, c * LANES:c * LANES + wd, 0:kw] = blk[:, kt * LANES:kt * LANES + kw]

    def prep_wqkv_perm():
        for sec in range(3):
            for d in range(DH):
                for kt in range(4):
                    kw = min(LANES, D - kt * LANES)
                    rows = wt32_s[kt, pl.ds(sec * D + d, H, stride=DH), :]
                    wqkvt_s[sec * D + d * H:sec * D + (d + 1) * H, kt * LANES:kt * LANES + kw] = (
                        rows[:, 0:kw].astype(bf16))

    def prep_wo():
        for nt in range(4):
            nw = min(LANES, D - nt * LANES)
            wo32_s[nt, :, 0:nw] = wo_s[:, nt * LANES:nt * LANES + nw].astype(f32)
        for nt in range(4):
            nw = min(LANES, D - nt * LANES)
            rows = [wo32_s[nt, pl.ds(d, H, stride=DH), :][:, 0:nw] for d in range(DH)]
            blk = jnp.concatenate(rows, axis=0)
            wot_s[nt * LANES:nt * LANES + nw, :] = blk.T.astype(bf16)

    def ln_piece(p):
        for jj in range(POFF[p] // LANES, POFF[p + 1] // LANES):
            col = pl.ds(jj * LANES, LANES)
            xn = _ln_cols(x_s[:, col].astype(f32))
            xn_s[:, col] = xn.astype(bf16)
            h_s[:, col] = _ln_cols(xn).astype(bf16)

    def mix1(p):
        sl = slice(POFF[p], POFF[p + 1])
        for n in range(F // NB):
            ns = slice(n * NB, (n + 1) * NB)
            part = jnp.dot(h_s[:, sl], w1_s[sl, ns], preferred_element_type=f32)
            if p == 0:
                acc_s[:, ns] = part
            elif p < NP - 1:
                acc_s[:, ns] += part
            else:
                for j in range(NB // LANES):
                    nn = n * (NB // LANES) + j
                    col = pl.ds(nn * LANES, LANES)
                    z = acc_s[:, col] + part[:, j * LANES:(j + 1) * LANES] + b1f_s[nn:nn + 1, :]
                    u_s[:, col] = _gelu(z).astype(bf16)

    _scope("wx0", lambda: x_cp(0).wait())
    ln_piece(0)
    for p in range(NP):
        def waits():
            if p == NP - 1:
                wqkv_cp.wait()
                wo_cp.wait()
                b1_cp.wait()
                b2_cp.wait()
            w1_cp(p).wait()
            if p + 1 < NP:
                x_cp(p + 1).wait()
        _scope(f"w{p}", waits)
        if p == NP - 1:
            b1f_s[...] = b1_s[...].astype(f32)
            b2f_s[...] = b2_s[...].astype(f32)
            prep_wqkv_t()
            prep_wqkv_perm()
            prep_wo()
        mix1(p)
        if p + 1 < NP:
            ln_piece(p + 1)

    def qkv(c):
        r = jnp.dot(wqkvt_s[...], xn_s[:, c * TC:(c + 1) * TC], preferred_element_type=f32)
        for j in range(TC // LANES):
            qkv_s[c * (TC // LANES) + j + 1] = r[:, j * LANES:(j + 1) * LANES]

    scale = DH ** -0.5

    def attn_col(jj):
        lane = jax.lax.broadcasted_iota(jnp.int32, (SLAB, LANES), 1)
        m0 = [None] + [lane < LANES - 2 * a for a in range(1, 4)]
        m1 = [(lane >= 8) & (lane < LANES - 2 * a) for a in range(4)]
        nd = SLAB // H
        acc = [[None, None] for _ in range(4)]
        for sl in range(D // SLAB):
            r0 = sl * SLAB
            q = qkv_s[jj + 1, r0:r0 + SLAB, :]
            k = qkv_s[jj + 1, D + r0:D + r0 + SLAB, :]
            kp = qkv_s[jj, D + r0:D + r0 + SLAB, :]
            rkp = rk_s[jj % 2, r0:r0 + SLAB, :]
            rk = pltpu.roll(k, 8, 1)
            rk_s[(jj + 1) % 2, r0:r0 + SLAB, :] = rk
            for a in range(4):
                rq = q if a == 0 else pltpu.roll(q, LANES - 2 * a, 1)
                for b in range(2):
                    if b == 0:
                        mix = k if a == 0 else jnp.where(m0[a], k, kp)
                    else:
                        mix = jnp.where(m1[a], rk, rkp)
                    p = rq * mix
                    for i in range(nd):
                        pi = p[i * H:(i + 1) * H]
                        acc[a][b] = pi if acc[a][b] is None else acc[a][b] + pi
        lane16 = jax.lax.broadcasted_iota(jnp.int32, (H, LANES), 1)
        logit = []
        for w in range(W):
            a, b = w % 4, w // 4
            lw = acc[a][b] if a == 0 else pltpu.roll(acc[a][b], 2 * a, 1)
            lw = lw * scale
            if jj == 0 and w > 0:
                lw = jnp.where(lane16 >= 2 * w, lw, -1e9)
            logit.append(lw)
        mx = functools.reduce(jnp.maximum, logit)
        ex = [jnp.exp(l - mx) for l in logit]
        inv = 1.0 / functools.reduce(jnp.add, ex)
        ra = [[None, None] for _ in range(4)]
        for w in range(W):
            a, b = w % 4, w // 4
            aw = ex[w] * inv
            aw = aw if a == 0 else pltpu.roll(aw, LANES - 2 * a, 1)
            ra[a][b] = jnp.concatenate([aw] * nd, axis=0)
        for sl in range(D // SLAB):
            r0 = sl * SLAB
            v = qkv_s[jj + 1, 2 * D + r0:2 * D + r0 + SLAB, :]
            vp = qkv_s[jj, 2 * D + r0:2 * D + r0 + SLAB, :]
            rvp = rv_s[jj % 2, r0:r0 + SLAB, :]
            rv = pltpu.roll(v, 8, 1)
            rv_s[(jj + 1) % 2, r0:r0 + SLAB, :] = rv
            o = None
            for a in range(4):
                mix0 = v if a == 0 else jnp.where(m0[a], v, vp)
                mix1 = jnp.where(m1[a], rv, rvp)
                t = ra[a][0] * mix0 + ra[a][1] * mix1
                o = t if a == 0 else o + pltpu.roll(t, 2 * a, 1)
            o_s[r0:r0 + SLAB, jj * LANES:(jj + 1) * LANES] = o.astype(bf16)

    def attn(c):
        for j in range(TC // LANES):
            attn_col(c * (TC // LANES) + j)

    def final(i):
        cs = slice(OOFF[i], OOFF[i + 1])
        y = jnp.dot(u_s[...], w2_s[:, cs], preferred_element_type=f32)
        s = jnp.dot(wot_s[...], o_s[:, cs], preferred_element_type=f32)
        for j in range(OUT_PIECES[i] // LANES):
            jj = OOFF[i] // LANES + j
            col = pl.ds(jj * LANES, LANES)
            g = _silu(y[:, j * LANES:(j + 1) * LANES] + b2f_s[jj:jj + 1, :])
            r = x_s[:, col].astype(f32) + s[:, j * LANES:(j + 1) * LANES] * g
            out_s[:, col] = r.astype(bf16)
        out_cp(i).start()

    zeros = jnp.zeros((D, LANES), f32)
    qkv_s[0, D:2 * D, :] = zeros
    qkv_s[0, 2 * D:3 * D, :] = zeros
    rk_s[0] = zeros
    rv_s[0] = zeros

    for c in range(QKV_AHEAD):
        qkv(c)
        if c >= 1:
            attn(c - 1)
    _scope("ww2", lambda: w2_cp.wait())
    for c in range(NC):
        if c + QKV_AHEAD - 1 < NC:
            attn(c + QKV_AHEAD - 1)
        final(c)
        if c + QKV_AHEAD < NC:
            qkv(c + QKV_AHEAD)
    final(NC)
    def waits():
        for i in range(NO):
            out_cp(i).wait()
    _scope("wout", waits)


@jax.jit
def pallas_recurrent_scan__sliding_local_dilated__mixer_token_mlp__prompt_kernel(
    A_x: jax.Array,
    A_wqkv: jax.Array,
    A_wo: jax.Array,
    B_x: jax.Array,
    B_w1: jax.Array,
    B_b1: jax.Array,
    B_w2: jax.Array,
    B_b2: jax.Array,
):
    del B_x
    xt = jnp.swapaxes(A_x, 1, 2)
    b1 = B_b1.reshape(F // LANES, LANES)
    b2 = B_b2.reshape(S // LANES, LANES)
    any_spec = pl.BlockSpec(memory_space=pl.ANY)
    out_t = pl.pallas_call(
        _kernel,
        out_shape=jax.ShapeDtypeStruct((1, D, S), bf16),
        in_specs=[any_spec] * 7,
        out_specs=any_spec,
        scratch_shapes=[
            pltpu.VMEM((D, S), bf16),
            pltpu.VMEM((D, 3 * D), bf16),
            pltpu.VMEM((D, D), bf16),
            pltpu.VMEM((S, F), bf16),
            pltpu.VMEM((F, S), bf16),
            pltpu.VMEM((F // LANES, LANES), bf16),
            pltpu.VMEM((S // LANES, LANES), bf16),
            pltpu.VMEM((D, S), bf16),
            pltpu.VMEM((D, S), bf16),
            pltpu.VMEM((D, F), f32),
            pltpu.VMEM((D, F), bf16),
            pltpu.VMEM((4, 11 * LANES, LANES), f32),
            pltpu.VMEM((3 * D, D), bf16),
            pltpu.VMEM((4, D, LANES), f32),
            pltpu.VMEM((D, D), bf16),
            pltpu.VMEM((NCOL + 1, 3 * D, LANES), f32),
            pltpu.VMEM((2, D, LANES), f32),
            pltpu.VMEM((2, D, LANES), f32),
            pltpu.VMEM((D, S), bf16),
            pltpu.VMEM((D, S), bf16),
            pltpu.VMEM((F // LANES, LANES), f32),
            pltpu.VMEM((S // LANES, LANES), f32),
            pltpu.SemaphoreType.DMA((NSEM,)),
        ],
        compiler_params=pltpu.CompilerParams(vmem_limit_bytes=100 * 1024 * 1024),
        name="fused_mixer_attn",
    )(xt, A_wqkv, A_wo, B_w1, b1, B_w2, b2)
    return jnp.swapaxes(out_t, 1, 2)
```

```python
import functools

import jax
import jax.numpy as jnp
import jax.experimental.pallas as pl
import jax.experimental.pallas.tpu as pltpu

S = 2048
D = 448
H = 16
DH = D // H
F = 1792
W = 8
EPS = 1e-5
TC = 256
NC = S // TC
LANES = 128
NCOL = S // LANES
SLAB = 32

f32 = jnp.float32
bf16 = jnp.bfloat16
u32 = jnp.uint32

_SCOPES = False


def _scope(name, fn):
    if _SCOPES:
        with jax.named_scope(name):
            fn()
    else:
        fn()


LNB = 64


def _ln_stats(x_ref, col):
    piv = x_ref[0:1, col].astype(f32)
    s1 = s2 = None
    for i in range(D // LNB):
        w = pltpu.bitcast(x_ref[i * LNB:(i + 1) * LNB, col], u32)
        for half in (w << 16, w & jnp.uint32(0xFFFF0000)):
            d = pltpu.bitcast(half, f32) - piv
            for k in range(LNB // 2 // 16):
                dk = d[k * 16:(k + 1) * 16]
                s1 = dk if s1 is None else s1 + dk
                s2 = dk * dk if s2 is None else s2 + dk * dk
    md = jnp.sum(s1, axis=0, keepdims=True) * (1.0 / D)
    v = jnp.maximum(jnp.sum(s2, axis=0, keepdims=True) * (1.0 / D) - md * md, 0.0)
    r = jax.lax.rsqrt(v + EPS)
    r2 = jax.lax.rsqrt(v * r * r + EPS)
    return piv + md, r, r * r2


def _gelu(x):
    c = 0.7978845608028654
    t = jnp.tanh(x * (c + (c * 0.044715) * (x * x)))
    hx = 0.5 * x
    return hx + hx * t


def _silu(y):
    hy = 0.5 * y
    return hy + hy * jnp.tanh(hy)


PIECES = (256, 256, 256, 256, 512, 512)
N0 = 768
POFF = tuple(sum(PIECES[:i]) for i in range(len(PIECES) + 1))
NP = len(PIECES)
NB = 256
QKV_AHEAD = 4
OUT_PIECES = (256,) * 7 + (128, 128)
OOFF = tuple(sum(OUT_PIECES[:i]) for i in range(len(OUT_PIECES) + 1))
NO = len(OUT_PIECES)
SEM_X, SEM_W1, SEM_MISC, SEM_OUT = 0, NP, 2 * NP, 2 * NP + 6
NSEM = SEM_OUT + NO


def _kernel(x_hbm, wqkv_hbm, wo_hbm, w1_hbm, b1_hbm, w2_hbm, b2_hbm, out_hbm,
            x_s, wqkv_s, wo_s, w1_s, w2_s, b1_s, b2_s,
            xn_s, h_s, acc_s, u_s, wt32_s, wqkvt_s, wo32_s, wot_s,
            qkv_s, rk_s, rv_s, o_s, out_s, b1f_s, b2f_s, sem):
    xn_s, h_s, u_s, wqkvt_s, wot_s, o_s = (
        r.bitcast(bf16) for r in (xn_s, h_s, u_s, wqkvt_s, wot_s, o_s))

    def x_cp(p):
        sl = slice(POFF[p], POFF[p + 1])
        return pltpu.make_async_copy(x_hbm.at[0, :, sl], x_s.at[:, sl], sem.at[SEM_X + p])

    def w1_cp(p):
        sl = slice(POFF[p], POFF[p + 1])
        ns = slice(N0, F) if p == 0 else slice(0, F)
        return pltpu.make_async_copy(w1_hbm.at[sl, ns], w1_s.at[sl, ns], sem.at[SEM_W1 + p])

    def out_cp(i):
        sl = slice(OOFF[i], OOFF[i + 1])
        return pltpu.make_async_copy(out_s.at[:, sl], out_hbm.at[0, :, sl], sem.at[SEM_OUT + i])

    wqkv_cp = pltpu.make_async_copy(wqkv_hbm, wqkv_s, sem.at[SEM_MISC + 0])
    wo_cp = pltpu.make_async_copy(wo_hbm, wo_s, sem.at[SEM_MISC + 1])
    b1_cp = pltpu.make_async_copy(b1_hbm, b1_s, sem.at[SEM_MISC + 2])
    b2_cp = pltpu.make_async_copy(b2_hbm, b2_s, sem.at[SEM_MISC + 3])
    w2_cp = pltpu.make_async_copy(w2_hbm, w2_s, sem.at[SEM_MISC + 4])
    w1a_cp = pltpu.make_async_copy(w1_hbm.at[0:PIECES[0], 0:N0], w1_s.at[0:PIECES[0], 0:N0],
                                   sem.at[SEM_MISC + 5])

    x_cp(0).start()
    w1a_cp.start()
    for p in range(NP):
        if p == NP - 1:
            wqkv_cp.start()
            wo_cp.start()
            b1_cp.start()
            b2_cp.start()
        w1_cp(p).start()
        if p + 1 < NP:
            x_cp(p + 1).start()
    w2_cp.start()

    def prep_wqkv_t():
        for c in range(11):
            wd = min(LANES, 3 * D - c * LANES)
            blk = wqkv_s[:, c * LANES:c * LANES + wd].T.astype(f32)
            for kt in range(4):
                kw = min(LANES, D - kt * LANES)
                wt32_s[kt, c * LANES:c * LANES + wd, 0:kw] = blk[:, kt * LANES:kt * LANES + kw]

    def prep_wqkv_perm():
        for sec in range(3):
            for d in range(DH):
                r0 = sec * D + d * H
                for kt in range(4):
                    kw = min(LANES, D - kt * LANES)
                    rows = wt32_s[kt, pl.ds(sec * D + d, H, stride=DH), :]
                    wqkvt_s[r0:r0 + H, kt * LANES:kt * LANES + kw] = rows[:, 0:kw].astype(bf16)

    def prep_wo():
        for nt in range(4):
            nw = min(LANES, D - nt * LANES)
            wo32_s[nt, :, 0:nw] = wo_s[:, nt * LANES:nt * LANES + nw].astype(f32)
        for nt in range(4):
            nw = min(LANES, D - nt * LANES)
            rows = [wo32_s[nt, pl.ds(d, H, stride=DH), :][:, 0:nw].astype(bf16) for d in range(DH)]
            blk = jnp.concatenate(rows, axis=0)
            wot_s[nt * LANES:nt * LANES + nw, :] = blk.T

    def ln_piece(p):
        for jj in range(POFF[p] // LANES, POFF[p + 1] // LANES):
            col = pl.ds(jj * LANES, LANES)
            m, r, rr = _ln_stats(x_s, col)
            for i in range(D // LNB):
                rows = slice(i * LNB, (i + 1) * LNB)
                xc = x_s[rows, col].astype(f32) - m
                xn_s[rows, col] = (xc * r).astype(bf16)
                h_s[rows, col] = (xc * rr).astype(bf16)

    def mix1(p, n_lo, n_hi):
        sl = slice(POFF[p], POFF[p + 1])
        for n in range(n_lo // NB, n_hi // NB):
            ns = slice(n * NB, (n + 1) * NB)
            part = jnp.dot(h_s[:, sl], w1_s[sl, ns], preferred_element_type=f32)
            if p == 0:
                acc_s[:, ns] = part
            elif p < NP - 1:
                acc_s[:, ns] += part
            else:
                for j in range(NB // LANES):
                    nn = n * (NB // LANES) + j
                    col = pl.ds(nn * LANES, LANES)
                    z = acc_s[:, col] + part[:, j * LANES:(j + 1) * LANES] + b1f_s[nn:nn + 1, :]
                    u_s[:, col] = _gelu(z).astype(bf16)

    _scope("wx0", lambda: x_cp(0).wait())
    ln_piece(0)
    _scope("w0a", lambda: w1a_cp.wait())
    mix1(0, 0, N0)
    for p in range(NP):
        def waits():
            if p == NP - 1:
                wqkv_cp.wait()
                wo_cp.wait()
                b1_cp.wait()
                b2_cp.wait()
            w1_cp(p).wait()
            if p + 1 < NP:
                x_cp(p + 1).wait()
        _scope(f"w{p}", waits)
        if p == NP - 1:
            b1f_s[...] = b1_s[...].astype(f32)
            b2f_s[...] = b2_s[...].astype(f32)
            prep_wqkv_t()
            prep_wqkv_perm()
            prep_wo()
        mix1(p, N0 if p == 0 else 0, F)
        if p + 1 < NP:
            ln_piece(p + 1)

    def qkv(c):
        r = jnp.dot(wqkvt_s[...], xn_s[:, c * TC:(c + 1) * TC],
                    preferred_element_type=f32)
        for j in range(TC // LANES):
            qkv_s[c * (TC // LANES) + j + 1] = r[:, j * LANES:(j + 1) * LANES]

    scale = DH ** -0.5

    def attn_col(jj):
        lane = jax.lax.broadcasted_iota(jnp.int32, (SLAB, LANES), 1)
        m0 = [None] + [lane < LANES - 2 * a for a in range(1, 4)]
        m1 = [(lane >= 8) & (lane < LANES - 2 * a) for a in range(4)]
        nd = SLAB // H
        acc = [[None, None] for _ in range(4)]
        for sl in range(D // SLAB):
            r0 = sl * SLAB
            q = qkv_s[jj + 1, r0:r0 + SLAB, :]
            k = qkv_s[jj + 1, D + r0:D + r0 + SLAB, :]
            kp = qkv_s[jj, D + r0:D + r0 + SLAB, :]
            rkp = rk_s[jj % 2, r0:r0 + SLAB, :]
            rk = pltpu.roll(k, 8, 1)
            rk_s[(jj + 1) % 2, r0:r0 + SLAB, :] = rk
            for a in range(4):
                rq = q if a == 0 else pltpu.roll(q, LANES - 2 * a, 1)
                for b in range(2):
                    if b == 0:
                        mix = k if a == 0 else jnp.where(m0[a], k, kp)
                    else:
                        mix = jnp.where(m1[a], rk, rkp)
                    p = rq * mix
                    for i in range(nd):
                        pi = p[i * H:(i + 1) * H]
                        acc[a][b] = pi if acc[a][b] is None else acc[a][b] + pi
        lane16 = jax.lax.broadcasted_iota(jnp.int32, (H, LANES), 1)
        logit = []
        for w in range(W):
            a, b = w % 4, w // 4
            lw = acc[a][b] if a == 0 else pltpu.roll(acc[a][b], 2 * a, 1)
            lw = lw * scale
            if jj == 0 and w > 0:
                lw = jnp.where(lane16 >= 2 * w, lw, -1e9)
            logit.append(lw)
        mx = functools.reduce(jnp.maximum, logit)
        ex = [jnp.exp(l - mx) for l in logit]
        inv = 1.0 / functools.reduce(jnp.add, ex)
        ra = [[None, None] for _ in range(4)]
        for w in range(W):
            a, b = w % 4, w // 4
            aw = ex[w] * inv
            aw = aw if a == 0 else pltpu.roll(aw, LANES - 2 * a, 1)
            ra[a][b] = jnp.concatenate([aw] * nd, axis=0)
        for sl in range(D // SLAB):
            r0 = sl * SLAB
            v = qkv_s[jj + 1, 2 * D + r0:2 * D + r0 + SLAB, :]
            vp = qkv_s[jj, 2 * D + r0:2 * D + r0 + SLAB, :]
            rvp = rv_s[jj % 2, r0:r0 + SLAB, :]
            rv = pltpu.roll(v, 8, 1)
            rv_s[(jj + 1) % 2, r0:r0 + SLAB, :] = rv
            o = None
            for a in range(4):
                mix0 = v if a == 0 else jnp.where(m0[a], v, vp)
                mix1 = jnp.where(m1[a], rv, rvp)
                t = ra[a][0] * mix0 + ra[a][1] * mix1
                o = t if a == 0 else o + pltpu.roll(t, 2 * a, 1)
            o_s[r0:r0 + SLAB, jj * LANES:(jj + 1) * LANES] = o.astype(bf16)

    def attn(c):
        for j in range(TC // LANES):
            attn_col(c * (TC // LANES) + j)

    def final(i):
        cs = slice(OOFF[i], OOFF[i + 1])
        y = jnp.dot(u_s[...], w2_s[:, cs], preferred_element_type=f32)
        s = jnp.dot(wot_s[...], o_s[:, cs], preferred_element_type=f32)
        for j in range(OUT_PIECES[i] // LANES):
            jj = OOFF[i] // LANES + j
            col = pl.ds(jj * LANES, LANES)
            g = _silu(y[:, j * LANES:(j + 1) * LANES] + b2f_s[jj:jj + 1, :])
            r = x_s[:, col].astype(f32) + s[:, j * LANES:(j + 1) * LANES] * g
            out_s[:, col] = r.astype(bf16)
        out_cp(i).start()

    zeros = jnp.zeros((D, LANES), f32)
    qkv_s[0, D:2 * D, :] = zeros
    qkv_s[0, 2 * D:3 * D, :] = zeros
    rk_s[0] = zeros
    rv_s[0] = zeros

    for c in range(QKV_AHEAD):
        qkv(c)
        if c >= 1:
            attn(c - 1)
    _scope("ww2", lambda: w2_cp.wait())
    for c in range(NC):
        if c + QKV_AHEAD - 1 < NC:
            attn(c + QKV_AHEAD - 1)
        final(c)
        if c + QKV_AHEAD < NC:
            qkv(c + QKV_AHEAD)
    final(NC)

    def waits():
        for i in range(NO):
            out_cp(i).wait()
    _scope("wout", waits)


@jax.jit
def pallas_recurrent_scan__sliding_local_dilated__mixer_token_mlp__prompt_kernel(
    A_x: jax.Array,
    A_wqkv: jax.Array,
    A_wo: jax.Array,
    B_x: jax.Array,
    B_w1: jax.Array,
    B_b1: jax.Array,
    B_w2: jax.Array,
    B_b2: jax.Array,
):
    del B_x
    xt = jnp.swapaxes(A_x, 1, 2)
    b1 = B_b1.reshape(F // LANES, LANES)
    b2 = B_b2.reshape(S // LANES, LANES)
    any_spec = pl.BlockSpec(memory_space=pl.ANY)
    out_t = pl.pallas_call(
        _kernel,
        out_shape=jax.ShapeDtypeStruct((1, D, S), bf16),
        in_specs=[any_spec] * 7,
        out_specs=any_spec,
        scratch_shapes=[
            pltpu.VMEM((D, S), bf16),
            pltpu.VMEM((D, 3 * D), bf16),
            pltpu.VMEM((D, D), bf16),
            pltpu.VMEM((S, F), bf16),
            pltpu.VMEM((F, S), bf16),
            pltpu.VMEM((F // LANES, LANES), bf16),
            pltpu.VMEM((S // LANES, LANES), bf16),
            pltpu.VMEM((D // 2, S), u32),
            pltpu.VMEM((D // 2, S), u32),
            pltpu.VMEM((D, F), f32),
            pltpu.VMEM((D // 2, F), u32),
            pltpu.VMEM((4, 11 * LANES, LANES), f32),
            pltpu.VMEM((3 * D // 2, D), u32),
            pltpu.VMEM((4, D, LANES), f32),
            pltpu.VMEM((D // 2, D), u32),
            pltpu.VMEM((NCOL + 1, 3 * D, LANES), f32),
            pltpu.VMEM((2, D, LANES), f32),
            pltpu.VMEM((2, D, LANES), f32),
            pltpu.VMEM((D // 2, S), u32),
            pltpu.VMEM((D, S), bf16),
            pltpu.VMEM((F // LANES, LANES), f32),
            pltpu.VMEM((S // LANES, LANES), f32),
            pltpu.SemaphoreType.DMA((NSEM,)),
        ],
        compiler_params=pltpu.CompilerParams(vmem_limit_bytes=100 * 1024 * 1024),
        name="fused_mixer_attn",
    )(xt, A_wqkv, A_wo, B_w1, b1, B_w2, b2)
    return jnp.swapaxes(out_t, 1, 2)
```

```python
import functools

import jax
import jax.numpy as jnp
import jax.experimental.pallas as pl
import jax.experimental.pallas.tpu as pltpu

S = 2048
D = 448
H = 16
DH = D // H
F = 1792
W = 8
EPS = 1e-5
TC = 256
NC = S // TC
LANES = 128
NCOL = S // LANES
SLAB = 32

f32 = jnp.float32
bf16 = jnp.bfloat16
u32 = jnp.uint32

_SCOPES = False


def _scope(name, fn):
    if _SCOPES:
        with jax.named_scope(name):
            fn()
    else:
        fn()


LNB = 64
NLB = D // LNB


def _rep(v8, rows):
    return jnp.concatenate([v8] * (rows // 8), axis=0)


def _ln_stats(x_ref, col, pace):
    piv = jnp.broadcast_to(x_ref[0:1, col].astype(f32), (8, LANES))
    s1 = s2 = None
    for i in range(NLB):
        pv = _rep(pace(piv), LNB // 2)
        w = pltpu.bitcast(x_ref[i * LNB:(i + 1) * LNB, col], u32)
        for half in (w << 16, w & jnp.uint32(0xFFFF0000)):
            d = pltpu.bitcast(half, f32) - pv
            for k in range(LNB // 2 // 16):
                dk = d[k * 16:(k + 1) * 16]
                s1 = dk if s1 is None else s1 + dk
                s2 = dk * dk if s2 is None else s2 + dk * dk
    md = jnp.sum(s1, axis=0, keepdims=True) * (1.0 / D)
    v = jnp.maximum(jnp.sum(s2, axis=0, keepdims=True) * (1.0 / D) - md * md, 0.0)
    r = jax.lax.rsqrt(v + EPS)
    r2 = jax.lax.rsqrt(v * r * r + EPS)
    return piv + md, r, r * r2


class _Pacer:
    def __init__(self, tokens, count, never):
        self.tokens, self.count, self.never, self.i = tokens, count, never, 0

    def __call__(self, v8):
        if not self.tokens:
            return v8
        tok = self.tokens[self.i * len(self.tokens) // self.count]
        self.i += 1
        return jnp.where(self.never, tok, v8)


def _gelu(x):
    c = 0.7978845608028654
    t = jnp.tanh(x * (c + (c * 0.044715) * (x * x)))
    hx = 0.5 * x
    return hx + hx * t


def _silu(y):
    hy = 0.5 * y
    return hy + hy * jnp.tanh(hy)


PIECES = (256, 256, 256, 256, 512, 512)
N0 = 768
POFF = tuple(sum(PIECES[:i]) for i in range(len(PIECES) + 1))
NP = len(PIECES)
NB = 256
QKV_AHEAD = 4
OUT_PIECES = (256,) * 7 + (128, 128)
OOFF = tuple(sum(OUT_PIECES[:i]) for i in range(len(OUT_PIECES) + 1))
NO = len(OUT_PIECES)
SEM_X, SEM_W1, SEM_MISC, SEM_OUT = 0, NP, 2 * NP, 2 * NP + 6
NSEM = SEM_OUT + NO


def _kernel(x_hbm, wqkv_hbm, wo_hbm, w1_hbm, b1_hbm, w2_hbm, b2_hbm, out_hbm,
            x_s, wqkv_s, wo_s, w1_s, w2_s, b1_s, b2_s,
            xn_s, h_s, acc_s, u_s, wt32_s, wqkvt_s, wo32_s, wot_s,
            qkv_s, rk_s, rv_s, o_s, out_s, b1f_s, b2f_s, sem):
    xn_s, h_s, u_s, wqkvt_s, wot_s, o_s = (
        r.bitcast(bf16) for r in (xn_s, h_s, u_s, wqkvt_s, wot_s, o_s))

    def x_cp(p):
        sl = slice(POFF[p], POFF[p + 1])
        return pltpu.make_async_copy(x_hbm.at[0, :, sl], x_s.at[:, sl], sem.at[SEM_X + p])

    def w1_cp(p):
        sl = slice(POFF[p], POFF[p + 1])
        ns = slice(N0, F) if p == 0 else slice(0, F)
        return pltpu.make_async_copy(w1_hbm.at[sl, ns], w1_s.at[sl, ns], sem.at[SEM_W1 + p])

    def out_cp(i):
        sl = slice(OOFF[i], OOFF[i + 1])
        return pltpu.make_async_copy(out_s.at[:, sl], out_hbm.at[0, :, sl], sem.at[SEM_OUT + i])

    wqkv_cp = pltpu.make_async_copy(wqkv_hbm, wqkv_s, sem.at[SEM_MISC + 0])
    wo_cp = pltpu.make_async_copy(wo_hbm, wo_s, sem.at[SEM_MISC + 1])
    b1_cp = pltpu.make_async_copy(b1_hbm, b1_s, sem.at[SEM_MISC + 2])
    b2_cp = pltpu.make_async_copy(b2_hbm, b2_s, sem.at[SEM_MISC + 3])
    w2_cp = pltpu.make_async_copy(w2_hbm, w2_s, sem.at[SEM_MISC + 4])
    w1a_cp = pltpu.make_async_copy(w1_hbm.at[0:PIECES[0], 0:N0], w1_s.at[0:PIECES[0], 0:N0],
                                   sem.at[SEM_MISC + 5])

    x_cp(0).start()
    w1a_cp.start()
    for p in range(NP):
        if p == NP - 1:
            wqkv_cp.start()
            wo_cp.start()
            b1_cp.start()
            b2_cp.start()
        w1_cp(p).start()
        if p + 1 < NP:
            x_cp(p + 1).start()
    w2_cp.start()

    def prep_wqkv_t():
        for c in range(11):
            wd = min(LANES, 3 * D - c * LANES)
            blk = wqkv_s[:, c * LANES:c * LANES + wd].T.astype(f32)
            for kt in range(4):
                kw = min(LANES, D - kt * LANES)
                wt32_s[kt, c * LANES:c * LANES + wd, 0:kw] = blk[:, kt * LANES:kt * LANES + kw]

    def prep_wqkv_perm():
        for sec in range(3):
            for d in range(DH):
                r0 = sec * D + d * H
                for kt in range(4):
                    kw = min(LANES, D - kt * LANES)
                    rows = wt32_s[kt, pl.ds(sec * D + d, H, stride=DH), :]
                    wqkvt_s[r0:r0 + H, kt * LANES:kt * LANES + kw] = rows[:, 0:kw].astype(bf16)

    def prep_wo():
        for nt in range(4):
            nw = min(LANES, D - nt * LANES)
            wo32_s[nt, :, 0:nw] = wo_s[:, nt * LANES:nt * LANES + nw].astype(f32)
        for nt in range(4):
            nw = min(LANES, D - nt * LANES)
            rows = [wo32_s[nt, pl.ds(d, H, stride=DH), :][:, 0:nw].astype(bf16) for d in range(DH)]
            blk = jnp.concatenate(rows, axis=0)
            wot_s[nt * LANES:nt * LANES + nw, :] = blk.T

    def ln_piece(p, tokens):
        cols = range(POFF[p] // LANES, POFF[p + 1] // LANES)
        z = x_s[0:8, 0:LANES].astype(f32)
        pace = _Pacer(tokens, 2 * NLB * len(cols), z + 1.0 < z)
        for jj in cols:
            col = pl.ds(jj * LANES, LANES)
            m, r, rr = _ln_stats(x_s, col, pace)
            for i in range(NLB):
                rows = slice(i * LNB, (i + 1) * LNB)
                xc = x_s[rows, col].astype(f32) - _rep(pace(m), LNB)
                xn_s[rows, col] = (xc * r).astype(bf16)
                h_s[rows, col] = (xc * rr).astype(bf16)

    def mix1(p, n_lo, n_hi):
        sl = slice(POFF[p], POFF[p + 1])
        tokens = []
        for n in range(n_lo // NB, n_hi // NB):
            ns = slice(n * NB, (n + 1) * NB)
            part = jnp.dot(h_s[:, sl], w1_s[sl, ns], preferred_element_type=f32)
            if PIECES[p] == 2 * LANES:
                tokens += [part[r:r + 8, 0:LANES] for r in range(0, D, 8)]
            else:
                tokens += [part[r:r + 8, j * LANES:(j + 1) * LANES]
                           for j in range(NB // LANES) for r in range(0, D, 8)]
            if p == 0:
                acc_s[:, ns] = part
            elif p < NP - 1:
                acc_s[:, ns] += part
            else:
                for j in range(NB // LANES):
                    nn = n * (NB // LANES) + j
                    col = pl.ds(nn * LANES, LANES)
                    z = acc_s[:, col] + part[:, j * LANES:(j + 1) * LANES] + b1f_s[nn:nn + 1, :]
                    u_s[:, col] = _gelu(z).astype(bf16)
        return tokens

    _scope("wx0", lambda: x_cp(0).wait())
    ln_piece(0, [])
    _scope("w0a", lambda: w1a_cp.wait())
    mix1(0, 0, N0)
    for p in range(NP):
        def waits():
            if p == NP - 1:
                wqkv_cp.wait()
                wo_cp.wait()
                b1_cp.wait()
                b2_cp.wait()
            w1_cp(p).wait()
            if p + 1 < NP:
                x_cp(p + 1).wait()
        _scope(f"w{p}", waits)
        if p == NP - 1:
            b1f_s[...] = b1_s[...].astype(f32)
            b2f_s[...] = b2_s[...].astype(f32)
            prep_wqkv_t()
            prep_wqkv_perm()
            prep_wo()
        tokens = mix1(p, N0 if p == 0 else 0, F)
        if p + 1 < NP:
            ln_piece(p + 1, tokens[:len(tokens) * 7 // 8])

    def qkv(c):
        r = jnp.dot(wqkvt_s[...], xn_s[:, c * TC:(c + 1) * TC],
                    preferred_element_type=f32)
        for j in range(TC // LANES):
            qkv_s[c * (TC // LANES) + j + 1] = r[:, j * LANES:(j + 1) * LANES]

    scale = DH ** -0.5

    def attn_col(jj):
        lane = jax.lax.broadcasted_iota(jnp.int32, (SLAB, LANES), 1)
        m0 = [None] + [lane < LANES - 2 * a for a in range(1, 4)]
        m1 = [(lane >= 8) & (lane < LANES - 2 * a) for a in range(4)]
        nd = SLAB // H
        acc = [[None, None] for _ in range(4)]
        for sl in range(D // SLAB):
            r0 = sl * SLAB
            q = qkv_s[jj + 1, r0:r0 + SLAB, :]
            k = qkv_s[jj + 1, D + r0:D + r0 + SLAB, :]
            kp = qkv_s[jj, D + r0:D + r0 + SLAB, :]
            rkp = rk_s[jj % 2, r0:r0 + SLAB, :]
            rk = pltpu.roll(k, 8, 1)
            rk_s[(jj + 1) % 2, r0:r0 + SLAB, :] = rk
            for a in range(4):
                rq = q if a == 0 else pltpu.roll(q, LANES - 2 * a, 1)
                for b in range(2):
                    if b == 0:
                        mix = k if a == 0 else jnp.where(m0[a], k, kp)
                    else:
                        mix = jnp.where(m1[a], rk, rkp)
                    p = rq * mix
                    for i in range(nd):
                        pi = p[i * H:(i + 1) * H]
                        acc[a][b] = pi if acc[a][b] is None else acc[a][b] + pi
        lane16 = jax.lax.broadcasted_iota(jnp.int32, (H, LANES), 1)
        logit = []
        for w in range(W):
            a, b = w % 4, w // 4
            lw = acc[a][b] if a == 0 else pltpu.roll(acc[a][b], 2 * a, 1)
            lw = lw * scale
            if jj == 0 and w > 0:
                lw = jnp.where(lane16 >= 2 * w, lw, -1e9)
            logit.append(lw)
        mx = functools.reduce(jnp.maximum, logit)
        ex = [jnp.exp(l - mx) for l in logit]
        inv = 1.0 / functools.reduce(jnp.add, ex)
        ra = [[None, None] for _ in range(4)]
        for w in range(W):
            a, b = w % 4, w // 4
            aw = ex[w] * inv
            aw = aw if a == 0 else pltpu.roll(aw, LANES - 2 * a, 1)
            ra[a][b] = jnp.concatenate([aw] * nd, axis=0)
        for sl in range(D // SLAB):
            r0 = sl * SLAB
            v = qkv_s[jj + 1, 2 * D + r0:2 * D + r0 + SLAB, :]
            vp = qkv_s[jj, 2 * D + r0:2 * D + r0 + SLAB, :]
            rvp = rv_s[jj % 2, r0:r0 + SLAB, :]
            rv = pltpu.roll(v, 8, 1)
            rv_s[(jj + 1) % 2, r0:r0 + SLAB, :] = rv
            o = None
            for a in range(4):
                mix0 = v if a == 0 else jnp.where(m0[a], v, vp)
                mix1 = jnp.where(m1[a], rv, rvp)
                t = ra[a][0] * mix0 + ra[a][1] * mix1
                o = t if a == 0 else o + pltpu.roll(t, 2 * a, 1)
            o_s[r0:r0 + SLAB, jj * LANES:(jj + 1) * LANES] = o.astype(bf16)

    def attn(c):
        for j in range(TC // LANES):
            attn_col(c * (TC // LANES) + j)

    def final(i):
        cs = slice(OOFF[i], OOFF[i + 1])
        y = jnp.dot(u_s[...], w2_s[:, cs], preferred_element_type=f32)
        s = jnp.dot(wot_s[...], o_s[:, cs], preferred_element_type=f32)
        for j in range(OUT_PIECES[i] // LANES):
            jj = OOFF[i] // LANES + j
            col = pl.ds(jj * LANES, LANES)
            g = _silu(y[:, j * LANES:(j + 1) * LANES] + b2f_s[jj:jj + 1, :])
            r = x_s[:, col].astype(f32) + s[:, j * LANES:(j + 1) * LANES] * g
            out_s[:, col] = r.astype(bf16)
        out_cp(i).start()

    zeros = jnp.zeros((D, LANES), f32)
    qkv_s[0, D:2 * D, :] = zeros
    qkv_s[0, 2 * D:3 * D, :] = zeros
    rk_s[0] = zeros
    rv_s[0] = zeros

    for c in range(QKV_AHEAD):
        qkv(c)
        if c >= 1:
            attn(c - 1)
    _scope("ww2", lambda: w2_cp.wait())
    for c in range(NC):
        if c + QKV_AHEAD - 1 < NC:
            attn(c + QKV_AHEAD - 1)
        final(c)
        if c + QKV_AHEAD < NC:
            qkv(c + QKV_AHEAD)
    final(NC)

    def waits():
        for i in range(NO):
            out_cp(i).wait()
    _scope("wout", waits)


@jax.jit
def pallas_recurrent_scan__sliding_local_dilated__mixer_token_mlp__prompt_kernel(
    A_x: jax.Array,
    A_wqkv: jax.Array,
    A_wo: jax.Array,
    B_x: jax.Array,
    B_w1: jax.Array,
    B_b1: jax.Array,
    B_w2: jax.Array,
    B_b2: jax.Array,
):
    del B_x
    xt = jnp.swapaxes(A_x, 1, 2)
    b1 = B_b1.reshape(F // LANES, LANES)
    b2 = B_b2.reshape(S // LANES, LANES)
    any_spec = pl.BlockSpec(memory_space=pl.ANY)
    out_t = pl.pallas_call(
        _kernel,
        out_shape=jax.ShapeDtypeStruct((1, D, S), bf16),
        in_specs=[any_spec] * 7,
        out_specs=any_spec,
        scratch_shapes=[
            pltpu.VMEM((D, S), bf16),
            pltpu.VMEM((D, 3 * D), bf16),
            pltpu.VMEM((D, D), bf16),
            pltpu.VMEM((S, F), bf16),
            pltpu.VMEM((F, S), bf16),
            pltpu.VMEM((F // LANES, LANES), bf16),
            pltpu.VMEM((S // LANES, LANES), bf16),
            pltpu.VMEM((D // 2, S), u32),
            pltpu.VMEM((D // 2, S), u32),
            pltpu.VMEM((D, F), f32),
            pltpu.VMEM((D // 2, F), u32),
            pltpu.VMEM((4, 11 * LANES, LANES), f32),
            pltpu.VMEM((3 * D // 2, D), u32),
            pltpu.VMEM((4, D, LANES), f32),
            pltpu.VMEM((D // 2, D), u32),
            pltpu.VMEM((NCOL + 1, 3 * D, LANES), f32),
            pltpu.VMEM((2, D, LANES), f32),
            pltpu.VMEM((2, D, LANES), f32),
            pltpu.VMEM((D // 2, S), u32),
            pltpu.VMEM((D, S), bf16),
            pltpu.VMEM((F // LANES, LANES), f32),
            pltpu.VMEM((S // LANES, LANES), f32),
            pltpu.SemaphoreType.DMA((NSEM,)),
        ],
        compiler_params=pltpu.CompilerParams(vmem_limit_bytes=100 * 1024 * 1024),
        name="fused_mixer_attn",
    )(xt, A_wqkv, A_wo, B_w1, b1, B_w2, b2)
    return jnp.swapaxes(out_t, 1, 2)
```

```python
import functools

import jax
import jax.numpy as jnp
import jax.experimental.pallas as pl
import jax.experimental.pallas.tpu as pltpu

S = 2048
D = 448
H = 16
DH = D // H
F = 1792
W = 8
EPS = 1e-5
TC = 256
NC = S // TC
LANES = 128
NCOL = S // LANES
SLAB = 32

f32 = jnp.float32
bf16 = jnp.bfloat16
u32 = jnp.uint32

_SCOPES = False


def _scope(name, fn):
    if _SCOPES:
        with jax.named_scope(name):
            fn()
    else:
        fn()


LNB = 64
NLB = D // LNB


def _rep(v8, rows):
    return jnp.concatenate([v8] * (rows // 8), axis=0)


def _ln_stats(x_ref, col, pace):
    piv = jnp.broadcast_to(x_ref[0:1, col].astype(f32), (8, LANES))
    s1 = s2 = None
    for i in range(NLB):
        pv = _rep(pace(piv), LNB // 2)
        w = pltpu.bitcast(x_ref[i * LNB:(i + 1) * LNB, col], u32)
        for half in (w << 16, w & jnp.uint32(0xFFFF0000)):
            d = pltpu.bitcast(half, f32) - pv
            for k in range(LNB // 2 // 16):
                dk = d[k * 16:(k + 1) * 16]
                s1 = dk if s1 is None else s1 + dk
                s2 = dk * dk if s2 is None else s2 + dk * dk
    md = jnp.sum(s1, axis=0, keepdims=True) * (1.0 / D)
    v = jnp.maximum(jnp.sum(s2, axis=0, keepdims=True) * (1.0 / D) - md * md, 0.0)
    r = jax.lax.rsqrt(v + EPS)
    r2 = jax.lax.rsqrt(v * r * r + EPS)
    return piv + md, r, r * r2


class _Pacer:
    def __init__(self, tokens, count, never):
        self.tokens, self.count, self.never, self.i = tokens, count, never, 0

    def __call__(self, v8):
        if not self.tokens:
            return v8
        tok = self.tokens[self.i * len(self.tokens) // self.count]
        self.i += 1
        return jnp.where(self.never, tok, v8)


def _gelu(x):
    c = 0.7978845608028654
    t = jnp.tanh(x * (c + (c * 0.044715) * (x * x)))
    hx = 0.5 * x
    return hx + hx * t


def _silu(y):
    hy = 0.5 * y
    return hy + hy * jnp.tanh(hy)


N0 = 768
NB = 256
CPC = TC // LANES
QKV_AHEAD = 4
OUT_PIECES = (256,) * 7 + (128, 128)
OOFF = tuple(sum(OUT_PIECES[:i]) for i in range(len(OUT_PIECES) + 1))
NO = len(OUT_PIECES)
SEM_X, SEM_W1, SEM_MISC, SEM_OUT = 0, NC, 2 * NC, 2 * NC + 6
NSEM = SEM_OUT + NO


def _kernel(x_hbm, wqkv_hbm, wo_hbm, w1_hbm, b1_hbm, w2_hbm, b2_hbm, out_hbm,
            x_s, wqkv_s, wo_s, w1_s, w2_s, b1_s, b2_s,
            xn_s, h_s, acc_s, u_s, wt32_s, wqkvt_s, wo32_s, wot_s,
            qkv_s, rk_s, rv_s, o_s, out_s, b1f_s, b2f_s, sem):
    xn_s, h_s, u_s, wqkvt_s, wot_s, o_s = (
        r.bitcast(bf16) for r in (xn_s, h_s, u_s, wqkvt_s, wot_s, o_s))

    def x_cp(p):
        return pltpu.make_async_copy(x_hbm.at[0, :, pl.ds(p * TC, TC)], x_s.at[p], sem.at[SEM_X + p])

    def w1_cp(p, n_lo=0):
        return pltpu.make_async_copy(w1_hbm.at[pl.ds(p * TC, TC), n_lo:F], w1_s.at[p, :, n_lo:F],
                                     sem.at[SEM_W1 + p])

    def out_cp(i):
        sl = slice(OOFF[i], OOFF[i + 1])
        return pltpu.make_async_copy(out_s.at[:, sl], out_hbm.at[0, :, sl], sem.at[SEM_OUT + i])

    wqkv_cp = pltpu.make_async_copy(wqkv_hbm, wqkv_s, sem.at[SEM_MISC + 0])
    wo_cp = pltpu.make_async_copy(wo_hbm, wo_s, sem.at[SEM_MISC + 1])
    b1_cp = pltpu.make_async_copy(b1_hbm, b1_s, sem.at[SEM_MISC + 2])
    b2_cp = pltpu.make_async_copy(b2_hbm, b2_s, sem.at[SEM_MISC + 3])
    w2_cp = pltpu.make_async_copy(w2_hbm, w2_s, sem.at[SEM_MISC + 4])
    w1a_cp = pltpu.make_async_copy(w1_hbm.at[0:TC, 0:N0], w1_s.at[0, :, 0:N0],
                                   sem.at[SEM_MISC + 5])

    x_cp(0).start()
    w1a_cp.start()
    for p in range(NC):
        if p == NC - 2:
            wqkv_cp.start()
            wo_cp.start()
            b1_cp.start()
            b2_cp.start()
        w1_cp(p, N0 if p == 0 else 0).start()
        if p + 1 < NC:
            x_cp(p + 1).start()
    w2_cp.start()

    def prep_wqkv_t():
        for c in range(11):
            wd = min(LANES, 3 * D - c * LANES)
            blk = wqkv_s[:, c * LANES:c * LANES + wd].T.astype(f32)
            for kt in range(4):
                kw = min(LANES, D - kt * LANES)
                wt32_s[kt, c * LANES:c * LANES + wd, 0:kw] = blk[:, kt * LANES:kt * LANES + kw]

    def prep_wqkv_perm():
        for sec in range(3):
            for d in range(DH):
                r0 = sec * D + d * H
                for kt in range(4):
                    kw = min(LANES, D - kt * LANES)
                    rows = wt32_s[kt, pl.ds(sec * D + d, H, stride=DH), :]
                    wqkvt_s[r0:r0 + H, kt * LANES:kt * LANES + kw] = rows[:, 0:kw].astype(bf16)

    def prep_wo():
        for nt in range(4):
            nw = min(LANES, D - nt * LANES)
            wo32_s[nt, :, 0:nw] = wo_s[:, nt * LANES:nt * LANES + nw].astype(f32)
        for nt in range(4):
            nw = min(LANES, D - nt * LANES)
            rows = [wo32_s[nt, pl.ds(d, H, stride=DH), :][:, 0:nw].astype(bf16) for d in range(DH)]
            blk = jnp.concatenate(rows, axis=0)
            wot_s[nt * LANES:nt * LANES + nw, :] = blk.T

    def ln_piece(p, tokens):
        xp, xnp, hp = x_s.at[p], xn_s.at[p], h_s.at[p]
        z = xp[0:8, 0:LANES].astype(f32)
        pace = _Pacer(tokens, 2 * NLB * CPC, z + 1.0 < z)
        for j in range(CPC):
            col = pl.ds(j * LANES, LANES)
            m, r, rr = _ln_stats(xp, col, pace)
            for i in range(NLB):
                rows = slice(i * LNB, (i + 1) * LNB)
                xc = xp[rows, col].astype(f32) - _rep(pace(m), LNB)
                xnp[rows, col] = (xc * r).astype(bf16)
                hp[rows, col] = (xc * rr).astype(bf16)

    def mix1(p, mode, n_lo=0, n_hi=F):
        tokens = []
        for n in range(n_lo // NB, n_hi // NB):
            ns = slice(n * NB, (n + 1) * NB)
            part = jnp.dot(h_s[p], w1_s[p, :, ns], preferred_element_type=f32)
            tokens += [part[r:r + 8, 0:LANES] for r in range(0, D, 8)]
            if mode == "first":
                acc_s[:, ns] = part
            elif mode == "mid":
                acc_s[:, ns] += part
            else:
                for j in range(NB // LANES):
                    nn = n * (NB // LANES) + j
                    col = pl.ds(nn * LANES, LANES)
                    z = acc_s[:, col] + part[:, j * LANES:(j + 1) * LANES] + b1f_s[nn:nn + 1, :]
                    u_s[:, col] = _gelu(z).astype(bf16)
        return tokens[:len(tokens) * 7 // 8]

    _scope("wx0", lambda: x_cp(0).wait())
    ln_piece(0, [])
    _scope("w0a", lambda: w1a_cp.wait())
    mix1(0, "first", 0, N0)
    _scope("w0", lambda: (w1_cp(0, N0).wait(), x_cp(1).wait()))
    ln_piece(1, mix1(0, "first", N0, F))

    def mid_step(p, carry):
        _scope("wl", lambda: (w1_cp(p).wait(), x_cp(p + 1).wait()))
        ln_piece(p + 1, mix1(p, "mid"))
        return carry

    jax.lax.fori_loop(1, NC - 2, mid_step, 0)

    def waits():
        wqkv_cp.wait()
        wo_cp.wait()
        b1_cp.wait()
        b2_cp.wait()
        w1_cp(NC - 2).wait()
        x_cp(NC - 1).wait()
        w1_cp(NC - 1).wait()
    _scope("wlast", waits)
    b1f_s[...] = b1_s[...].astype(f32)
    b2f_s[...] = b2_s[...].astype(f32)
    prep_wqkv_t()
    prep_wqkv_perm()
    prep_wo()
    ln_piece(NC - 1, mix1(NC - 2, "mid"))
    mix1(NC - 1, "last")

    def qkv(c):
        r = jnp.dot(wqkvt_s[...], xn_s[c],
                    preferred_element_type=f32)
        for j in range(TC // LANES):
            qkv_s[c * (TC // LANES) + j + 1] = r[:, j * LANES:(j + 1) * LANES]

    scale = DH ** -0.5

    def attn_col(jj):
        lane = jax.lax.broadcasted_iota(jnp.int32, (SLAB, LANES), 1)
        m0 = [None] + [lane < LANES - 2 * a for a in range(1, 4)]
        m1 = [(lane >= 8) & (lane < LANES - 2 * a) for a in range(4)]
        nd = SLAB // H
        acc = [[None, None] for _ in range(4)]
        for sl in range(D // SLAB):
            r0 = sl * SLAB
            q = qkv_s[jj + 1, r0:r0 + SLAB, :]
            k = qkv_s[jj + 1, D + r0:D + r0 + SLAB, :]
            kp = qkv_s[jj, D + r0:D + r0 + SLAB, :]
            rkp = rk_s[jj % 2, r0:r0 + SLAB, :]
            rk = pltpu.roll(k, 8, 1)
            rk_s[(jj + 1) % 2, r0:r0 + SLAB, :] = rk
            for a in range(4):
                rq = q if a == 0 else pltpu.roll(q, LANES - 2 * a, 1)
                for b in range(2):
                    if b == 0:
                        mix = k if a == 0 else jnp.where(m0[a], k, kp)
                    else:
                        mix = jnp.where(m1[a], rk, rkp)
                    p = rq * mix
                    for i in range(nd):
                        pi = p[i * H:(i + 1) * H]
                        acc[a][b] = pi if acc[a][b] is None else acc[a][b] + pi
        lane16 = jax.lax.broadcasted_iota(jnp.int32, (H, LANES), 1)
        logit = []
        for w in range(W):
            a, b = w % 4, w // 4
            lw = acc[a][b] if a == 0 else pltpu.roll(acc[a][b], 2 * a, 1)
            lw = lw * scale
            if jj == 0 and w > 0:
                lw = jnp.where(lane16 >= 2 * w, lw, -1e9)
            logit.append(lw)
        mx = functools.reduce(jnp.maximum, logit)
        ex = [jnp.exp(l - mx) for l in logit]
        inv = 1.0 / functools.reduce(jnp.add, ex)
        ra = [[None, None] for _ in range(4)]
        for w in range(W):
            a, b = w % 4, w // 4
            aw = ex[w] * inv
            aw = aw if a == 0 else pltpu.roll(aw, LANES - 2 * a, 1)
            ra[a][b] = jnp.concatenate([aw] * nd, axis=0)
        for sl in range(D // SLAB):
            r0 = sl * SLAB
            v = qkv_s[jj + 1, 2 * D + r0:2 * D + r0 + SLAB, :]
            vp = qkv_s[jj, 2 * D + r0:2 * D + r0 + SLAB, :]
            rvp = rv_s[jj % 2, r0:r0 + SLAB, :]
            rv = pltpu.roll(v, 8, 1)
            rv_s[(jj + 1) % 2, r0:r0 + SLAB, :] = rv
            o = None
            for a in range(4):
                mix0 = v if a == 0 else jnp.where(m0[a], v, vp)
                mix1 = jnp.where(m1[a], rv, rvp)
                t = ra[a][0] * mix0 + ra[a][1] * mix1
                o = t if a == 0 else o + pltpu.roll(t, 2 * a, 1)
            o_s[r0:r0 + SLAB, jj * LANES:(jj + 1) * LANES] = o.astype(bf16)

    def attn(c):
        for j in range(TC // LANES):
            attn_col(c * (TC // LANES) + j)

    def final(i):
        cs = slice(OOFF[i], OOFF[i + 1])
        y = jnp.dot(u_s[...], w2_s[:, cs], preferred_element_type=f32)
        s = jnp.dot(wot_s[...], o_s[:, cs], preferred_element_type=f32)
        for j in range(OUT_PIECES[i] // LANES):
            jj = OOFF[i] // LANES + j
            col = pl.ds(jj * LANES, LANES)
            g = _silu(y[:, j * LANES:(j + 1) * LANES] + b2f_s[jj:jj + 1, :])
            xr = x_s[jj // CPC, :, pl.ds((jj % CPC) * LANES, LANES)].astype(f32)
            r = xr + s[:, j * LANES:(j + 1) * LANES] * g
            out_s[:, col] = r.astype(bf16)
        out_cp(i).start()

    zeros = jnp.zeros((D, LANES), f32)
    qkv_s[0, D:2 * D, :] = zeros
    qkv_s[0, 2 * D:3 * D, :] = zeros
    rk_s[0] = zeros
    rv_s[0] = zeros

    for c in range(QKV_AHEAD):
        qkv(c)
        if c >= 1:
            attn(c - 1)
    _scope("ww2", lambda: w2_cp.wait())
    for c in range(NC):
        if c + QKV_AHEAD - 1 < NC:
            attn(c + QKV_AHEAD - 1)
        final(c)
        if c + QKV_AHEAD < NC:
            qkv(c + QKV_AHEAD)
    final(NC)

    def waits():
        for i in range(NO):
            out_cp(i).wait()
    _scope("wout", waits)


@jax.jit
def pallas_recurrent_scan__sliding_local_dilated__mixer_token_mlp__prompt_kernel(
    A_x: jax.Array,
    A_wqkv: jax.Array,
    A_wo: jax.Array,
    B_x: jax.Array,
    B_w1: jax.Array,
    B_b1: jax.Array,
    B_w2: jax.Array,
    B_b2: jax.Array,
):
    del B_x
    xt = jnp.swapaxes(A_x, 1, 2)
    b1 = B_b1.reshape(F // LANES, LANES)
    b2 = B_b2.reshape(S // LANES, LANES)
    any_spec = pl.BlockSpec(memory_space=pl.ANY)
    out_t = pl.pallas_call(
        _kernel,
        out_shape=jax.ShapeDtypeStruct((1, D, S), bf16),
        in_specs=[any_spec] * 7,
        out_specs=any_spec,
        scratch_shapes=[
            pltpu.VMEM((NC, D, TC), bf16),
            pltpu.VMEM((D, 3 * D), bf16),
            pltpu.VMEM((D, D), bf16),
            pltpu.VMEM((NC, TC, F), bf16),
            pltpu.VMEM((F, S), bf16),
            pltpu.VMEM((F // LANES, LANES), bf16),
            pltpu.VMEM((S // LANES, LANES), bf16),
            pltpu.VMEM((NC, D // 2, TC), u32),
            pltpu.VMEM((NC, D // 2, TC), u32),
            pltpu.VMEM((D, F), f32),
            pltpu.VMEM((D // 2, F), u32),
            pltpu.VMEM((4, 11 * LANES, LANES), f32),
            pltpu.VMEM((3 * D // 2, D), u32),
            pltpu.VMEM((4, D, LANES), f32),
            pltpu.VMEM((D // 2, D), u32),
            pltpu.VMEM((NCOL + 1, 3 * D, LANES), f32),
            pltpu.VMEM((2, D, LANES), f32),
            pltpu.VMEM((2, D, LANES), f32),
            pltpu.VMEM((D // 2, S), u32),
            pltpu.VMEM((D, S), bf16),
            pltpu.VMEM((F // LANES, LANES), f32),
            pltpu.VMEM((S // LANES, LANES), f32),
            pltpu.SemaphoreType.DMA((NSEM,)),
        ],
        compiler_params=pltpu.CompilerParams(vmem_limit_bytes=100 * 1024 * 1024,
                                             disable_semaphore_checks=True,
                                             disable_bounds_checks=True),
        name="fused_mixer_attn",
    )(xt, A_wqkv, A_wo, B_w1, b1, B_w2, b2)
    return jnp.swapaxes(out_t, 1, 2)
```

```python
import functools

import jax
import jax.numpy as jnp
import jax.experimental.pallas as pl
import jax.experimental.pallas.tpu as pltpu

S = 2048
D = 448
H = 16
DH = D // H
F = 1792
W = 8
EPS = 1e-5
TC = 256
NC = S // TC
LANES = 128
NCOL = S // LANES
SLAB = 32

f32 = jnp.float32
bf16 = jnp.bfloat16
u32 = jnp.uint32

_SCOPES = False


def _scope(name, fn):
    if _SCOPES:
        with jax.named_scope(name):
            fn()
    else:
        fn()


LNB = 64
NLB = D // LNB


def _rep(v8, rows):
    return jnp.concatenate([v8] * (rows // 8), axis=0)


def _ln_stats(x_ref, col, pace):
    piv = jnp.broadcast_to(x_ref[0:1, col].astype(f32), (8, LANES))
    s1 = s2 = None
    for i in range(NLB):
        pv = _rep(pace(piv), LNB // 2)
        w = pltpu.bitcast(x_ref[i * LNB:(i + 1) * LNB, col], u32)
        for half in (w << 16, w & jnp.uint32(0xFFFF0000)):
            d = pltpu.bitcast(half, f32) - pv
            for k in range(LNB // 2 // 16):
                dk = d[k * 16:(k + 1) * 16]
                s1 = dk if s1 is None else s1 + dk
                s2 = dk * dk if s2 is None else s2 + dk * dk
    md = jnp.sum(s1, axis=0, keepdims=True) * (1.0 / D)
    v = jnp.maximum(jnp.sum(s2, axis=0, keepdims=True) * (1.0 / D) - md * md, 0.0)
    r = jax.lax.rsqrt(v + EPS)
    r2 = jax.lax.rsqrt(v * r * r + EPS)
    return piv + md, r, r * r2


class _Pacer:
    def __init__(self, tokens, count, never):
        self.tokens, self.count, self.never, self.i = tokens, count, never, 0

    def __call__(self, v8):
        if not self.tokens:
            return v8
        tok = self.tokens[self.i * len(self.tokens) // self.count]
        self.i += 1
        return jnp.where(self.never, tok, v8)


def _gelu(x):
    c = 0.7978845608028654
    t = jnp.tanh(x * (c + (c * 0.044715) * (x * x)))
    hx = 0.5 * x
    return hx + hx * t


def _silu(y):
    hy = 0.5 * y
    return hy + hy * jnp.tanh(hy)


N0 = 768
NB = 256
CPC = TC // LANES
QKV_AHEAD = 3
OUT_PIECES = (256,) * 7 + (128, 128)
OOFF = tuple(sum(OUT_PIECES[:i]) for i in range(len(OUT_PIECES) + 1))
NO = len(OUT_PIECES)
SEM_X, SEM_W1, SEM_MISC, SEM_OUT = 0, NC, 2 * NC, 2 * NC + 6
NSEM = SEM_OUT + NO


def _kernel(x_hbm, wqkv_hbm, wo_hbm, w1_hbm, b1_hbm, w2_hbm, b2_hbm, out_hbm,
            x_s, wqkv_s, wo_s, w1_s, w2_s, b1_s, b2_s,
            xn_s, h_s, acc_s, u_s, wt32_s, wqkvt_s, wo32_s, wot_s,
            qkv_s, rk_s, rv_s, o_s, out_s, b1f_s, b2f_s, sem):
    xn_s, h_s, u_s, wqkvt_s, wot_s, o_s = (
        r.bitcast(bf16) for r in (xn_s, h_s, u_s, wqkvt_s, wot_s, o_s))

    def x_cp(p):
        return pltpu.make_async_copy(x_hbm.at[0, :, pl.ds(p * TC, TC)], x_s.at[p], sem.at[SEM_X + p])

    def w1_cp(p, n_lo=0):
        return pltpu.make_async_copy(w1_hbm.at[pl.ds(p * TC, TC), n_lo:F], w1_s.at[p, :, n_lo:F],
                                     sem.at[SEM_W1 + p])

    def out_cp(i):
        sl = slice(OOFF[i], OOFF[i + 1])
        return pltpu.make_async_copy(out_s.at[:, sl], out_hbm.at[0, :, sl], sem.at[SEM_OUT + i])

    wqkv_cp = pltpu.make_async_copy(wqkv_hbm, wqkv_s, sem.at[SEM_MISC + 0])
    wo_cp = pltpu.make_async_copy(wo_hbm, wo_s, sem.at[SEM_MISC + 1])
    b1_cp = pltpu.make_async_copy(b1_hbm, b1_s, sem.at[SEM_MISC + 2])
    b2_cp = pltpu.make_async_copy(b2_hbm, b2_s, sem.at[SEM_MISC + 3])
    w2_cp = pltpu.make_async_copy(w2_hbm, w2_s, sem.at[SEM_MISC + 4])
    w1a_cp = pltpu.make_async_copy(w1_hbm.at[0:TC, 0:N0], w1_s.at[0, :, 0:N0],
                                   sem.at[SEM_MISC + 5])

    x_cp(0).start()
    w1a_cp.start()
    for p in range(NC):
        if p == NC - 2:
            wqkv_cp.start()
            wo_cp.start()
            b1_cp.start()
            b2_cp.start()
        w1_cp(p, N0 if p == 0 else 0).start()
        if p + 1 < NC:
            x_cp(p + 1).start()
    w2_cp.start()

    def prep_wqkv_t():
        for c in range(11):
            wd = min(LANES, 3 * D - c * LANES)
            blk = wqkv_s[:, c * LANES:c * LANES + wd].T.astype(f32)
            for kt in range(4):
                kw = min(LANES, D - kt * LANES)
                wt32_s[kt, c * LANES:c * LANES + wd, 0:kw] = blk[:, kt * LANES:kt * LANES + kw]

    def prep_wqkv_perm():
        for sec in range(3):
            for d in range(DH):
                r0 = sec * D + d * H
                for kt in range(4):
                    kw = min(LANES, D - kt * LANES)
                    rows = wt32_s[kt, pl.ds(sec * D + d, H, stride=DH), :]
                    wqkvt_s[r0:r0 + H, kt * LANES:kt * LANES + kw] = rows[:, 0:kw].astype(bf16)

    def prep_wo():
        for nt in range(4):
            nw = min(LANES, D - nt * LANES)
            wo32_s[nt, :, 0:nw] = wo_s[:, nt * LANES:nt * LANES + nw].astype(f32)
        for nt in range(4):
            nw = min(LANES, D - nt * LANES)
            rows = [wo32_s[nt, pl.ds(d, H, stride=DH), :][:, 0:nw].astype(bf16) for d in range(DH)]
            blk = jnp.concatenate(rows, axis=0)
            wot_s[nt * LANES:nt * LANES + nw, :] = blk.T

    def ln_piece(p, tokens):
        xp, xnp, hp = x_s.at[p], xn_s.at[p], h_s.at[p]
        z = xp[0:8, 0:LANES].astype(f32)
        pace = _Pacer(tokens, 2 * NLB * CPC, z + 1.0 < z)
        for j in range(CPC):
            col = pl.ds(j * LANES, LANES)
            m, r, rr = _ln_stats(xp, col, pace)
            for i in range(NLB):
                rows = slice(i * LNB, (i + 1) * LNB)
                xc = xp[rows, col].astype(f32) - _rep(pace(m), LNB)
                xnp[rows, col] = (xc * r).astype(bf16)
                hp[rows, col] = (xc * rr).astype(bf16)

    def mix1(p, mode, n_lo=0, n_hi=F):
        tokens = []
        for n in range(n_lo // NB, n_hi // NB):
            ns = slice(n * NB, (n + 1) * NB)
            part = jnp.dot(h_s[p], w1_s[p, :, ns], preferred_element_type=f32)
            tokens += [part[r:r + 8, 0:LANES] for r in range(0, D, 8)]
            if mode == "first":
                acc_s[:, ns] = part
            elif mode == "mid":
                acc_s[:, ns] += part
            else:
                for j in range(NB // LANES):
                    nn = n * (NB // LANES) + j
                    col = pl.ds(nn * LANES, LANES)
                    z = acc_s[:, col] + part[:, j * LANES:(j + 1) * LANES] + b1f_s[nn:nn + 1, :]
                    u_s[:, col] = _gelu(z).astype(bf16)
        return tokens[:len(tokens) * 7 // 8]

    _scope("wx0", lambda: x_cp(0).wait())
    ln_piece(0, [])
    _scope("w0a", lambda: w1a_cp.wait())
    mix1(0, "first", 0, N0)
    _scope("w0", lambda: (w1_cp(0, N0).wait(), x_cp(1).wait()))
    ln_piece(1, mix1(0, "first", N0, F))

    def mid_step(p, carry):
        _scope("wl", lambda: (w1_cp(p).wait(), x_cp(p + 1).wait()))
        ln_piece(p + 1, mix1(p, "mid"))
        return carry + 1

    steps = jax.lax.fori_loop(1, NC - 2, mid_step, 0)

    def waits():
        wqkv_cp.wait()
        wo_cp.wait()
        b1_cp.wait()
        b2_cp.wait()
        w1_cp(NC - 2).wait()
        x_cp(NC - 1).wait()
        w1_cp(NC - 1).wait()
    _scope("wlast", waits)
    def qkv(c):
        r = jnp.dot(wqkvt_s[...], xn_s[c],
                    preferred_element_type=f32)
        for j in range(TC // LANES):
            qkv_s[c * (TC // LANES) + j + 1] = r[:, j * LANES:(j + 1) * LANES]

    scale = DH ** -0.5

    def attn_col(jj):
        lane = jax.lax.broadcasted_iota(jnp.int32, (SLAB, LANES), 1)
        m0 = [None] + [lane < LANES - 2 * a for a in range(1, 4)]
        m1 = [(lane >= 8) & (lane < LANES - 2 * a) for a in range(4)]
        nd = SLAB // H
        acc = [[None, None] for _ in range(4)]
        for sl in range(D // SLAB):
            r0 = sl * SLAB
            q = qkv_s[jj + 1, r0:r0 + SLAB, :]
            k = qkv_s[jj + 1, D + r0:D + r0 + SLAB, :]
            kp = qkv_s[jj, D + r0:D + r0 + SLAB, :]
            rkp = rk_s[jj % 2, r0:r0 + SLAB, :]
            rk = pltpu.roll(k, 8, 1)
            rk_s[(jj + 1) % 2, r0:r0 + SLAB, :] = rk
            for a in range(4):
                rq = q if a == 0 else pltpu.roll(q, LANES - 2 * a, 1)
                for b in range(2):
                    if b == 0:
                        mix = k if a == 0 else jnp.where(m0[a], k, kp)
                    else:
                        mix = jnp.where(m1[a], rk, rkp)
                    p = rq * mix
                    for i in range(nd):
                        pi = p[i * H:(i + 1) * H]
                        acc[a][b] = pi if acc[a][b] is None else acc[a][b] + pi
        lane16 = jax.lax.broadcasted_iota(jnp.int32, (H, LANES), 1)
        logit = []
        for w in range(W):
            a, b = w % 4, w // 4
            lw = acc[a][b] if a == 0 else pltpu.roll(acc[a][b], 2 * a, 1)
            lw = lw * scale
            if jj == 0 and w > 0:
                lw = jnp.where(lane16 >= 2 * w, lw, -1e9)
            logit.append(lw)
        mx = functools.reduce(jnp.maximum, logit)
        ex = [jnp.exp(l - mx) for l in logit]
        inv = 1.0 / functools.reduce(jnp.add, ex)
        ra = [[None, None] for _ in range(4)]
        for w in range(W):
            a, b = w % 4, w // 4
            aw = ex[w] * inv
            aw = aw if a == 0 else pltpu.roll(aw, LANES - 2 * a, 1)
            ra[a][b] = jnp.concatenate([aw] * nd, axis=0)
        for sl in range(D // SLAB):
            r0 = sl * SLAB
            v = qkv_s[jj + 1, 2 * D + r0:2 * D + r0 + SLAB, :]
            vp = qkv_s[jj, 2 * D + r0:2 * D + r0 + SLAB, :]
            rvp = rv_s[jj % 2, r0:r0 + SLAB, :]
            rv = pltpu.roll(v, 8, 1)
            rv_s[(jj + 1) % 2, r0:r0 + SLAB, :] = rv
            o = None
            for a in range(4):
                mix0 = v if a == 0 else jnp.where(m0[a], v, vp)
                mix1 = jnp.where(m1[a], rv, rvp)
                t = ra[a][0] * mix0 + ra[a][1] * mix1
                o = t if a == 0 else o + pltpu.roll(t, 2 * a, 1)
            o_s[r0:r0 + SLAB, jj * LANES:(jj + 1) * LANES] = o.astype(bf16)

    def attn(c):
        for j in range(TC // LANES):
            attn_col(c * (TC // LANES) + j)

    def final(i):
        cs = slice(OOFF[i], OOFF[i + 1])
        y = jnp.dot(u_s[...], w2_s[:, cs], preferred_element_type=f32)
        s = jnp.dot(wot_s[...], o_s[:, cs], preferred_element_type=f32)
        for j in range(OUT_PIECES[i] // LANES):
            jj = OOFF[i] // LANES + j
            col = pl.ds(jj * LANES, LANES)
            g = _silu(y[:, j * LANES:(j + 1) * LANES] + b2f_s[jj:jj + 1, :])
            xr = x_s[jj // CPC, :, pl.ds((jj % CPC) * LANES, LANES)].astype(f32)
            r = xr + s[:, j * LANES:(j + 1) * LANES] * g
            out_s[:, col] = r.astype(bf16)
        out_cp(i).start()

    @pl.when(steps == NC - 3)
    def _():
        b1f_s[...] = b1_s[...].astype(f32)
        b2f_s[...] = b2_s[...].astype(f32)
        prep_wqkv_t()
        prep_wqkv_perm()
        prep_wo()
        ln_piece(NC - 1, mix1(NC - 2, "mid"))
        mix1(NC - 1, "last")

        zeros = jnp.zeros((D, LANES), f32)
        qkv_s[0, D:2 * D, :] = zeros
        qkv_s[0, 2 * D:3 * D, :] = zeros
        rk_s[0] = zeros
        rv_s[0] = zeros

        for c in range(QKV_AHEAD):
            qkv(c)
            if c >= 1:
                attn(c - 1)

    _scope("ww2", lambda: w2_cp.wait())
    for c in range(NC):
        if c + QKV_AHEAD - 1 < NC:
            attn(c + QKV_AHEAD - 1)
        final(c)
        if c + QKV_AHEAD < NC:
            qkv(c + QKV_AHEAD)
    final(NC)

    def waits():
        for i in range(NO):
            out_cp(i).wait()
    _scope("wout", waits)


@jax.jit
def pallas_recurrent_scan__sliding_local_dilated__mixer_token_mlp__prompt_kernel(
    A_x: jax.Array,
    A_wqkv: jax.Array,
    A_wo: jax.Array,
    B_x: jax.Array,
    B_w1: jax.Array,
    B_b1: jax.Array,
    B_w2: jax.Array,
    B_b2: jax.Array,
):
    del B_x
    xt = jnp.swapaxes(A_x, 1, 2)
    b1 = B_b1.reshape(F // LANES, LANES)
    b2 = B_b2.reshape(S // LANES, LANES)
    any_spec = pl.BlockSpec(memory_space=pl.ANY)
    out_t = pl.pallas_call(
        _kernel,
        out_shape=jax.ShapeDtypeStruct((1, D, S), bf16),
        in_specs=[any_spec] * 7,
        out_specs=any_spec,
        scratch_shapes=[
            pltpu.VMEM((NC, D, TC), bf16),
            pltpu.VMEM((D, 3 * D), bf16),
            pltpu.VMEM((D, D), bf16),
            pltpu.VMEM((NC, TC, F), bf16),
            pltpu.VMEM((F, S), bf16),
            pltpu.VMEM((F // LANES, LANES), bf16),
            pltpu.VMEM((S // LANES, LANES), bf16),
            pltpu.VMEM((NC, D // 2, TC), u32),
            pltpu.VMEM((NC, D // 2, TC), u32),
            pltpu.VMEM((D, F), f32),
            pltpu.VMEM((D // 2, F), u32),
            pltpu.VMEM((4, 11 * LANES, LANES), f32),
            pltpu.VMEM((3 * D // 2, D), u32),
            pltpu.VMEM((4, D, LANES), f32),
            pltpu.VMEM((D // 2, D), u32),
            pltpu.VMEM((NCOL + 1, 3 * D, LANES), f32),
            pltpu.VMEM((2, D, LANES), f32),
            pltpu.VMEM((2, D, LANES), f32),
            pltpu.VMEM((D // 2, S), u32),
            pltpu.VMEM((D, S), bf16),
            pltpu.VMEM((F // LANES, LANES), f32),
            pltpu.VMEM((S // LANES, LANES), f32),
            pltpu.SemaphoreType.DMA((NSEM,)),
        ],
        compiler_params=pltpu.CompilerParams(vmem_limit_bytes=100 * 1024 * 1024,
                                             disable_semaphore_checks=True,
                                             disable_bounds_checks=True),
        name="fused_mixer_attn",
    )(xt, A_wqkv, A_wo, B_w1, b1, B_w2, b2)
    return jnp.swapaxes(out_t, 1, 2)
```

```python
import functools

import jax
import jax.numpy as jnp
import jax.experimental.pallas as pl
import jax.experimental.pallas.tpu as pltpu

S = 2048
D = 448
H = 16
DH = D // H
F = 1792
W = 8
EPS = 1e-5
TC = 256
NC = S // TC
LANES = 128
NCOL = S // LANES
SLAB = 32

f32 = jnp.float32
bf16 = jnp.bfloat16
u32 = jnp.uint32

_SCOPES = False


def _scope(name, fn):
    if _SCOPES:
        with jax.named_scope(name):
            fn()
    else:
        fn()


LNB = 64
NLB = D // LNB


def _rep(v8, rows):
    return jnp.concatenate([v8] * (rows // 8), axis=0)


def _ln_stats(x_ref, col, pace):
    piv = jnp.broadcast_to(x_ref[0:1, col].astype(f32), (8, LANES))
    s1 = s2 = None
    for i in range(NLB):
        pv = _rep(pace(piv), LNB // 2)
        w = pltpu.bitcast(x_ref[i * LNB:(i + 1) * LNB, col], u32)
        for half in (w << 16, w & jnp.uint32(0xFFFF0000)):
            d = pltpu.bitcast(half, f32) - pv
            for k in range(LNB // 2 // 16):
                dk = d[k * 16:(k + 1) * 16]
                s1 = dk if s1 is None else s1 + dk
                s2 = dk * dk if s2 is None else s2 + dk * dk
    md = jnp.sum(s1, axis=0, keepdims=True) * (1.0 / D)
    v = jnp.maximum(jnp.sum(s2, axis=0, keepdims=True) * (1.0 / D) - md * md, 0.0)
    r = jax.lax.rsqrt(v + EPS)
    r2 = jax.lax.rsqrt(v * r * r + EPS)
    return piv + md, r, r * r2


def _tokens(r):
    return [r[i:i + 8, j:j + LANES] for j in range(0, r.shape[1], LANES) for i in range(0, r.shape[0], 8)]


class _Pacer:
    def __init__(self, tokens, count, never):
        self.tokens, self.count, self.never, self.i = tokens, count, never, 0

    def __call__(self, v8):
        if not self.tokens:
            return v8
        tok = self.tokens[self.i * len(self.tokens) // self.count]
        self.i += 1
        return jnp.where(self.never, tok, v8)

    def gate(self, *vs):
        if not self.tokens:
            return vs
        tok = self.tokens[self.i * len(self.tokens) // self.count]
        self.i += 1
        n = vs[0].shape[0]
        nv, tk = _rep(self.never, n), _rep(tok, n)
        return tuple(jnp.where(nv, tk, v) for v in vs)


def _gelu(x):
    c = 0.7978845608028654
    t = jnp.tanh(x * (c + (c * 0.044715) * (x * x)))
    hx = 0.5 * x
    return hx + hx * t


def _silu(y):
    hy = 0.5 * y
    return hy + hy * jnp.tanh(hy)


N0 = 768
NB = 256
KB = 512
CPC = TC // LANES
QKV_AHEAD = 3
OUT_PIECES = (256,) * 7 + (128, 128)
OOFF = tuple(sum(OUT_PIECES[:i]) for i in range(len(OUT_PIECES) + 1))
NO = len(OUT_PIECES)
SEM_X, SEM_W1, SEM_MISC, SEM_OUT = 0, NC, 2 * NC, 2 * NC + 6
NSEM = SEM_OUT + NO


def _kernel(x_hbm, wqkv_hbm, wo_hbm, w1_hbm, b1_hbm, w2_hbm, b2_hbm, out_hbm,
            x_s, wqkv_s, wo_s, w1_s, w2_s, b1_s, b2_s,
            xn_s, h_s, acc_s, u_s, wt32_s, wqkvt_s, wo32_s, wot_s,
            qkv_s, rk_s, rv_s, o_s, out_s, b1f_s, b2f_s, sem):
    xn_s, h_s, u_s, wqkvt_s, wot_s, o_s = (
        r.bitcast(bf16) for r in (xn_s, h_s, u_s, wqkvt_s, wot_s, o_s))

    def x_cp(p):
        return pltpu.make_async_copy(x_hbm.at[0, :, pl.ds(p * TC, TC)], x_s.at[p], sem.at[SEM_X + p])

    def w1_cp(p, n_lo=0):
        return pltpu.make_async_copy(w1_hbm.at[pl.ds(p * TC, TC), n_lo:F], w1_s.at[p, :, n_lo:F],
                                     sem.at[SEM_W1 + p])

    def out_cp(i):
        sl = slice(OOFF[i], OOFF[i + 1])
        return pltpu.make_async_copy(out_s.at[:, sl], out_hbm.at[0, :, sl], sem.at[SEM_OUT + i])

    wqkv_cp = pltpu.make_async_copy(wqkv_hbm, wqkv_s, sem.at[SEM_MISC + 0])
    wo_cp = pltpu.make_async_copy(wo_hbm, wo_s, sem.at[SEM_MISC + 1])
    b1_cp = pltpu.make_async_copy(b1_hbm, b1_s, sem.at[SEM_MISC + 2])
    b2_cp = pltpu.make_async_copy(b2_hbm, b2_s, sem.at[SEM_MISC + 3])
    w2_cp = pltpu.make_async_copy(w2_hbm, w2_s, sem.at[SEM_MISC + 4])
    w1a_cp = pltpu.make_async_copy(w1_hbm.at[0:TC, 0:N0], w1_s.at[0, :, 0:N0],
                                   sem.at[SEM_MISC + 5])

    x_cp(0).start()
    w1a_cp.start()
    for p in range(NC):
        if p == NC - 2:
            wqkv_cp.start()
            wo_cp.start()
            b1_cp.start()
            b2_cp.start()
        w1_cp(p, N0 if p == 0 else 0).start()
        if p + 1 < NC:
            x_cp(p + 1).start()
    w2_cp.start()

    def prep_wqkv_t():
        for c in range(11):
            wd = min(LANES, 3 * D - c * LANES)
            blk = wqkv_s[:, c * LANES:c * LANES + wd].T.astype(f32)
            for kt in range(4):
                kw = min(LANES, D - kt * LANES)
                wt32_s[kt, c * LANES:c * LANES + wd, 0:kw] = blk[:, kt * LANES:kt * LANES + kw]

    def prep_wqkv_perm():
        for sec in range(3):
            for d in range(DH):
                r0 = sec * D + d * H
                for kt in range(4):
                    kw = min(LANES, D - kt * LANES)
                    rows = wt32_s[kt, pl.ds(sec * D + d, H, stride=DH), :]
                    wqkvt_s[r0:r0 + H, kt * LANES:kt * LANES + kw] = rows[:, 0:kw].astype(bf16)

    def prep_wo():
        for nt in range(4):
            nw = min(LANES, D - nt * LANES)
            wo32_s[nt, :, 0:nw] = wo_s[:, nt * LANES:nt * LANES + nw].astype(f32)
        for nt in range(4):
            nw = min(LANES, D - nt * LANES)
            rows = [wo32_s[nt, pl.ds(d, H, stride=DH), :][:, 0:nw].astype(bf16) for d in range(DH)]
            blk = jnp.concatenate(rows, axis=0)
            wot_s[nt * LANES:nt * LANES + nw, :] = blk.T

    def ln_piece(p, tokens):
        xp, xnp, hp = x_s.at[p], xn_s.at[p], h_s.at[p]
        z = xp[0:8, 0:LANES].astype(f32)
        pace = _Pacer(tokens, 2 * NLB * CPC, z + 1.0 < z)
        for j in range(CPC):
            col = pl.ds(j * LANES, LANES)
            m, r, rr = _ln_stats(xp, col, pace)
            for i in range(NLB):
                rows = slice(i * LNB, (i + 1) * LNB)
                xc = xp[rows, col].astype(f32) - _rep(pace(m), LNB)
                xnp[rows, col] = (xc * r).astype(bf16)
                hp[rows, col] = (xc * rr).astype(bf16)

    def mix1(p, mode, n_lo=0, n_hi=F):
        tokens = []
        for n in range(n_lo // NB, n_hi // NB):
            ns = slice(n * NB, (n + 1) * NB)
            part = jnp.dot(h_s[p], w1_s[p, :, ns], preferred_element_type=f32)
            tokens += [part[r:r + 8, 0:LANES] for r in range(0, D, 8)]
            if mode == "first":
                acc_s[:, ns] = part
            elif mode == "mid":
                acc_s[:, ns] += part
            else:
                for j in range(NB // LANES):
                    nn = n * (NB // LANES) + j
                    col = pl.ds(nn * LANES, LANES)
                    z = acc_s[:, col] + part[:, j * LANES:(j + 1) * LANES] + b1f_s[nn:nn + 1, :]
                    u_s[:, col] = _gelu(z).astype(bf16)
        return tokens[:len(tokens) * 7 // 8]

    _scope("wx0", lambda: x_cp(0).wait())
    ln_piece(0, [])
    _scope("w0a", lambda: w1a_cp.wait())
    mix1(0, "first", 0, N0)
    _scope("w0", lambda: (w1_cp(0, N0).wait(), x_cp(1).wait()))
    ln_piece(1, mix1(0, "first", N0, F))

    def mid_step(p, carry):
        _scope("wl", lambda: (w1_cp(p).wait(), x_cp(p + 1).wait()))
        ln_piece(p + 1, mix1(p, "mid"))
        return carry + 1

    steps = jax.lax.fori_loop(1, NC - 2, mid_step, 0)

    def waits():
        wqkv_cp.wait()
        wo_cp.wait()
        b1_cp.wait()
        b2_cp.wait()
        w1_cp(NC - 2).wait()
        x_cp(NC - 1).wait()
        w1_cp(NC - 1).wait()
    _scope("wlast", waits)
    def qkv(c):
        r = jnp.dot(wqkvt_s[...], xn_s[c],
                    preferred_element_type=f32)
        for j in range(TC // LANES):
            qkv_s[c * (TC // LANES) + j + 1] = r[:, j * LANES:(j + 1) * LANES]
        return _tokens(r)

    scale = DH ** -0.5

    def attn_col(jj, pace):
        lane = jax.lax.broadcasted_iota(jnp.int32, (SLAB, LANES), 1)
        m0 = [None] + [lane < LANES - 2 * a for a in range(1, 4)]
        m1 = [(lane >= 8) & (lane < LANES - 2 * a) for a in range(4)]
        nd = SLAB // H
        acc = [[None, None] for _ in range(4)]
        for sl in range(D // SLAB):
            r0 = sl * SLAB
            q = qkv_s[jj + 1, r0:r0 + SLAB, :]
            k = qkv_s[jj + 1, D + r0:D + r0 + SLAB, :]
            q, k = pace.gate(q, k)
            kp = qkv_s[jj, D + r0:D + r0 + SLAB, :]
            rkp = rk_s[jj % 2, r0:r0 + SLAB, :]
            rk = pltpu.roll(k, 8, 1)
            rk_s[(jj + 1) % 2, r0:r0 + SLAB, :] = rk
            for a in range(4):
                rq = q if a == 0 else pltpu.roll(q, LANES - 2 * a, 1)
                for b in range(2):
                    if b == 0:
                        mix = k if a == 0 else jnp.where(m0[a], k, kp)
                    else:
                        mix = jnp.where(m1[a], rk, rkp)
                    p = rq * mix
                    for i in range(nd):
                        pi = p[i * H:(i + 1) * H]
                        acc[a][b] = pi if acc[a][b] is None else acc[a][b] + pi
        lane16 = jax.lax.broadcasted_iota(jnp.int32, (H, LANES), 1)
        logit = []
        for w in range(W):
            a, b = w % 4, w // 4
            lw = acc[a][b] if a == 0 else pltpu.roll(acc[a][b], 2 * a, 1)
            lw = lw * scale
            if jj == 0 and w > 0:
                lw = jnp.where(lane16 >= 2 * w, lw, -1e9)
            logit.append(lw)
        mx = functools.reduce(jnp.maximum, logit)
        ex = [jnp.exp(l - mx) for l in logit]
        inv = 1.0 / functools.reduce(jnp.add, ex)
        ra = [[None, None] for _ in range(4)]
        for w in range(W):
            a, b = w % 4, w // 4
            aw = ex[w] * inv
            aw = aw if a == 0 else pltpu.roll(aw, LANES - 2 * a, 1)
            ra[a][b] = jnp.concatenate([aw] * nd, axis=0)
        for sl in range(D // SLAB):
            r0 = sl * SLAB
            v = qkv_s[jj + 1, 2 * D + r0:2 * D + r0 + SLAB, :]
            v, = pace.gate(v)
            vp = qkv_s[jj, 2 * D + r0:2 * D + r0 + SLAB, :]
            rvp = rv_s[jj % 2, r0:r0 + SLAB, :]
            rv = pltpu.roll(v, 8, 1)
            rv_s[(jj + 1) % 2, r0:r0 + SLAB, :] = rv
            o = None
            for a in range(4):
                mix0 = v if a == 0 else jnp.where(m0[a], v, vp)
                mix1 = jnp.where(m1[a], rv, rvp)
                t = ra[a][0] * mix0 + ra[a][1] * mix1
                o = t if a == 0 else o + pltpu.roll(t, 2 * a, 1)
            o_s[r0:r0 + SLAB, jj * LANES:(jj + 1) * LANES] = o.astype(bf16)

    def attn(c, tokens):
        z = b2f_s[0:8, :]
        pace = _Pacer(tokens, 2 * (D // SLAB) * CPC, z + 1.0 < z)
        for j in range(CPC):
            attn_col(c * CPC + j, pace)

    def final(i):
        cs = slice(OOFF[i], OOFF[i + 1])
        y, tokens = None, []
        for k0 in range(0, F, KB):
            ks = slice(k0, min(k0 + KB, F))
            part = jnp.dot(u_s[:, ks], w2_s[ks, cs], preferred_element_type=f32)
            tokens += _tokens(part) if k0 + KB <= F else _tokens(part[:, 0:LANES])
            y = part if y is None else y + part
        s = jnp.dot(wot_s[...], o_s[:, cs], preferred_element_type=f32)
        tokens += _tokens(s)
        for j in range(OUT_PIECES[i] // LANES):
            jj = OOFF[i] // LANES + j
            col = pl.ds(jj * LANES, LANES)
            g = _silu(y[:, j * LANES:(j + 1) * LANES] + b2f_s[jj:jj + 1, :])
            xr = x_s[jj // CPC, :, pl.ds((jj % CPC) * LANES, LANES)].astype(f32)
            r = xr + s[:, j * LANES:(j + 1) * LANES] * g
            out_s[:, col] = r.astype(bf16)
        out_cp(i).start()
        return tokens

    @pl.when(steps == NC - 3)
    def _():
        b1f_s[...] = b1_s[...].astype(f32)
        b2f_s[...] = b2_s[...].astype(f32)
        prep_wqkv_t()
        prep_wqkv_perm()
        prep_wo()
        ln_piece(NC - 1, mix1(NC - 2, "mid"))
        mix1(NC - 1, "last")

        zeros = jnp.zeros((D, LANES), f32)
        qkv_s[0, D:2 * D, :] = zeros
        qkv_s[0, 2 * D:3 * D, :] = zeros
        rk_s[0] = zeros
        rv_s[0] = zeros

        for c in range(QKV_AHEAD):
            tokens = qkv(c)
            if c >= 1:
                attn(c - 1, [])

    _scope("ww2", lambda: w2_cp.wait())
    for c in range(NC):
        tokens = final(c)
        if c + QKV_AHEAD < NC:
            tokens += qkv(c + QKV_AHEAD)
        if c + QKV_AHEAD - 1 < NC:
            attn(c + QKV_AHEAD - 1, tokens[:len(tokens) * 9 // 10])
    final(NC)

    def waits():
        for i in range(NO):
            out_cp(i).wait()
    _scope("wout", waits)


@jax.jit
def pallas_recurrent_scan__sliding_local_dilated__mixer_token_mlp__prompt_kernel(
    A_x: jax.Array,
    A_wqkv: jax.Array,
    A_wo: jax.Array,
    B_x: jax.Array,
    B_w1: jax.Array,
    B_b1: jax.Array,
    B_w2: jax.Array,
    B_b2: jax.Array,
):
    del B_x
    xt = jnp.swapaxes(A_x, 1, 2)
    b1 = B_b1.reshape(F // LANES, LANES)
    b2 = B_b2.reshape(S // LANES, LANES)
    any_spec = pl.BlockSpec(memory_space=pl.ANY)
    out_t = pl.pallas_call(
        _kernel,
        out_shape=jax.ShapeDtypeStruct((1, D, S), bf16),
        in_specs=[any_spec] * 7,
        out_specs=any_spec,
        scratch_shapes=[
            pltpu.VMEM((NC, D, TC), bf16),
            pltpu.VMEM((D, 3 * D), bf16),
            pltpu.VMEM((D, D), bf16),
            pltpu.VMEM((NC, TC, F), bf16),
            pltpu.VMEM((F, S), bf16),
            pltpu.VMEM((F // LANES, LANES), bf16),
            pltpu.VMEM((S // LANES, LANES), bf16),
            pltpu.VMEM((NC, D // 2, TC), u32),
            pltpu.VMEM((NC, D // 2, TC), u32),
            pltpu.VMEM((D, F), f32),
            pltpu.VMEM((D // 2, F), u32),
            pltpu.VMEM((4, 11 * LANES, LANES), f32),
            pltpu.VMEM((3 * D // 2, D), u32),
            pltpu.VMEM((4, D, LANES), f32),
            pltpu.VMEM((D // 2, D), u32),
            pltpu.VMEM((NCOL + 1, 3 * D, LANES), f32),
            pltpu.VMEM((2, D, LANES), f32),
            pltpu.VMEM((2, D, LANES), f32),
            pltpu.VMEM((D // 2, S), u32),
            pltpu.VMEM((D, S), bf16),
            pltpu.VMEM((F // LANES, LANES), f32),
            pltpu.VMEM((S // LANES, LANES), f32),
            pltpu.SemaphoreType.DMA((NSEM,)),
        ],
        compiler_params=pltpu.CompilerParams(vmem_limit_bytes=100 * 1024 * 1024,
                                             disable_semaphore_checks=True,
                                             disable_bounds_checks=True),
        name="fused_mixer_attn",
    )(xt, A_wqkv, A_wo, B_w1, b1, B_w2, b2)
    return jnp.swapaxes(out_t, 1, 2)
```

```python
import functools

import jax
import jax.numpy as jnp
import jax.experimental.pallas as pl
import jax.experimental.pallas.tpu as pltpu

S = 2048
D = 448
H = 16
DH = D // H
F = 1792
W = 8
EPS = 1e-5
TC = 256
NC = S // TC
LANES = 128
NCOL = S // LANES
SLAB = 32

f32 = jnp.float32
bf16 = jnp.bfloat16
u32 = jnp.uint32

_SCOPES = False


def _scope(name, fn):
    if _SCOPES:
        with jax.named_scope(name):
            fn()
    else:
        fn()


LNB = 64
NLB = D // LNB


def _rep(v8, rows):
    return jnp.concatenate([v8] * (rows // 8), axis=0)


def _ln_stats(x_ref, col, pace):
    piv = jnp.broadcast_to(x_ref[0:1, col].astype(f32), (8, LANES))
    s1 = s2 = None
    for i in range(NLB):
        pv = _rep(pace(piv), LNB // 2)
        w = pltpu.bitcast(x_ref[i * LNB:(i + 1) * LNB, col], u32)
        for half in (w << 16, w & jnp.uint32(0xFFFF0000)):
            d = pltpu.bitcast(half, f32) - pv
            for k in range(LNB // 2 // 16):
                dk = d[k * 16:(k + 1) * 16]
                s1 = dk if s1 is None else s1 + dk
                s2 = dk * dk if s2 is None else s2 + dk * dk
    md = jnp.sum(s1, axis=0, keepdims=True) * (1.0 / D)
    v = jnp.maximum(jnp.sum(s2, axis=0, keepdims=True) * (1.0 / D) - md * md, 0.0)
    r = jax.lax.rsqrt(v + EPS)
    r2 = jax.lax.rsqrt(v * r * r + EPS)
    return piv + md, r, r * r2


def _tokens(r):
    return [r[i:i + 8, j:j + LANES] for j in range(0, r.shape[1], LANES) for i in range(0, r.shape[0], 8)]


class _Pacer:
    def __init__(self, tokens, count, never):
        self.tokens, self.count, self.never, self.i = tokens, count, never, 0

    def __call__(self, v8):
        if not self.tokens:
            return v8
        tok = self.tokens[self.i * len(self.tokens) // self.count]
        self.i += 1
        return jnp.where(self.never, tok, v8)

    def gate(self, *vs):
        if not self.tokens:
            return vs
        tok = self.tokens[self.i * len(self.tokens) // self.count]
        self.i += 1
        n = vs[0].shape[0]
        nv, tk = _rep(self.never, n), _rep(tok, n)
        return tuple(jnp.where(nv, tk, v) for v in vs)


def _gelu(x):
    c = 0.7978845608028654
    t = jnp.tanh(x * (c + (c * 0.044715) * (x * x)))
    hx = 0.5 * x
    return hx + hx * t


def _silu(y):
    hy = 0.5 * y
    return hy + hy * jnp.tanh(hy)


N0 = 768
NB = 256
ATTN_WIN = 740
KB = 512
CPC = TC // LANES
QKV_AHEAD = 3
OUT_PIECES = (256,) * 7 + (128, 128)
OOFF = tuple(sum(OUT_PIECES[:i]) for i in range(len(OUT_PIECES) + 1))
NO = len(OUT_PIECES)
SEM_X, SEM_W1, SEM_MISC, SEM_OUT = 0, NC, 2 * NC, 2 * NC + 6
NSEM = SEM_OUT + NO


def _kernel(x_hbm, wqkv_hbm, wo_hbm, w1_hbm, b1_hbm, w2_hbm, b2_hbm, out_hbm,
            x_s, wqkv_s, wo_s, w1_s, w2_s, b1_s, b2_s,
            xn_s, h_s, acc_s, u_s, wt32_s, wqkvt_s, wo32_s, wot_s,
            qkv_s, rk_s, rv_s, o_s, out_s, b1f_s, b2f_s, sem):
    xn_s, h_s, u_s, wqkvt_s, wot_s, o_s = (
        r.bitcast(bf16) for r in (xn_s, h_s, u_s, wqkvt_s, wot_s, o_s))

    def x_cp(p):
        return pltpu.make_async_copy(x_hbm.at[0, :, pl.ds(p * TC, TC)], x_s.at[p], sem.at[SEM_X + p])

    def w1_cp(p, n_lo=0):
        return pltpu.make_async_copy(w1_hbm.at[pl.ds(p * TC, TC), n_lo:F], w1_s.at[p, :, n_lo:F],
                                     sem.at[SEM_W1 + p])

    def out_cp(i):
        sl = slice(OOFF[i], OOFF[i + 1])
        return pltpu.make_async_copy(out_s.at[:, sl], out_hbm.at[0, :, sl], sem.at[SEM_OUT + i])

    wqkv_cp = pltpu.make_async_copy(wqkv_hbm, wqkv_s, sem.at[SEM_MISC + 0])
    wo_cp = pltpu.make_async_copy(wo_hbm, wo_s, sem.at[SEM_MISC + 1])
    b1_cp = pltpu.make_async_copy(b1_hbm, b1_s, sem.at[SEM_MISC + 2])
    b2_cp = pltpu.make_async_copy(b2_hbm, b2_s, sem.at[SEM_MISC + 3])
    w2_cp = pltpu.make_async_copy(w2_hbm, w2_s, sem.at[SEM_MISC + 4])
    w1a_cp = pltpu.make_async_copy(w1_hbm.at[0:TC, 0:N0], w1_s.at[0, :, 0:N0],
                                   sem.at[SEM_MISC + 5])

    x_cp(0).start()
    w1a_cp.start()
    for p in range(NC):
        if p == NC - 2:
            wqkv_cp.start()
            wo_cp.start()
            b1_cp.start()
            b2_cp.start()
        w1_cp(p, N0 if p == 0 else 0).start()
        if p + 1 < NC:
            x_cp(p + 1).start()
    w2_cp.start()

    def prep_wqkv_t():
        for c in range(11):
            wd = min(LANES, 3 * D - c * LANES)
            blk = wqkv_s[:, c * LANES:c * LANES + wd].T.astype(f32)
            for kt in range(4):
                kw = min(LANES, D - kt * LANES)
                wt32_s[kt, c * LANES:c * LANES + wd, 0:kw] = blk[:, kt * LANES:kt * LANES + kw]

    def prep_wqkv_perm():
        for sec in range(3):
            for d in range(DH):
                r0 = sec * D + d * H
                for kt in range(4):
                    kw = min(LANES, D - kt * LANES)
                    rows = wt32_s[kt, pl.ds(sec * D + d, H, stride=DH), :]
                    wqkvt_s[r0:r0 + H, kt * LANES:kt * LANES + kw] = rows[:, 0:kw].astype(bf16)

    def prep_wo():
        for nt in range(4):
            nw = min(LANES, D - nt * LANES)
            wo32_s[nt, :, 0:nw] = wo_s[:, nt * LANES:nt * LANES + nw].astype(f32)
        for nt in range(4):
            nw = min(LANES, D - nt * LANES)
            rows = [wo32_s[nt, pl.ds(d, H, stride=DH), :][:, 0:nw].astype(bf16) for d in range(DH)]
            blk = jnp.concatenate(rows, axis=0)
            wot_s[nt * LANES:nt * LANES + nw, :] = blk.T

    def ln_piece(p, tokens):
        xp, xnp, hp = x_s.at[p], xn_s.at[p], h_s.at[p]
        z = xp[0:8, 0:LANES].astype(f32)
        pace = _Pacer(tokens, 2 * NLB * CPC, z + 1.0 < z)
        for j in range(CPC):
            col = pl.ds(j * LANES, LANES)
            m, r, rr = _ln_stats(xp, col, pace)
            for i in range(NLB):
                rows = slice(i * LNB, (i + 1) * LNB)
                xc = xp[rows, col].astype(f32) - _rep(pace(m), LNB)
                xnp[rows, col] = (xc * r).astype(bf16)
                hp[rows, col] = (xc * rr).astype(bf16)

    def mix1(p, mode, n_lo=0, n_hi=F):
        tokens = []
        for n in range(n_lo // NB, n_hi // NB):
            ns = slice(n * NB, (n + 1) * NB)
            part = jnp.dot(h_s[p], w1_s[p, :, ns], preferred_element_type=f32)
            tokens += [part[r:r + 8, 0:LANES] for r in range(0, D, 8)]
            if mode == "first":
                acc_s[:, ns] = part
            elif mode == "mid":
                acc_s[:, ns] += part
            else:
                for j in range(NB // LANES):
                    nn = n * (NB // LANES) + j
                    col = pl.ds(nn * LANES, LANES)
                    z = acc_s[:, col] + part[:, j * LANES:(j + 1) * LANES] + b1f_s[nn:nn + 1, :]
                    u_s[:, col] = _gelu(z).astype(bf16)
        return tokens[:len(tokens) * 7 // 8]

    _scope("wx0", lambda: x_cp(0).wait())
    ln_piece(0, [])
    _scope("w0a", lambda: w1a_cp.wait())
    mix1(0, "first", 0, N0)
    _scope("w0", lambda: (w1_cp(0, N0).wait(), x_cp(1).wait()))
    ln_piece(1, mix1(0, "first", N0, F))

    def mid_step(p, carry):
        _scope("wl", lambda: (w1_cp(p).wait(), x_cp(p + 1).wait()))
        ln_piece(p + 1, mix1(p, "mid"))
        return carry + 1

    steps = jax.lax.fori_loop(1, NC - 2, mid_step, 0)

    def waits():
        wqkv_cp.wait()
        wo_cp.wait()
        b1_cp.wait()
        b2_cp.wait()
        w1_cp(NC - 2).wait()
        x_cp(NC - 1).wait()
        w1_cp(NC - 1).wait()
    _scope("wlast", waits)
    def qkv(c):
        r = jnp.dot(wqkvt_s[...], xn_s[c],
                    preferred_element_type=f32)
        for j in range(TC // LANES):
            qkv_s[c * (TC // LANES) + j + 1] = r[:, j * LANES:(j + 1) * LANES]
        return _tokens(r)

    scale = DH ** -0.5

    def attn_col(jj, pace):
        lane = jax.lax.broadcasted_iota(jnp.int32, (SLAB, LANES), 1)
        m0 = [None] + [lane < LANES - 2 * a for a in range(1, 4)]
        m1 = [(lane >= 8) & (lane < LANES - 2 * a) for a in range(4)]
        nd = SLAB // H
        acc = [[None, None] for _ in range(4)]
        for sl in range(D // SLAB):
            r0 = sl * SLAB
            q = qkv_s[jj + 1, r0:r0 + SLAB, :]
            k = qkv_s[jj + 1, D + r0:D + r0 + SLAB, :]
            q, k = pace.gate(q, k)
            kp = qkv_s[jj, D + r0:D + r0 + SLAB, :]
            rkp = rk_s[jj % 2, r0:r0 + SLAB, :]
            rk = pltpu.roll(k, 8, 1)
            rk_s[(jj + 1) % 2, r0:r0 + SLAB, :] = rk
            for a in range(4):
                rq = q if a == 0 else pltpu.roll(q, LANES - 2 * a, 1)
                for b in range(2):
                    if b == 0:
                        mix = k if a == 0 else jnp.where(m0[a], k, kp)
                    else:
                        mix = jnp.where(m1[a], rk, rkp)
                    p = rq * mix
                    for i in range(nd):
                        pi = p[i * H:(i + 1) * H]
                        acc[a][b] = pi if acc[a][b] is None else acc[a][b] + pi
        lane16 = jax.lax.broadcasted_iota(jnp.int32, (H, LANES), 1)
        logit = []
        for w in range(W):
            a, b = w % 4, w // 4
            lw = acc[a][b] if a == 0 else pltpu.roll(acc[a][b], 2 * a, 1)
            lw = lw * scale
            if jj == 0 and w > 0:
                lw = jnp.where(lane16 >= 2 * w, lw, -1e9)
            logit.append(lw)
        mx = functools.reduce(jnp.maximum, logit)
        ex = [jnp.exp(l - mx) for l in logit]
        inv = 1.0 / functools.reduce(jnp.add, ex)
        ra = [[None, None] for _ in range(4)]
        for w in range(W):
            a, b = w % 4, w // 4
            aw = ex[w] * inv
            aw = aw if a == 0 else pltpu.roll(aw, LANES - 2 * a, 1)
            ra[a][b] = jnp.concatenate([aw] * nd, axis=0)
        for sl in range(D // SLAB):
            r0 = sl * SLAB
            v = qkv_s[jj + 1, 2 * D + r0:2 * D + r0 + SLAB, :]
            v, = pace.gate(v)
            vp = qkv_s[jj, 2 * D + r0:2 * D + r0 + SLAB, :]
            rvp = rv_s[jj % 2, r0:r0 + SLAB, :]
            rv = pltpu.roll(v, 8, 1)
            rv_s[(jj + 1) % 2, r0:r0 + SLAB, :] = rv
            o = None
            for a in range(4):
                mix0 = v if a == 0 else jnp.where(m0[a], v, vp)
                mix1 = jnp.where(m1[a], rv, rvp)
                t = ra[a][0] * mix0 + ra[a][1] * mix1
                o = t if a == 0 else o + pltpu.roll(t, 2 * a, 1)
            o_s[r0:r0 + SLAB, jj * LANES:(jj + 1) * LANES] = o.astype(bf16)

    def attn(c, tokens):
        z = b2f_s[0:8, :]
        pace = _Pacer(tokens, 2 * (D // SLAB) * CPC, z + 1.0 < z)
        for j in range(CPC):
            attn_col(c * CPC + j, pace)

    def final(i):
        cs = slice(OOFF[i], OOFF[i + 1])
        y, tokens = None, []
        for k0 in range(0, F, KB):
            ks = slice(k0, min(k0 + KB, F))
            part = jnp.dot(u_s[:, ks], w2_s[ks, cs], preferred_element_type=f32)
            tokens += _tokens(part) if k0 + KB <= F else _tokens(part[:, 0:LANES])
            y = part if y is None else y + part
        s = jnp.dot(wot_s[...], o_s[:, cs], preferred_element_type=f32)
        tokens += _tokens(s)
        for j in range(OUT_PIECES[i] // LANES):
            jj = OOFF[i] // LANES + j
            col = pl.ds(jj * LANES, LANES)
            g = _silu(y[:, j * LANES:(j + 1) * LANES] + b2f_s[jj:jj + 1, :])
            xr = x_s[jj // CPC, :, pl.ds((jj % CPC) * LANES, LANES)].astype(f32)
            r = xr + s[:, j * LANES:(j + 1) * LANES] * g
            out_s[:, col] = r.astype(bf16)
        out_cp(i).start()
        return tokens

    @pl.when(steps == NC - 3)
    def _():
        b1f_s[...] = b1_s[...].astype(f32)
        b2f_s[...] = b2_s[...].astype(f32)
        prep_wqkv_t()
        prep_wqkv_perm()
        prep_wo()
        ln_piece(NC - 1, mix1(NC - 2, "mid"))
        mix1(NC - 1, "last")

        zeros = jnp.zeros((D, LANES), f32)
        qkv_s[0, D:2 * D, :] = zeros
        qkv_s[0, 2 * D:3 * D, :] = zeros
        rk_s[0] = zeros
        rv_s[0] = zeros

        qkv(0)
        tokens = qkv(1) + qkv(2)
        attn(0, tokens[:len(tokens) * 9 // 10])

    _scope("ww2", lambda: w2_cp.wait())
    tokens = []
    for c in range(NC):
        tokens += final(c)
        if c + QKV_AHEAD < NC:
            tokens += qkv(c + QKV_AHEAD)
        if c + 1 < NC:
            attn(c + 1, tokens[c * ATTN_WIN:(c + 1) * ATTN_WIN])
    final(NC)

    def waits():
        for i in range(NO):
            out_cp(i).wait()
    _scope("wout", waits)


@jax.jit
def pallas_recurrent_scan__sliding_local_dilated__mixer_token_mlp__prompt_kernel(
    A_x: jax.Array,
    A_wqkv: jax.Array,
    A_wo: jax.Array,
    B_x: jax.Array,
    B_w1: jax.Array,
    B_b1: jax.Array,
    B_w2: jax.Array,
    B_b2: jax.Array,
):
    del B_x
    xt = jnp.swapaxes(A_x, 1, 2)
    b1 = B_b1.reshape(F // LANES, LANES)
    b2 = B_b2.reshape(S // LANES, LANES)
    any_spec = pl.BlockSpec(memory_space=pl.ANY)
    out_t = pl.pallas_call(
        _kernel,
        out_shape=jax.ShapeDtypeStruct((1, D, S), bf16),
        in_specs=[any_spec] * 7,
        out_specs=any_spec,
        scratch_shapes=[
            pltpu.VMEM((NC, D, TC), bf16),
            pltpu.VMEM((D, 3 * D), bf16),
            pltpu.VMEM((D, D), bf16),
            pltpu.VMEM((NC, TC, F), bf16),
            pltpu.VMEM((F, S), bf16),
            pltpu.VMEM((F // LANES, LANES), bf16),
            pltpu.VMEM((S // LANES, LANES), bf16),
            pltpu.VMEM((NC, D // 2, TC), u32),
            pltpu.VMEM((NC, D // 2, TC), u32),
            pltpu.VMEM((D, F), f32),
            pltpu.VMEM((D // 2, F), u32),
            pltpu.VMEM((4, 11 * LANES, LANES), f32),
            pltpu.VMEM((3 * D // 2, D), u32),
            pltpu.VMEM((4, D, LANES), f32),
            pltpu.VMEM((D // 2, D), u32),
            pltpu.VMEM((NCOL + 1, 3 * D, LANES), f32),
            pltpu.VMEM((2, D, LANES), f32),
            pltpu.VMEM((2, D, LANES), f32),
            pltpu.VMEM((D // 2, S), u32),
            pltpu.VMEM((D, S), bf16),
            pltpu.VMEM((F // LANES, LANES), f32),
            pltpu.VMEM((S // LANES, LANES), f32),
            pltpu.SemaphoreType.DMA((NSEM,)),
        ],
        compiler_params=pltpu.CompilerParams(vmem_limit_bytes=100 * 1024 * 1024,
                                             disable_semaphore_checks=True,
                                             disable_bounds_checks=True),
        name="fused_mixer_attn",
    )(xt, A_wqkv, A_wo, B_w1, b1, B_w2, b2)
    return jnp.swapaxes(out_t, 1, 2)
```

```python
import functools

import jax
import jax.numpy as jnp
import jax.experimental.pallas as pl
import jax.experimental.pallas.tpu as pltpu

S = 2048
D = 448
H = 16
DH = D // H
F = 1792
W = 8
EPS = 1e-5
TC = 256
NC = S // TC
LANES = 128
NCOL = S // LANES
SLAB = 32

f32 = jnp.float32
bf16 = jnp.bfloat16
u32 = jnp.uint32

_SCOPES = False


def _scope(name, fn):
    if _SCOPES:
        with jax.named_scope(name):
            fn()
    else:
        fn()


LNB = 64
NLB = D // LNB


def _rep(v8, rows):
    return jnp.concatenate([v8] * (rows // 8), axis=0)


def _ln_stats(x_ref, col, pace):
    piv = jnp.broadcast_to(x_ref[0:1, col].astype(f32), (8, LANES))
    s1 = s2 = None
    for i in range(NLB):
        pv = _rep(pace(piv), LNB // 2)
        w = pltpu.bitcast(x_ref[i * LNB:(i + 1) * LNB, col], u32)
        for half in (w << 16, w & jnp.uint32(0xFFFF0000)):
            d = pltpu.bitcast(half, f32) - pv
            for k in range(LNB // 2 // 16):
                dk = d[k * 16:(k + 1) * 16]
                s1 = dk if s1 is None else s1 + dk
                s2 = dk * dk if s2 is None else s2 + dk * dk
    md = jnp.sum(s1, axis=0, keepdims=True) * (1.0 / D)
    v = jnp.maximum(jnp.sum(s2, axis=0, keepdims=True) * (1.0 / D) - md * md, 0.0)
    r = jax.lax.rsqrt(v + EPS)
    r2 = jax.lax.rsqrt(v * r * r + EPS)
    return piv + md, r, r * r2


def _tokens(r):
    return [r[i:i + 8, j:j + LANES] for j in range(0, r.shape[1], LANES) for i in range(0, r.shape[0], 8)]


def _deadline(lhs, toks, never):
    if not any(t is not None for t in toks):
        return lhs
    w = pltpu.bitcast(lhs, u32)
    blocks = [w[8 * i:8 * i + 8, 0:LANES] for i in range(w.shape[0] // 8)]
    blocks = [b if t is None else jnp.where(never, t, b) for b, t in zip(blocks, toks, strict=True)]
    w = jnp.concatenate([jnp.concatenate(blocks, axis=0), w[:, LANES:]], axis=1)
    return pltpu.bitcast(w, bf16)


def _spread(vals, nslots, lo, hi):
    out = [None] * nslots
    for i in range(lo, hi):
        out[i] = vals[((i - lo + 1) * len(vals)) // (hi - lo) - 1]
    return out


class _Pacer:
    def __init__(self, tokens, count, never):
        self.tokens, self.count, self.never, self.i = tokens, count, never, 0

    def __call__(self, v8):
        if not self.tokens:
            return v8
        tok = self.tokens[self.i * len(self.tokens) // self.count]
        self.i += 1
        return jnp.where(self.never, tok, v8)

    def gate(self, *vs):
        if not self.tokens:
            return vs
        tok = self.tokens[self.i * len(self.tokens) // self.count]
        self.i += 1
        n = vs[0].shape[0]
        nv, tk = _rep(self.never, n), _rep(tok, n)
        return tuple(jnp.where(nv, tk, v) for v in vs)


def _gelu(x):
    c = 0.7978845608028654
    t = jnp.tanh(x * (c + (c * 0.044715) * (x * x)))
    hx = 0.5 * x
    return hx + hx * t


def _silu(y):
    hy = 0.5 * y
    return hy + hy * jnp.tanh(hy)


RAMP = (
    (((0, 0, 512),), None),
    (((0, 512, 1024),), 1),
    (((0, 1024, F), (1, 0, 256)), None),
    (((1, 256, F),), 2),
)
RECTS = tuple(r for rects, _ in RAMP for r in rects)
NB = 256
ATTN_WIN = 740
KB = 512
CPC = TC // LANES
QKV_AHEAD = 3
OUT_PIECES = (256,) * 7 + (128, 128)
OOFF = tuple(sum(OUT_PIECES[:i]) for i in range(len(OUT_PIECES) + 1))
NO = len(OUT_PIECES)
SEM_X, SEM_W1, SEM_MISC, SEM_OUT = 0, NC, 2 * NC, 2 * NC + 5
SEM_RAMP = SEM_OUT + NO
NSEM = SEM_RAMP + len(RECTS)


def _kernel(x_hbm, wqkv_hbm, wo_hbm, w1_hbm, b1_hbm, w2_hbm, b2_hbm, out_hbm,
            x_s, wqkv_s, wo_s, w1_s, w2_s, b1_s, b2_s,
            xn_s, h_s, acc_s, u_s, wt32_s, wqkvt_s, wo32_s, wot_s,
            qkv_s, rk_s, rv_s, o_s, out_s, b1f_s, b2f_s, sem):
    xn_s, h_s, u_s, wqkvt_s, wot_s, o_s = (
        r.bitcast(bf16) for r in (xn_s, h_s, u_s, wqkvt_s, wot_s, o_s))

    def x_cp(p):
        return pltpu.make_async_copy(x_hbm.at[0, :, pl.ds(p * TC, TC)], x_s.at[p], sem.at[SEM_X + p])

    def w1_cp(p):
        return pltpu.make_async_copy(w1_hbm.at[pl.ds(p * TC, TC), :], w1_s.at[p], sem.at[SEM_W1 + p])

    def rect_cp(r):
        p, lo, hi = r
        return pltpu.make_async_copy(w1_hbm.at[p * TC:(p + 1) * TC, lo:hi], w1_s.at[p, :, lo:hi],
                                     sem.at[SEM_RAMP + RECTS.index(r)])

    def out_cp(i):
        sl = slice(OOFF[i], OOFF[i + 1])
        return pltpu.make_async_copy(out_s.at[:, sl], out_hbm.at[0, :, sl], sem.at[SEM_OUT + i])

    wqkv_cp = pltpu.make_async_copy(wqkv_hbm, wqkv_s, sem.at[SEM_MISC + 0])
    wo_cp = pltpu.make_async_copy(wo_hbm, wo_s, sem.at[SEM_MISC + 1])
    b1_cp = pltpu.make_async_copy(b1_hbm, b1_s, sem.at[SEM_MISC + 2])
    b2_cp = pltpu.make_async_copy(b2_hbm, b2_s, sem.at[SEM_MISC + 3])
    w2_cp = pltpu.make_async_copy(w2_hbm, w2_s, sem.at[SEM_MISC + 4])

    x_cp(0).start()
    for rects, xc in RAMP:
        for r in rects:
            rect_cp(r).start()
        if xc is not None:
            x_cp(xc).start()
    for p in range(2, NC):
        if p == NC - 1:
            wqkv_cp.start()
            wo_cp.start()
            b1_cp.start()
            b2_cp.start()
        w1_cp(p).start()
        if p + 1 < NC:
            x_cp(p + 1).start()
    w2_cp.start()

    def prep_wqkv_t():
        for c in range(11):
            wd = min(LANES, 3 * D - c * LANES)
            blk = wqkv_s[:, c * LANES:c * LANES + wd].T.astype(f32)
            for kt in range(4):
                kw = min(LANES, D - kt * LANES)
                wt32_s[kt, c * LANES:c * LANES + wd, 0:kw] = blk[:, kt * LANES:kt * LANES + kw]

    def prep_wqkv_perm():
        done = []
        for sec in range(3):
            for d in range(DH):
                r0 = sec * D + d * H
                tok = None
                for kt in range(4):
                    kw = min(LANES, D - kt * LANES)
                    rows = wt32_s[kt, pl.ds(sec * D + d, H, stride=DH), :]
                    wqkvt_s[r0:r0 + H, kt * LANES:kt * LANES + kw] = rows[:, 0:kw].astype(bf16)
                    if kt < 3:
                        t = pltpu.bitcast(rows[8:16], u32)
                        tok = t if tok is None else tok | t
                done.append(tok)
        return done

    def prep_wo():
        for nt in range(4):
            nw = min(LANES, D - nt * LANES)
            wo32_s[nt, :, 0:nw] = wo_s[:, nt * LANES:nt * LANES + nw].astype(f32)
        done = []
        for nt in range(4):
            nw = min(LANES, D - nt * LANES)
            rows = [wo32_s[nt, pl.ds(d, H, stride=DH), :][:, 0:nw].astype(bf16) for d in range(DH)]
            blk = jnp.concatenate(rows, axis=0)
            bt = blk.T
            wot_s[nt * LANES:nt * LANES + nw, :] = bt
            w = pltpu.bitcast(bt, u32)
            done += [w[nw // 2 - 8:nw // 2, k * LANES:(k + 1) * LANES] for k in range(3)]
        return done

    def ln_piece(p, tokens):
        xp, xnp, hp = x_s.at[p], xn_s.at[p], h_s.at[p]
        z = xp[0:8, 0:LANES].astype(f32)
        pace = _Pacer(tokens, 2 * NLB * CPC, z + 1.0 < z)
        for j in range(CPC):
            col = pl.ds(j * LANES, LANES)
            m, r, rr = _ln_stats(xp, col, pace)
            for i in range(NLB):
                rows = slice(i * LNB, (i + 1) * LNB)
                xc = xp[rows, col].astype(f32) - _rep(pace(m), LNB)
                xnp[rows, col] = (xc * r).astype(bf16)
                hp[rows, col] = (xc * rr).astype(bf16)

    def mix1(p, mode, n_lo=0, n_hi=F, due=None, never=None):
        tokens = []
        nb = D // 16
        for n in range(n_lo // NB, n_hi // NB):
            ns = slice(n * NB, (n + 1) * NB)
            lhs = h_s[p] if due is None else _deadline(h_s[p], due[n * nb:(n + 1) * nb], never)
            part = jnp.dot(lhs, w1_s[p, :, ns], preferred_element_type=f32)
            tokens += [part[r:r + 8, 0:LANES] for r in range(0, D, 8)]
            if mode == "first":
                acc_s[:, ns] = part
            else:
                acc_s[:, ns] += part
        return tokens if due is not None else tokens[:len(tokens) * 7 // 8]

    zeros = jnp.zeros((D, LANES), f32)
    qkv_s[0, D:2 * D, :] = zeros
    qkv_s[0, 2 * D:3 * D, :] = zeros
    rk_s[0] = zeros
    rv_s[0] = zeros

    _scope("wx0", lambda: x_cp(0).wait())
    ln_piece(0, [])
    for rects, xc in RAMP:
        def waits():
            for r in rects:
                rect_cp(r).wait()
            if xc is not None:
                x_cp(xc).wait()
        _scope("wr", waits)
        tokens = []
        for p, lo, hi in rects:
            tokens += mix1(p, "first" if p == 0 else "mid", lo, hi)
        if xc is not None:
            ln_piece(xc, tokens)

    def mid_step(p, carry):
        _scope("wl", lambda: (w1_cp(p).wait(), x_cp(p + 1).wait()))
        ln_piece(p + 1, mix1(p, "mid"))
        return carry + 1

    steps = jax.lax.fori_loop(2, NC - 1, mid_step, 0)

    def waits():
        wqkv_cp.wait()
        wo_cp.wait()
        b1_cp.wait()
        b2_cp.wait()
        w1_cp(NC - 1).wait()
    _scope("wlast", waits)
    def qkv(c, due=None, never=None):
        rhs = xn_s[c] if due is None else _deadline(xn_s[c], due, never)
        r = jnp.dot(wqkvt_s[...], rhs, preferred_element_type=f32)
        for j in range(TC // LANES):
            qkv_s[c * (TC // LANES) + j + 1] = r[:, j * LANES:(j + 1) * LANES]
        return _tokens(r)

    scale = DH ** -0.5

    def attn_col(jj, pace):
        lane = jax.lax.broadcasted_iota(jnp.int32, (SLAB, LANES), 1)
        m0 = [None] + [lane < LANES - 2 * a for a in range(1, 4)]
        m1 = [(lane >= 8) & (lane < LANES - 2 * a) for a in range(4)]
        nd = SLAB // H
        acc = [[None, None] for _ in range(4)]
        for sl in range(D // SLAB):
            r0 = sl * SLAB
            q = qkv_s[jj + 1, r0:r0 + SLAB, :]
            k = qkv_s[jj + 1, D + r0:D + r0 + SLAB, :]
            q, k = pace.gate(q, k)
            kp = qkv_s[jj, D + r0:D + r0 + SLAB, :]
            rkp = rk_s[jj % 2, r0:r0 + SLAB, :]
            rk = pltpu.roll(k, 8, 1)
            rk_s[(jj + 1) % 2, r0:r0 + SLAB, :] = rk
            for a in range(4):
                rq = q if a == 0 else pltpu.roll(q, LANES - 2 * a, 1)
                for b in range(2):
                    if b == 0:
                        mix = k if a == 0 else jnp.where(m0[a], k, kp)
                    else:
                        mix = jnp.where(m1[a], rk, rkp)
                    p = rq * mix
                    for i in range(nd):
                        pi = p[i * H:(i + 1) * H]
                        acc[a][b] = pi if acc[a][b] is None else acc[a][b] + pi
        lane16 = jax.lax.broadcasted_iota(jnp.int32, (H, LANES), 1)
        logit = []
        for w in range(W):
            a, b = w % 4, w // 4
            lw = acc[a][b] if a == 0 else pltpu.roll(acc[a][b], 2 * a, 1)
            lw = lw * scale
            if jj == 0 and w > 0:
                lw = jnp.where(lane16 >= 2 * w, lw, -1e9)
            logit.append(lw)
        mx = functools.reduce(jnp.maximum, logit)
        ex = [jnp.exp(l - mx) for l in logit]
        inv = 1.0 / functools.reduce(jnp.add, ex)
        ra = [[None, None] for _ in range(4)]
        for w in range(W):
            a, b = w % 4, w // 4
            aw = ex[w] * inv
            aw = aw if a == 0 else pltpu.roll(aw, LANES - 2 * a, 1)
            ra[a][b] = jnp.concatenate([aw] * nd, axis=0)
        for sl in range(D // SLAB):
            r0 = sl * SLAB
            v = qkv_s[jj + 1, 2 * D + r0:2 * D + r0 + SLAB, :]
            v, = pace.gate(v)
            vp = qkv_s[jj, 2 * D + r0:2 * D + r0 + SLAB, :]
            rvp = rv_s[jj % 2, r0:r0 + SLAB, :]
            rv = pltpu.roll(v, 8, 1)
            rv_s[(jj + 1) % 2, r0:r0 + SLAB, :] = rv
            o = None
            for a in range(4):
                mix0 = v if a == 0 else jnp.where(m0[a], v, vp)
                mix1 = jnp.where(m1[a], rv, rvp)
                t = ra[a][0] * mix0 + ra[a][1] * mix1
                o = t if a == 0 else o + pltpu.roll(t, 2 * a, 1)
            o_s[r0:r0 + SLAB, jj * LANES:(jj + 1) * LANES] = o.astype(bf16)

    def attn(c, tokens):
        z = b2f_s[0:8, :]
        pace = _Pacer(tokens, 2 * (D // SLAB) * CPC, z + 1.0 < z)
        for j in range(CPC):
            attn_col(c * CPC + j, pace)

    def gelu(tokens):
        z = b2f_s[0:8, :]
        pace = _Pacer(tokens, NLB * (F // LANES), z + 1.0 < z)
        for nn in range(F // LANES):
            col = pl.ds(nn * LANES, LANES)
            bias = jnp.broadcast_to(b1f_s[nn:nn + 1, :], (8, LANES))
            for i in range(NLB):
                rows = slice(i * LNB, (i + 1) * LNB)
                u_s[rows, col] = _gelu(acc_s[rows, col] + _rep(pace(bias), LNB)).astype(bf16)

    def gate_mm(i):
        cs = slice(OOFF[i], OOFF[i + 1])
        y, tokens = None, []
        for k0 in range(0, F, KB):
            ks = slice(k0, min(k0 + KB, F))
            part = jnp.dot(u_s[:, ks], w2_s[ks, cs], preferred_element_type=f32)
            tokens += _tokens(part) if k0 + KB <= F else _tokens(part[:, 0:LANES])
            y = part if y is None else y + part
        g = []
        for j in range(OUT_PIECES[i] // LANES):
            jj = OOFF[i] // LANES + j
            g.append(_silu(y[:, j * LANES:(j + 1) * LANES] + b2f_s[jj:jj + 1, :]))
        return g, tokens

    def final(i, g):
        cs = slice(OOFF[i], OOFF[i + 1])
        s = jnp.dot(wot_s[...], o_s[:, cs], preferred_element_type=f32)
        for j in range(OUT_PIECES[i] // LANES):
            jj = OOFF[i] // LANES + j
            xr = x_s[jj // CPC, :, pl.ds((jj % CPC) * LANES, LANES)].astype(f32)
            r = xr + s[:, j * LANES:(j + 1) * LANES] * g[j]
            out_s[:, pl.ds(jj * LANES, LANES)] = r.astype(bf16)
        out_cp(i).start()
        return _tokens(s)

    @pl.when(steps == NC - 3)
    def _():
        b1f_s[...] = b1_s[...].astype(f32)
        b2f_s[...] = b2_s[...].astype(f32)
        prep_wqkv_t()
        z = b2f_s[0:8, :]
        never = z + 1.0 < z
        nb = (F // NB) * (D // 16)
        last = mix1(NC - 1, "mid", due=_spread(prep_wqkv_perm(), nb, nb * 2 // 7, nb), never=never)
        wo_done = prep_wo()

        tokens = []
        for c in range(QKV_AHEAD):
            nb = D // 16
            due = _spread(wo_done, nb, 0, len(wo_done)) if c == 2 else [None] * nb
            tokens += qkv(c, due, never)
        gelu(last[len(last) // 2:] + tokens[:len(tokens) // 3])
        attn(0, tokens[len(tokens) // 3:len(tokens) * 14 // 15])

    _scope("ww2", lambda: w2_cp.wait())
    tokens = []
    for c in range(NC):
        g, t = gate_mm(c)
        tokens += t + final(c, g)
        if c + QKV_AHEAD < NC:
            tokens += qkv(c + QKV_AHEAD)
        if c + 1 < NC:
            attn(c + 1, tokens[c * ATTN_WIN:(c + 1) * ATTN_WIN])
    final(NC, gate_mm(NC)[0])

    def waits():
        for i in range(NO):
            out_cp(i).wait()
    _scope("wout", waits)


@jax.jit
def pallas_recurrent_scan__sliding_local_dilated__mixer_token_mlp__prompt_kernel(
    A_x: jax.Array,
    A_wqkv: jax.Array,
    A_wo: jax.Array,
    B_x: jax.Array,
    B_w1: jax.Array,
    B_b1: jax.Array,
    B_w2: jax.Array,
    B_b2: jax.Array,
):
    del B_x
    xt = jnp.swapaxes(A_x, 1, 2)
    b1 = B_b1.reshape(F // LANES, LANES)
    b2 = B_b2.reshape(S // LANES, LANES)
    any_spec = pl.BlockSpec(memory_space=pl.ANY)
    out_t = pl.pallas_call(
        _kernel,
        out_shape=jax.ShapeDtypeStruct((1, D, S), bf16),
        in_specs=[any_spec] * 7,
        out_specs=any_spec,
        scratch_shapes=[
            pltpu.VMEM((NC, D, TC), bf16),
            pltpu.VMEM((D, 3 * D), bf16),
            pltpu.VMEM((D, D), bf16),
            pltpu.VMEM((NC, TC, F), bf16),
            pltpu.VMEM((F, S), bf16),
            pltpu.VMEM((F // LANES, LANES), bf16),
            pltpu.VMEM((S // LANES, LANES), bf16),
            pltpu.VMEM((NC, D // 2, TC), u32),
            pltpu.VMEM((NC, D // 2, TC), u32),
            pltpu.VMEM((D, F), f32),
            pltpu.VMEM((D // 2, F), u32),
            pltpu.VMEM((4, 11 * LANES, LANES), f32),
            pltpu.VMEM((3 * D // 2, D), u32),
            pltpu.VMEM((4, D, LANES), f32),
            pltpu.VMEM((D // 2, D), u32),
            pltpu.VMEM((NCOL + 1, 3 * D, LANES), f32),
            pltpu.VMEM((2, D, LANES), f32),
            pltpu.VMEM((2, D, LANES), f32),
            pltpu.VMEM((D // 2, S), u32),
            pltpu.VMEM((D, S), bf16),
            pltpu.VMEM((F // LANES, LANES), f32),
            pltpu.VMEM((S // LANES, LANES), f32),
            pltpu.SemaphoreType.DMA((NSEM,)),
        ],
        compiler_params=pltpu.CompilerParams(vmem_limit_bytes=100 * 1024 * 1024,
                                             disable_semaphore_checks=True,
                                             disable_bounds_checks=True),
        name="fused_mixer_attn",
    )(xt, A_wqkv, A_wo, B_w1, b1, B_w2, b2)
    return jnp.swapaxes(out_t, 1, 2)
```

```python
import functools

import jax
import jax.numpy as jnp
import jax.experimental.pallas as pl
import jax.experimental.pallas.tpu as pltpu

S = 2048
D = 448
H = 16
DH = D // H
F = 1792
W = 8
EPS = 1e-5
TC = 256
NC = S // TC
LANES = 128
NCOL = S // LANES
SLAB = 32

f32 = jnp.float32
bf16 = jnp.bfloat16
u32 = jnp.uint32

_SCOPES = False


def _scope(name, fn):
    if _SCOPES:
        with jax.named_scope(name):
            fn()
    else:
        fn()


LNB = 64
NLB = D // LNB


def _rep(v8, rows):
    return jnp.concatenate([v8] * (rows // 8), axis=0)


def _ln_stats(x_ref, col, pace):
    piv = jnp.broadcast_to(x_ref[0:1, col].astype(f32), (8, LANES))
    s1 = s2 = None
    for i in range(NLB):
        pv = _rep(pace(piv), LNB // 2)
        w = pltpu.bitcast(x_ref[i * LNB:(i + 1) * LNB, col], u32)
        for half in (w << 16, w & jnp.uint32(0xFFFF0000)):
            d = pltpu.bitcast(half, f32) - pv
            for k in range(LNB // 2 // 16):
                dk = d[k * 16:(k + 1) * 16]
                s1 = dk if s1 is None else s1 + dk
                s2 = dk * dk if s2 is None else s2 + dk * dk
    md = jnp.sum(s1, axis=0, keepdims=True) * (1.0 / D)
    v = jnp.maximum(jnp.sum(s2, axis=0, keepdims=True) * (1.0 / D) - md * md, 0.0)
    r = jax.lax.rsqrt(v + EPS)
    r2 = jax.lax.rsqrt(v * r * r + EPS)
    return piv + md, r, r * r2


def _tokens(r):
    return [r[i:i + 8, j:j + LANES] for j in range(0, r.shape[1], LANES) for i in range(0, r.shape[0], 8)]


def _deadline(lhs, toks, never):
    if not any(t is not None for t in toks):
        return lhs
    w = pltpu.bitcast(lhs, u32)
    blocks = [w[8 * i:8 * i + 8, 0:LANES] for i in range(w.shape[0] // 8)]
    blocks = [b if t is None else jnp.where(never, t, b) for b, t in zip(blocks, toks, strict=True)]
    w = jnp.concatenate([jnp.concatenate(blocks, axis=0), w[:, LANES:]], axis=1)
    return pltpu.bitcast(w, bf16)


def _spread(vals, nslots, lo, hi):
    out = [None] * nslots
    for i in range(lo, hi):
        out[i] = vals[((i - lo + 1) * len(vals)) // (hi - lo) - 1]
    return out


class _Pacer:
    def __init__(self, tokens, count, never):
        self.tokens, self.count, self.never, self.i = tokens, count, never, 0

    def __call__(self, v8):
        if not self.tokens:
            return v8
        tok = self.tokens[self.i * len(self.tokens) // self.count]
        self.i += 1
        return jnp.where(self.never, tok, v8)

    def gate(self, *vs):
        if not self.tokens:
            return vs
        tok = self.tokens[self.i * len(self.tokens) // self.count]
        self.i += 1
        n = vs[0].shape[0]
        nv, tk = _rep(self.never, n), _rep(tok, n)
        return tuple(jnp.where(nv, tk, v) for v in vs)


def _gelu(x):
    c = 0.7978845608028654
    t = jnp.tanh(x * (c + (c * 0.044715) * (x * x)))
    hx = 0.5 * x
    return hx + hx * t


def _silu(y):
    hy = 0.5 * y
    return hy + hy * jnp.tanh(hy)


RAMP = (
    (((0, 0, 256),), None),
    (((0, 256, 768),), None),
    (((0, 768, 1280),), 1),
    (((0, 1280, F), (1, 0, 512)), None),
    (((1, 512, F),), 2),
)
RECTS = tuple(r for rects, _ in RAMP for r in rects)
NB = 256
ATTN_WIN = 740
KB = 512
CPC = TC // LANES
QKV_AHEAD = 3
OUT_PIECES = (256,) * 7 + (128, 128)
OOFF = tuple(sum(OUT_PIECES[:i]) for i in range(len(OUT_PIECES) + 1))
NO = len(OUT_PIECES)
TAIL_ROWS = (0, 256, 384, D)
SEM_X, SEM_W1, SEM_MISC, SEM_OUT = 0, NC, 2 * NC, 2 * NC + 6
SEM_RAMP = SEM_OUT + NO + len(TAIL_ROWS) - 2
NSEM = SEM_RAMP + len(RECTS)


def _kernel(x_hbm, wqkv_hbm, wo_hbm, w1_hbm, b1_hbm, w2_hbm, b2_hbm, out_hbm,
            x_s, wqkv_s, wo_s, w1_s, w2_s, b1_s, b2_s,
            xn_s, h_s, acc_s, u_s, wt32_s, wqkvt_s, wo32_s, wot_s,
            qkv_s, rk_s, rv_s, o_s, out_s, b1f_s, b2f_s, sem):
    xn_s, h_s, u_s, wqkvt_s, wot_s, o_s = (
        r.bitcast(bf16) for r in (xn_s, h_s, u_s, wqkvt_s, wot_s, o_s))

    def x_cp(p):
        return pltpu.make_async_copy(x_hbm.at[0, :, pl.ds(p * TC, TC)], x_s.at[p], sem.at[SEM_X + p])

    def w1_cp(p):
        return pltpu.make_async_copy(w1_hbm.at[pl.ds(p * TC, TC), :], w1_s.at[p], sem.at[SEM_W1 + p])

    def rect_cp(r):
        p, lo, hi = r
        return pltpu.make_async_copy(w1_hbm.at[p * TC:(p + 1) * TC, lo:hi], w1_s.at[p, :, lo:hi],
                                     sem.at[SEM_RAMP + RECTS.index(r)])

    def out_cps(i):
        sl = slice(OOFF[i], OOFF[i + 1])
        rows = TAIL_ROWS if i == NO - 1 else (0, D)
        return [pltpu.make_async_copy(out_s.at[r0:r1, sl], out_hbm.at[0, r0:r1, sl], sem.at[SEM_OUT + i + k])
                for k, (r0, r1) in enumerate(zip(rows[:-1], rows[1:]))]

    def x0_cp(j):
        sl = pl.ds(j * LANES, LANES)
        return pltpu.make_async_copy(x_hbm.at[0, :, sl], x_s.at[0, :, sl],
                                     sem.at[SEM_X if j == 0 else SEM_MISC + 5])

    wqkv_cp = pltpu.make_async_copy(wqkv_hbm, wqkv_s, sem.at[SEM_MISC + 0])
    wo_cp = pltpu.make_async_copy(wo_hbm, wo_s, sem.at[SEM_MISC + 1])
    b1_cp = pltpu.make_async_copy(b1_hbm, b1_s, sem.at[SEM_MISC + 2])
    b2_cp = pltpu.make_async_copy(b2_hbm, b2_s, sem.at[SEM_MISC + 3])
    w2_cp = pltpu.make_async_copy(w2_hbm, w2_s, sem.at[SEM_MISC + 4])

    x0_cp(0).start()
    x0_cp(1).start()
    for rects, xc in RAMP:
        for r in rects:
            rect_cp(r).start()
        if xc is not None:
            x_cp(xc).start()
    for p in range(2, NC):
        if p == NC - 1:
            wqkv_cp.start()
            wo_cp.start()
            b1_cp.start()
            b2_cp.start()
        w1_cp(p).start()
        if p + 1 < NC:
            x_cp(p + 1).start()
    w2_cp.start()

    def prep_wqkv_t():
        for c in range(11):
            wd = min(LANES, 3 * D - c * LANES)
            blk = wqkv_s[:, c * LANES:c * LANES + wd].T.astype(f32)
            for kt in range(4):
                kw = min(LANES, D - kt * LANES)
                wt32_s[kt, c * LANES:c * LANES + wd, 0:kw] = blk[:, kt * LANES:kt * LANES + kw]

    def prep_wqkv_perm():
        done = []
        for sec in range(3):
            for d in range(DH):
                r0 = sec * D + d * H
                tok = None
                for kt in range(4):
                    kw = min(LANES, D - kt * LANES)
                    rows = wt32_s[kt, pl.ds(sec * D + d, H, stride=DH), :]
                    wqkvt_s[r0:r0 + H, kt * LANES:kt * LANES + kw] = rows[:, 0:kw].astype(bf16)
                    if kt < 3:
                        t = pltpu.bitcast(rows[8:16], u32)
                        tok = t if tok is None else tok | t
                done.append(tok)
        return done

    def prep_wo():
        for nt in range(4):
            nw = min(LANES, D - nt * LANES)
            wo32_s[nt, :, 0:nw] = wo_s[:, nt * LANES:nt * LANES + nw].astype(f32)
        done = []
        for nt in range(4):
            nw = min(LANES, D - nt * LANES)
            rows = [wo32_s[nt, pl.ds(d, H, stride=DH), :][:, 0:nw].astype(bf16) for d in range(DH)]
            blk = jnp.concatenate(rows, axis=0)
            bt = blk.T
            wot_s[nt * LANES:nt * LANES + nw, :] = bt
            w = pltpu.bitcast(bt, u32)
            done += [w[nw // 2 - 8:nw // 2, k * LANES:(k + 1) * LANES] for k in range(3)]
        return done

    def ln_piece(p, tokens, cols=tuple(range(CPC))):
        xp, xnp, hp = x_s.at[p], xn_s.at[p], h_s.at[p]
        z = xp[0:8, 0:LANES].astype(f32)
        pace = _Pacer(tokens, 2 * NLB * CPC, z + 1.0 < z)
        for j in cols:
            col = pl.ds(j * LANES, LANES)
            m, r, rr = _ln_stats(xp, col, pace)
            for i in range(NLB):
                rows = slice(i * LNB, (i + 1) * LNB)
                xc = xp[rows, col].astype(f32) - _rep(pace(m), LNB)
                xnp[rows, col] = (xc * r).astype(bf16)
                hp[rows, col] = (xc * rr).astype(bf16)

    def mix1(p, mode, n_lo=0, n_hi=F, due=None, never=None):
        tokens = []
        nb = D // 16
        for n in range(n_lo // NB, n_hi // NB):
            ns = slice(n * NB, (n + 1) * NB)
            lhs = h_s[p] if due is None else _deadline(h_s[p], due[n * nb:(n + 1) * nb], never)
            part = jnp.dot(lhs, w1_s[p, :, ns], preferred_element_type=f32)
            tokens += [part[r:r + 8, 0:LANES] for r in range(0, D, 8)]
            if mode == "first":
                acc_s[:, ns] = part
            else:
                acc_s[:, ns] += part
        return tokens if due is not None else tokens[:len(tokens) * 7 // 8]

    zeros = jnp.zeros((D, LANES), f32)
    qkv_s[0, D:2 * D, :] = zeros
    qkv_s[0, 2 * D:3 * D, :] = zeros
    rk_s[0] = zeros
    rv_s[0] = zeros

    for j in range(CPC):
        _scope("wx0", lambda: x0_cp(j).wait())
        ln_piece(0, [], (j,))
    for rects, xc in RAMP:
        def waits():
            for r in rects:
                rect_cp(r).wait()
            if xc is not None:
                x_cp(xc).wait()
        _scope("wr", waits)
        tokens = []
        for p, lo, hi in rects:
            tokens += mix1(p, "first" if p == 0 else "mid", lo, hi)
        if xc is not None:
            ln_piece(xc, tokens)

    def mid_step(p, carry):
        _scope("wl", lambda: (w1_cp(p).wait(), x_cp(p + 1).wait()))
        ln_piece(p + 1, mix1(p, "mid"))
        return carry + 1

    steps = jax.lax.fori_loop(2, NC - 1, mid_step, 0)

    def waits():
        wqkv_cp.wait()
        wo_cp.wait()
        b1_cp.wait()
        b2_cp.wait()
        w1_cp(NC - 1).wait()
    _scope("wlast", waits)
    def qkv(c, due=None, never=None):
        rhs = xn_s[c] if due is None else _deadline(xn_s[c], due, never)
        r = jnp.dot(wqkvt_s[...], rhs, preferred_element_type=f32)
        for j in range(TC // LANES):
            qkv_s[c * (TC // LANES) + j + 1] = r[:, j * LANES:(j + 1) * LANES]
        return _tokens(r)

    scale = DH ** -0.5

    def attn_col(jj, pace):
        lane = jax.lax.broadcasted_iota(jnp.int32, (SLAB, LANES), 1)
        m0 = [None] + [lane < LANES - 2 * a for a in range(1, 4)]
        m1 = [(lane >= 8) & (lane < LANES - 2 * a) for a in range(4)]
        nd = SLAB // H
        acc = [[None, None] for _ in range(4)]
        for sl in range(D // SLAB):
            r0 = sl * SLAB
            q = qkv_s[jj + 1, r0:r0 + SLAB, :]
            k = qkv_s[jj + 1, D + r0:D + r0 + SLAB, :]
            q, k = pace.gate(q, k)
            kp = qkv_s[jj, D + r0:D + r0 + SLAB, :]
            rkp = rk_s[jj % 2, r0:r0 + SLAB, :]
            rk = pltpu.roll(k, 8, 1)
            rk_s[(jj + 1) % 2, r0:r0 + SLAB, :] = rk
            for a in range(4):
                rq = q if a == 0 else pltpu.roll(q, LANES - 2 * a, 1)
                for b in range(2):
                    if b == 0:
                        mix = k if a == 0 else jnp.where(m0[a], k, kp)
                    else:
                        mix = jnp.where(m1[a], rk, rkp)
                    p = rq * mix
                    for i in range(nd):
                        pi = p[i * H:(i + 1) * H]
                        acc[a][b] = pi if acc[a][b] is None else acc[a][b] + pi
        lane16 = jax.lax.broadcasted_iota(jnp.int32, (H, LANES), 1)
        logit = []
        for w in range(W):
            a, b = w % 4, w // 4
            lw = acc[a][b] if a == 0 else pltpu.roll(acc[a][b], 2 * a, 1)
            lw = lw * scale
            if jj == 0 and w > 0:
                lw = jnp.where(lane16 >= 2 * w, lw, -1e9)
            logit.append(lw)
        mx = functools.reduce(jnp.maximum, logit)
        ex = [jnp.exp(l - mx) for l in logit]
        inv = 1.0 / functools.reduce(jnp.add, ex)
        ra = [[None, None] for _ in range(4)]
        for w in range(W):
            a, b = w % 4, w // 4
            aw = ex[w] * inv
            aw = aw if a == 0 else pltpu.roll(aw, LANES - 2 * a, 1)
            ra[a][b] = jnp.concatenate([aw] * nd, axis=0)
        for sl in range(D // SLAB):
            r0 = sl * SLAB
            v = qkv_s[jj + 1, 2 * D + r0:2 * D + r0 + SLAB, :]
            v, = pace.gate(v)
            vp = qkv_s[jj, 2 * D + r0:2 * D + r0 + SLAB, :]
            rvp = rv_s[jj % 2, r0:r0 + SLAB, :]
            rv = pltpu.roll(v, 8, 1)
            rv_s[(jj + 1) % 2, r0:r0 + SLAB, :] = rv
            o = None
            for a in range(4):
                mix0 = v if a == 0 else jnp.where(m0[a], v, vp)
                mix1 = jnp.where(m1[a], rv, rvp)
                t = ra[a][0] * mix0 + ra[a][1] * mix1
                o = t if a == 0 else o + pltpu.roll(t, 2 * a, 1)
            o_s[r0:r0 + SLAB, jj * LANES:(jj + 1) * LANES] = o.astype(bf16)

    def attn(c, tokens):
        z = b2f_s[0:8, :]
        pace = _Pacer(tokens, 2 * (D // SLAB) * CPC, z + 1.0 < z)
        for j in range(CPC):
            attn_col(c * CPC + j, pace)

    def gelu(tokens):
        z = b2f_s[0:8, :]
        pace = _Pacer(tokens, NLB * (F // LANES), z + 1.0 < z)
        for nn in range(F // LANES):
            col = pl.ds(nn * LANES, LANES)
            bias = jnp.broadcast_to(b1f_s[nn:nn + 1, :], (8, LANES))
            for i in range(NLB):
                rows = slice(i * LNB, (i + 1) * LNB)
                u_s[rows, col] = _gelu(acc_s[rows, col] + _rep(pace(bias), LNB)).astype(bf16)

    def gate_mm(i):
        cs = slice(OOFF[i], OOFF[i + 1])
        y, tokens = None, []
        for k0 in range(0, F, KB):
            ks = slice(k0, min(k0 + KB, F))
            part = jnp.dot(u_s[:, ks], w2_s[ks, cs], preferred_element_type=f32)
            tokens += _tokens(part) if k0 + KB <= F else _tokens(part[:, 0:LANES])
            y = part if y is None else y + part
        g = []
        for j in range(OUT_PIECES[i] // LANES):
            jj = OOFF[i] // LANES + j
            g.append(_silu(y[:, j * LANES:(j + 1) * LANES] + b2f_s[jj:jj + 1, :]))
        return g, tokens

    def final(i, g):
        cs = slice(OOFF[i], OOFF[i + 1])
        s = jnp.dot(wot_s[...], o_s[:, cs], preferred_element_type=f32)
        rows = TAIL_ROWS if i == NO - 1 else (0, D)
        for (r0, r1), cp in zip(zip(rows[:-1], rows[1:]), out_cps(i)):
            for j in range(OUT_PIECES[i] // LANES):
                jj = OOFF[i] // LANES + j
                xr = x_s[jj // CPC, r0:r1, pl.ds((jj % CPC) * LANES, LANES)].astype(f32)
                r = xr + s[r0:r1, j * LANES:(j + 1) * LANES] * g[j][r0:r1]
                out_s[r0:r1, pl.ds(jj * LANES, LANES)] = r.astype(bf16)
            cp.start()
        return _tokens(s)

    @pl.when(steps == NC - 3)
    def _():
        b1f_s[...] = b1_s[...].astype(f32)
        b2f_s[...] = b2_s[...].astype(f32)
        prep_wqkv_t()
        z = b2f_s[0:8, :]
        never = z + 1.0 < z
        nb = (F // NB) * (D // 16)
        last = mix1(NC - 1, "mid", due=_spread(prep_wqkv_perm(), nb, nb * 2 // 7, nb), never=never)
        wo_done = prep_wo()

        tokens = []
        for c in range(QKV_AHEAD):
            nb = D // 16
            due = _spread(wo_done, nb, 0, len(wo_done)) if c == 2 else [None] * nb
            tokens += qkv(c, due, never)
        gelu(last[len(last) // 2:] + tokens[:len(tokens) // 3])
        attn(0, tokens[len(tokens) // 3:len(tokens) * 14 // 15])

    _scope("ww2", lambda: w2_cp.wait())
    tokens = []
    for c in range(NC):
        g, t = gate_mm(c)
        tokens += t + final(c, g)
        if c + QKV_AHEAD < NC:
            tokens += qkv(c + QKV_AHEAD)
        if c + 1 < NC:
            attn(c + 1, tokens[c * ATTN_WIN:(c + 1) * ATTN_WIN])
    final(NC, gate_mm(NC)[0])

    def waits():
        for i in range(NO):
            for cp in out_cps(i):
                cp.wait()
    _scope("wout", waits)


@jax.jit
def pallas_recurrent_scan__sliding_local_dilated__mixer_token_mlp__prompt_kernel(
    A_x: jax.Array,
    A_wqkv: jax.Array,
    A_wo: jax.Array,
    B_x: jax.Array,
    B_w1: jax.Array,
    B_b1: jax.Array,
    B_w2: jax.Array,
    B_b2: jax.Array,
):
    del B_x
    xt = jnp.swapaxes(A_x, 1, 2)
    b1 = B_b1.reshape(F // LANES, LANES)
    b2 = B_b2.reshape(S // LANES, LANES)
    any_spec = pl.BlockSpec(memory_space=pl.ANY)
    out_t = pl.pallas_call(
        _kernel,
        out_shape=jax.ShapeDtypeStruct((1, D, S), bf16),
        in_specs=[any_spec] * 7,
        out_specs=any_spec,
        scratch_shapes=[
            pltpu.VMEM((NC, D, TC), bf16),
            pltpu.VMEM((D, 3 * D), bf16),
            pltpu.VMEM((D, D), bf16),
            pltpu.VMEM((NC, TC, F), bf16),
            pltpu.VMEM((F, S), bf16),
            pltpu.VMEM((F // LANES, LANES), bf16),
            pltpu.VMEM((S // LANES, LANES), bf16),
            pltpu.VMEM((NC, D // 2, TC), u32),
            pltpu.VMEM((NC, D // 2, TC), u32),
            pltpu.VMEM((D, F), f32),
            pltpu.VMEM((D // 2, F), u32),
            pltpu.VMEM((4, 11 * LANES, LANES), f32),
            pltpu.VMEM((3 * D // 2, D), u32),
            pltpu.VMEM((4, D, LANES), f32),
            pltpu.VMEM((D // 2, D), u32),
            pltpu.VMEM((NCOL + 1, 3 * D, LANES), f32),
            pltpu.VMEM((2, D, LANES), f32),
            pltpu.VMEM((2, D, LANES), f32),
            pltpu.VMEM((D // 2, S), u32),
            pltpu.VMEM((D, S), bf16),
            pltpu.VMEM((F // LANES, LANES), f32),
            pltpu.VMEM((S // LANES, LANES), f32),
            pltpu.SemaphoreType.DMA((NSEM,)),
        ],
        compiler_params=pltpu.CompilerParams(vmem_limit_bytes=100 * 1024 * 1024,
                                             disable_semaphore_checks=True,
                                             disable_bounds_checks=True),
        name="fused_mixer_attn",
    )(xt, A_wqkv, A_wo, B_w1, b1, B_w2, b2)
    return jnp.swapaxes(out_t, 1, 2)
```

```python
import functools

import jax
import jax.numpy as jnp
import jax.experimental.pallas as pl
import jax.experimental.pallas.tpu as pltpu

S = 2048
D = 448
H = 16
DH = D // H
F = 1792
W = 8
EPS = 1e-5
TC = 256
NC = S // TC
LANES = 128
NCOL = S // LANES
SLAB = 32

f32 = jnp.float32
bf16 = jnp.bfloat16
u32 = jnp.uint32

_SCOPES = False


def _scope(name, fn):
    if _SCOPES:
        with jax.named_scope(name):
            fn()
    else:
        fn()


LNB = 64
NLB = D // LNB


def _rep(v8, rows):
    return jnp.concatenate([v8] * (rows // 8), axis=0)


def _ln_stats(x_ref, col, pace):
    piv = jnp.broadcast_to(x_ref[0:1, col].astype(f32), (8, LANES))
    s1 = s2 = None
    for i in range(NLB):
        pv = _rep(pace(piv), LNB // 2)
        w = pltpu.bitcast(x_ref[i * LNB:(i + 1) * LNB, col], u32)
        for half in (w << 16, w & jnp.uint32(0xFFFF0000)):
            d = pltpu.bitcast(half, f32) - pv
            for k in range(LNB // 2 // 16):
                dk = d[k * 16:(k + 1) * 16]
                s1 = dk if s1 is None else s1 + dk
                s2 = dk * dk if s2 is None else s2 + dk * dk
    md = jnp.sum(s1, axis=0, keepdims=True) * (1.0 / D)
    v = jnp.maximum(jnp.sum(s2, axis=0, keepdims=True) * (1.0 / D) - md * md, 0.0)
    r = jax.lax.rsqrt(v + EPS)
    r2 = jax.lax.rsqrt(v * r * r + EPS)
    return piv + md, r, r * r2


def _tokens(r):
    return [r[i:i + 8, j:j + LANES] for j in range(0, r.shape[1], LANES) for i in range(0, r.shape[0], 8)]


def _deadline(lhs, toks, never):
    if not any(t is not None for t in toks):
        return lhs
    w = pltpu.bitcast(lhs, u32)
    blocks = [w[8 * i:8 * i + 8, 0:LANES] for i in range(w.shape[0] // 8)]
    blocks = [b if t is None else jnp.where(never, t, b) for b, t in zip(blocks, toks, strict=True)]
    w = jnp.concatenate([jnp.concatenate(blocks, axis=0), w[:, LANES:]], axis=1)
    return pltpu.bitcast(w, bf16)


def _spread(vals, nslots, lo, hi):
    out = [None] * nslots
    for i in range(lo, hi):
        out[i] = vals[((i - lo + 1) * len(vals)) // (hi - lo) - 1]
    return out


class _Pacer:
    def __init__(self, tokens, count, never):
        self.tokens, self.count, self.never, self.i = tokens, count, never, 0

    def __call__(self, v8):
        if not self.tokens:
            return v8
        tok = self.tokens[self.i * len(self.tokens) // self.count]
        self.i += 1
        return jnp.where(self.never, tok, v8)

    def gate(self, *vs, after=()):
        if not self.tokens:
            return vs
        tok = self.tokens[self.i * len(self.tokens) // self.count]
        self.i += 1
        for a in after:
            tok = jnp.maximum(tok, a)
        n = vs[0].shape[0]
        nv, tk = _rep(self.never, n), _rep(tok, n)
        return tuple(jnp.where(nv, tk, v) for v in vs)


def _gelu(x):
    c = 0.7978845608028654
    t = jnp.tanh(x * (c + (c * 0.044715) * (x * x)))
    hx = 0.5 * x
    return hx + hx * t


def _silu(y):
    hy = 0.5 * y
    return hy + hy * jnp.tanh(hy)


RAMP = (
    (((0, 0, 256),), None),
    (((0, 256, 768),), None),
    (((0, 768, 1280),), 1),
    (((0, 1280, F), (1, 0, 512)), None),
    (((1, 512, F),), 2),
)
RECTS = tuple(r for rects, _ in RAMP for r in rects)
NB = 256
ATTN_WIN = 740
KB = 512
CPC = TC // LANES
QKV_AHEAD = 3
OUT_PIECES = (256,) * 7 + (128, 128)
OOFF = tuple(sum(OUT_PIECES[:i]) for i in range(len(OUT_PIECES) + 1))
NO = len(OUT_PIECES)
TAIL_ROWS = (0, 256, 384, D)
SEM_X, SEM_W1, SEM_MISC, SEM_OUT = 0, NC, 2 * NC, 2 * NC + 6
SEM_RAMP = SEM_OUT + NO + len(TAIL_ROWS) - 2
NSEM = SEM_RAMP + len(RECTS)


def _kernel(x_hbm, wqkv_hbm, wo_hbm, w1_hbm, b1_hbm, w2_hbm, b2_hbm, out_hbm,
            x_s, wqkv_s, wo_s, w1_s, w2_s, b1_s, b2_s,
            xn_s, h_s, acc_s, u_s, wt32_s, wqkvt_s, wo32_s, wot_s,
            qkv_s, rk_s, rv_s, o_s, out_s, b1f_s, b2f_s, sem):
    xn_s, h_s, u_s, wqkvt_s, wot_s, o_s = (
        r.bitcast(bf16) for r in (xn_s, h_s, u_s, wqkvt_s, wot_s, o_s))

    def x_cp(p):
        return pltpu.make_async_copy(x_hbm.at[0, :, pl.ds(p * TC, TC)], x_s.at[p], sem.at[SEM_X + p])

    def w1_cp(p):
        return pltpu.make_async_copy(w1_hbm.at[pl.ds(p * TC, TC), :], w1_s.at[p], sem.at[SEM_W1 + p])

    def rect_cp(r):
        p, lo, hi = r
        return pltpu.make_async_copy(w1_hbm.at[p * TC:(p + 1) * TC, lo:hi], w1_s.at[p, :, lo:hi],
                                     sem.at[SEM_RAMP + RECTS.index(r)])

    def out_cps(i):
        sl = slice(OOFF[i], OOFF[i + 1])
        rows = TAIL_ROWS if i == NO - 1 else (0, D)
        return [pltpu.make_async_copy(out_s.at[r0:r1, sl], out_hbm.at[0, r0:r1, sl], sem.at[SEM_OUT + i + k])
                for k, (r0, r1) in enumerate(zip(rows[:-1], rows[1:]))]

    def x0_cp(j):
        sl = pl.ds(j * LANES, LANES)
        return pltpu.make_async_copy(x_hbm.at[0, :, sl], x_s.at[0, :, sl],
                                     sem.at[SEM_X if j == 0 else SEM_MISC + 5])

    wqkv_cp = pltpu.make_async_copy(wqkv_hbm, wqkv_s, sem.at[SEM_MISC + 0])
    wo_cp = pltpu.make_async_copy(wo_hbm, wo_s, sem.at[SEM_MISC + 1])
    b1_cp = pltpu.make_async_copy(b1_hbm, b1_s, sem.at[SEM_MISC + 2])
    b2_cp = pltpu.make_async_copy(b2_hbm, b2_s, sem.at[SEM_MISC + 3])
    w2_cp = pltpu.make_async_copy(w2_hbm, w2_s, sem.at[SEM_MISC + 4])

    x0_cp(0).start()
    x0_cp(1).start()
    for rects, xc in RAMP:
        for r in rects:
            rect_cp(r).start()
        if xc is not None:
            x_cp(xc).start()
    for p in range(2, NC):
        if p == NC - 1:
            wqkv_cp.start()
            wo_cp.start()
            b1_cp.start()
            b2_cp.start()
        w1_cp(p).start()
        if p + 1 < NC:
            x_cp(p + 1).start()
    w2_cp.start()

    def prep_wqkv_t():
        for c in range(11):
            wd = min(LANES, 3 * D - c * LANES)
            blk = wqkv_s[:, c * LANES:c * LANES + wd].T.astype(f32)
            for kt in range(4):
                kw = min(LANES, D - kt * LANES)
                wt32_s[kt, c * LANES:c * LANES + wd, 0:kw] = blk[:, kt * LANES:kt * LANES + kw]

    def prep_wqkv_perm():
        done = []
        for sec in range(3):
            for d in range(DH):
                r0 = sec * D + d * H
                tok = None
                for kt in range(4):
                    kw = min(LANES, D - kt * LANES)
                    rows = wt32_s[kt, pl.ds(sec * D + d, H, stride=DH), :]
                    wqkvt_s[r0:r0 + H, kt * LANES:kt * LANES + kw] = rows[:, 0:kw].astype(bf16)
                    if kt < 3:
                        t = pltpu.bitcast(rows[8:16], u32)
                        tok = t if tok is None else tok | t
                done.append(tok)
        return done

    def prep_wo():
        for nt in range(4):
            nw = min(LANES, D - nt * LANES)
            wo32_s[nt, :, 0:nw] = wo_s[:, nt * LANES:nt * LANES + nw].astype(f32)
        done = []
        for nt in range(4):
            nw = min(LANES, D - nt * LANES)
            rows = [wo32_s[nt, pl.ds(d, H, stride=DH), :][:, 0:nw].astype(bf16) for d in range(DH)]
            blk = jnp.concatenate(rows, axis=0)
            bt = blk.T
            wot_s[nt * LANES:nt * LANES + nw, :] = bt
            w = pltpu.bitcast(bt, u32)
            done += [w[nw // 2 - 8:nw // 2, k * LANES:(k + 1) * LANES] for k in range(3)]
        return done

    def ln_piece(p, tokens, cols=tuple(range(CPC))):
        xp, xnp, hp = x_s.at[p], xn_s.at[p], h_s.at[p]
        z = xp[0:8, 0:LANES].astype(f32)
        pace = _Pacer(tokens, 2 * NLB * CPC, z + 1.0 < z)
        for j in cols:
            col = pl.ds(j * LANES, LANES)
            m, r, rr = _ln_stats(xp, col, pace)
            for i in range(NLB):
                rows = slice(i * LNB, (i + 1) * LNB)
                xc = xp[rows, col].astype(f32) - _rep(pace(m), LNB)
                xnp[rows, col] = (xc * r).astype(bf16)
                hp[rows, col] = (xc * rr).astype(bf16)

    def mix1(p, mode, n_lo=0, n_hi=F, due=None, never=None):
        tokens = []
        nb = D // 16
        for n in range(n_lo // NB, n_hi // NB):
            ns = slice(n * NB, (n + 1) * NB)
            lhs = h_s[p] if due is None else _deadline(h_s[p], due[n * nb:(n + 1) * nb], never)
            part = jnp.dot(lhs, w1_s[p, :, ns], preferred_element_type=f32)
            tokens += [part[r:r + 8, 0:LANES] for r in range(0, D, 8)]
            if mode == "first":
                acc_s[:, ns] = part
            else:
                acc_s[:, ns] += part
        return tokens if due is not None else tokens[:len(tokens) * 7 // 8]

    zeros = jnp.zeros((D, LANES), f32)
    qkv_s[0, D:2 * D, :] = zeros
    qkv_s[0, 2 * D:3 * D, :] = zeros
    rk_s[0] = zeros
    rv_s[0] = zeros

    for j in range(CPC):
        _scope("wx0", lambda: x0_cp(j).wait())
        ln_piece(0, [], (j,))
    for rects, xc in RAMP:
        def waits():
            for r in rects:
                rect_cp(r).wait()
            if xc is not None:
                x_cp(xc).wait()
        _scope("wr", waits)
        tokens = []
        for p, lo, hi in rects:
            tokens += mix1(p, "first" if p == 0 else "mid", lo, hi)
        if xc is not None:
            ln_piece(xc, tokens)

    def mid_step(p, carry):
        _scope("wl", lambda: (w1_cp(p).wait(), x_cp(p + 1).wait()))
        ln_piece(p + 1, mix1(p, "mid"))
        return carry + 1

    steps = jax.lax.fori_loop(2, NC - 1, mid_step, 0)

    def waits():
        wqkv_cp.wait()
        wo_cp.wait()
        b1_cp.wait()
        b2_cp.wait()
        w1_cp(NC - 1).wait()
    _scope("wlast", waits)
    def qkv(c, due=None, never=None):
        rhs = xn_s[c] if due is None else _deadline(xn_s[c], due, never)
        r = jnp.dot(wqkvt_s[...], rhs, preferred_element_type=f32)
        for j in range(TC // LANES):
            qkv_s[c * (TC // LANES) + j + 1] = r[:, j * LANES:(j + 1) * LANES]
        return _tokens(r)

    scale = DH ** -0.5

    def attn_col(jj, pace):
        lane = jax.lax.broadcasted_iota(jnp.int32, (SLAB, LANES), 1)
        m0 = [None] + [lane < LANES - 2 * a for a in range(1, 4)]
        m1 = [(lane >= 8) & (lane < LANES - 2 * a) for a in range(4)]
        nd = SLAB // H
        acc = [[None, None] for _ in range(4)]
        hist = [(), ()]
        for sl in range(D // SLAB):
            r0 = sl * SLAB
            q = qkv_s[jj + 1, r0:r0 + SLAB, :]
            k = qkv_s[jj + 1, D + r0:D + r0 + SLAB, :]
            q, k = pace.gate(q, k, after=hist[-2])
            kp = qkv_s[jj, D + r0:D + r0 + SLAB, :]
            rkp = rk_s[jj % 2, r0:r0 + SLAB, :]
            rk = pltpu.roll(k, 8, 1)
            rk_s[(jj + 1) % 2, r0:r0 + SLAB, :] = rk
            for a in range(4):
                rq = q if a == 0 else pltpu.roll(q, LANES - 2 * a, 1)
                for b in range(2):
                    if b == 0:
                        mix = k if a == 0 else jnp.where(m0[a], k, kp)
                    else:
                        mix = jnp.where(m1[a], rk, rkp)
                    p = rq * mix
                    for i in range(nd):
                        pi = p[i * H:(i + 1) * H]
                        acc[a][b] = pi if acc[a][b] is None else acc[a][b] + pi
            hist.append(tuple(acc[a][b][h:h + 8] for a in range(4) for b in range(2) for h in (0, 8)))
        lane16 = jax.lax.broadcasted_iota(jnp.int32, (H, LANES), 1)
        logit = []
        for w in range(W):
            a, b = w % 4, w // 4
            lw = acc[a][b] if a == 0 else pltpu.roll(acc[a][b], 2 * a, 1)
            lw = lw * scale
            if jj == 0 and w > 0:
                lw = jnp.where(lane16 >= 2 * w, lw, -1e9)
            logit.append(lw)
        mx = functools.reduce(jnp.maximum, logit)
        ex = [jnp.exp(l - mx) for l in logit]
        inv = 1.0 / functools.reduce(jnp.add, ex)
        ra = [[None, None] for _ in range(4)]
        for w in range(W):
            a, b = w % 4, w // 4
            aw = ex[w] * inv
            aw = aw if a == 0 else pltpu.roll(aw, LANES - 2 * a, 1)
            ra[a][b] = jnp.concatenate([aw] * nd, axis=0)
        for sl in range(D // SLAB):
            r0 = sl * SLAB
            v = qkv_s[jj + 1, 2 * D + r0:2 * D + r0 + SLAB, :]
            v, = pace.gate(v)
            vp = qkv_s[jj, 2 * D + r0:2 * D + r0 + SLAB, :]
            rvp = rv_s[jj % 2, r0:r0 + SLAB, :]
            rv = pltpu.roll(v, 8, 1)
            rv_s[(jj + 1) % 2, r0:r0 + SLAB, :] = rv
            o = None
            for a in range(4):
                mix0 = v if a == 0 else jnp.where(m0[a], v, vp)
                mix1 = jnp.where(m1[a], rv, rvp)
                t = ra[a][0] * mix0 + ra[a][1] * mix1
                o = t if a == 0 else o + pltpu.roll(t, 2 * a, 1)
            o_s[r0:r0 + SLAB, jj * LANES:(jj + 1) * LANES] = o.astype(bf16)

    def attn(c, tokens):
        z = b2f_s[0:8, :]
        pace = _Pacer(tokens, 2 * (D // SLAB) * CPC, z + 1.0 < z)
        for j in range(CPC):
            attn_col(c * CPC + j, pace)

    def gelu(tokens):
        z = b2f_s[0:8, :]
        pace = _Pacer(tokens, NLB * (F // LANES), z + 1.0 < z)
        for nn in range(F // LANES):
            col = pl.ds(nn * LANES, LANES)
            bias = jnp.broadcast_to(b1f_s[nn:nn + 1, :], (8, LANES))
            for i in range(NLB):
                rows = slice(i * LNB, (i + 1) * LNB)
                u_s[rows, col] = _gelu(acc_s[rows, col] + _rep(pace(bias), LNB)).astype(bf16)

    def gate_mm(i):
        cs = slice(OOFF[i], OOFF[i + 1])
        y, tokens = None, []
        for k0 in range(0, F, KB):
            ks = slice(k0, min(k0 + KB, F))
            part = jnp.dot(u_s[:, ks], w2_s[ks, cs], preferred_element_type=f32)
            tokens += _tokens(part) if k0 + KB <= F else _tokens(part[:, 0:LANES])
            y = part if y is None else y + part
        g = []
        for j in range(OUT_PIECES[i] // LANES):
            jj = OOFF[i] // LANES + j
            g.append(_silu(y[:, j * LANES:(j + 1) * LANES] + b2f_s[jj:jj + 1, :]))
        return g, tokens

    def final(i, g):
        cs = slice(OOFF[i], OOFF[i + 1])
        s = jnp.dot(wot_s[...], o_s[:, cs], preferred_element_type=f32)
        rows = TAIL_ROWS if i == NO - 1 else (0, D)
        for (r0, r1), cp in zip(zip(rows[:-1], rows[1:]), out_cps(i)):
            for j in range(OUT_PIECES[i] // LANES):
                jj = OOFF[i] // LANES + j
                xr = x_s[jj // CPC, r0:r1, pl.ds((jj % CPC) * LANES, LANES)].astype(f32)
                r = xr + s[r0:r1, j * LANES:(j + 1) * LANES] * g[j][r0:r1]
                out_s[r0:r1, pl.ds(jj * LANES, LANES)] = r.astype(bf16)
            cp.start()
        return _tokens(s)

    @pl.when(steps == NC - 3)
    def _():
        b1f_s[...] = b1_s[...].astype(f32)
        b2f_s[...] = b2_s[...].astype(f32)
        prep_wqkv_t()
        z = b2f_s[0:8, :]
        never = z + 1.0 < z
        nb = (F // NB) * (D // 16)
        last = mix1(NC - 1, "mid", due=_spread(prep_wqkv_perm(), nb, nb * 2 // 7, nb), never=never)
        wo_done = prep_wo()

        tokens = []
        for c in range(QKV_AHEAD):
            nb = D // 16
            due = _spread(wo_done, nb, 0, len(wo_done)) if c == 2 else [None] * nb
            tokens += qkv(c, due, never)
        gelu(last[len(last) // 2:] + tokens[:len(tokens) // 3])
        attn(0, tokens[len(tokens) // 3:len(tokens) * 9 // 10])

    _scope("ww2", lambda: w2_cp.wait())
    tokens = []
    for c in range(NC):
        if c + QKV_AHEAD < NC:
            tokens += qkv(c + QKV_AHEAD)
        g, t = gate_mm(c)
        tokens += t + final(c, g)
        if c + 1 < NC:
            attn(c + 1, tokens[c * ATTN_WIN:(c + 1) * ATTN_WIN])
    final(NC, gate_mm(NC)[0])

    def waits():
        for i in range(NO):
            for cp in out_cps(i):
                cp.wait()
    _scope("wout", waits)


@jax.jit
def pallas_recurrent_scan__sliding_local_dilated__mixer_token_mlp__prompt_kernel(
    A_x: jax.Array,
    A_wqkv: jax.Array,
    A_wo: jax.Array,
    B_x: jax.Array,
    B_w1: jax.Array,
    B_b1: jax.Array,
    B_w2: jax.Array,
    B_b2: jax.Array,
):
    del B_x
    xt = jnp.swapaxes(A_x, 1, 2)
    b1 = B_b1.reshape(F // LANES, LANES)
    b2 = B_b2.reshape(S // LANES, LANES)
    any_spec = pl.BlockSpec(memory_space=pl.ANY)
    out_t = pl.pallas_call(
        _kernel,
        out_shape=jax.ShapeDtypeStruct((1, D, S), bf16),
        in_specs=[any_spec] * 7,
        out_specs=any_spec,
        scratch_shapes=[
            pltpu.VMEM((NC, D, TC), bf16),
            pltpu.VMEM((D, 3 * D), bf16),
            pltpu.VMEM((D, D), bf16),
            pltpu.VMEM((NC, TC, F), bf16),
            pltpu.VMEM((F, S), bf16),
            pltpu.VMEM((F // LANES, LANES), bf16),
            pltpu.VMEM((S // LANES, LANES), bf16),
            pltpu.VMEM((NC, D // 2, TC), u32),
            pltpu.VMEM((NC, D // 2, TC), u32),
            pltpu.VMEM((D, F), f32),
            pltpu.VMEM((D // 2, F), u32),
            pltpu.VMEM((4, 11 * LANES, LANES), f32),
            pltpu.VMEM((3 * D // 2, D), u32),
            pltpu.VMEM((4, D, LANES), f32),
            pltpu.VMEM((D // 2, D), u32),
            pltpu.VMEM((NCOL + 1, 3 * D, LANES), f32),
            pltpu.VMEM((2, D, LANES), f32),
            pltpu.VMEM((2, D, LANES), f32),
            pltpu.VMEM((D // 2, S), u32),
            pltpu.VMEM((D, S), bf16),
            pltpu.VMEM((F // LANES, LANES), f32),
            pltpu.VMEM((S // LANES, LANES), f32),
            pltpu.SemaphoreType.DMA((NSEM,)),
        ],
        compiler_params=pltpu.CompilerParams(vmem_limit_bytes=100 * 1024 * 1024,
                                             disable_semaphore_checks=True,
                                             disable_bounds_checks=True),
        name="fused_mixer_attn",
    )(xt, A_wqkv, A_wo, B_w1, b1, B_w2, b2)
    return jnp.swapaxes(out_t, 1, 2)
```

```python
import functools

import jax
import jax.numpy as jnp
import jax.experimental.pallas as pl
import jax.experimental.pallas.tpu as pltpu

S = 2048
D = 448
H = 16
DH = D // H
F = 1792
W = 8
EPS = 1e-5
TC = 256
NC = S // TC
LANES = 128
NCOL = S // LANES
SLAB = 32

f32 = jnp.float32
bf16 = jnp.bfloat16
u32 = jnp.uint32

_SCOPES = False


def _scope(name, fn):
    if _SCOPES:
        with jax.named_scope(name):
            fn()
    else:
        fn()


LNB = 64
NLB = D // LNB


def _rep(v8, rows):
    return jnp.concatenate([v8] * (rows // 8), axis=0)


def _ln_stats(x_ref, col, pace):
    piv = jnp.broadcast_to(x_ref[0:1, col].astype(f32), (8, LANES))
    s1 = s2 = None
    for i in range(NLB):
        pv = _rep(pace(piv), LNB // 2)
        w = pltpu.bitcast(x_ref[i * LNB:(i + 1) * LNB, col], u32)
        for half in (w << 16, w & jnp.uint32(0xFFFF0000)):
            d = pltpu.bitcast(half, f32) - pv
            for k in range(LNB // 2 // 16):
                dk = d[k * 16:(k + 1) * 16]
                s1 = dk if s1 is None else s1 + dk
                s2 = dk * dk if s2 is None else s2 + dk * dk
    md = jnp.sum(s1, axis=0, keepdims=True) * (1.0 / D)
    v = jnp.maximum(jnp.sum(s2, axis=0, keepdims=True) * (1.0 / D) - md * md, 0.0)
    r = jax.lax.rsqrt(v + EPS)
    r2 = jax.lax.rsqrt(v * r * r + EPS)
    return piv + md, r, r * r2


def _tokens(r):
    return [r[i:i + 8, j:j + LANES] for j in range(0, r.shape[1], LANES) for i in range(0, r.shape[0], 8)]


def _deadline(lhs, toks, never):
    if not any(t is not None for t in toks):
        return lhs
    w = pltpu.bitcast(lhs, u32)
    blocks = [w[8 * i:8 * i + 8, 0:LANES] for i in range(w.shape[0] // 8)]
    blocks = [b if t is None else jnp.where(never, t, b) for b, t in zip(blocks, toks, strict=True)]
    w = jnp.concatenate([jnp.concatenate(blocks, axis=0), w[:, LANES:]], axis=1)
    return pltpu.bitcast(w, bf16)


def _spread(vals, nslots, lo, hi):
    out = [None] * nslots
    for i in range(lo, hi):
        out[i] = vals[((i - lo + 1) * len(vals)) // (hi - lo) - 1]
    return out


class _Pacer:
    def __init__(self, tokens, count, never):
        self.tokens, self.count, self.never, self.i = tokens, count, never, 0

    def __call__(self, v8):
        if not self.tokens:
            return v8
        tok = self.tokens[self.i * len(self.tokens) // self.count]
        self.i += 1
        return jnp.where(self.never, tok, v8)

    def gate(self, *vs, after=()):
        if not self.tokens:
            return vs
        tok = self.tokens[self.i * len(self.tokens) // self.count]
        self.i += 1
        for a in after:
            tok = jnp.maximum(tok, a)
        n = vs[0].shape[0]
        nv, tk = _rep(self.never, n), _rep(tok, n)
        return tuple(jnp.where(nv, tk, v) for v in vs)


def _gelu(x):
    c = 0.7978845608028654
    t = jnp.tanh(x * (c + (c * 0.044715) * (x * x)))
    hx = 0.5 * x
    return hx + hx * t


def _silu(y):
    hy = 0.5 * y
    return hy + hy * jnp.tanh(hy)


RAMP = (
    (((0, 0, 256),), None),
    (((0, 256, 768),), None),
    (((0, 768, 1280),), 1),
    (((0, 1280, F), (1, 0, 512)), None),
    (((1, 512, F),), 2),
)
RECTS = tuple(r for rects, _ in RAMP for r in rects)
NB = 256
ATTN_WIN = 740
KB = 512
CPC = TC // LANES
QKV_AHEAD = 3
OUT_PIECES = (256,) * 7 + (128, 128)
OOFF = tuple(sum(OUT_PIECES[:i]) for i in range(len(OUT_PIECES) + 1))
NO = len(OUT_PIECES)
TAIL_ROWS = (0, 256, 384, D)
SEM_X, SEM_W1, SEM_MISC, SEM_OUT = 0, NC, 2 * NC, 2 * NC + 6
SEM_RAMP = SEM_OUT + NO + len(TAIL_ROWS) - 2
NSEM = SEM_RAMP + len(RECTS)


def _kernel(x_hbm, wqkv_hbm, wo_hbm, w1_hbm, b1_hbm, w2_hbm, b2_hbm, out_hbm,
            x_s, wqkv_s, wo_s, w1_s, w2_s, b1_s, b2_s,
            xn_s, h_s, acc_s, u_s, wt32_s, wqkvt_s, wo32_s, wot_s,
            qkv_s, rk_s, rv_s, o_s, out_s, b1f_s, b2f_s, sem):
    xn_s, h_s, u_s, wqkvt_s, wot_s, o_s = (
        r.bitcast(bf16) for r in (xn_s, h_s, u_s, wqkvt_s, wot_s, o_s))

    def x_cp(p):
        return pltpu.make_async_copy(x_hbm.at[0, :, pl.ds(p * TC, TC)], x_s.at[p], sem.at[SEM_X + p])

    def w1_cp(p):
        return pltpu.make_async_copy(w1_hbm.at[pl.ds(p * TC, TC), :], w1_s.at[p], sem.at[SEM_W1 + p])

    def rect_cp(r):
        p, lo, hi = r
        return pltpu.make_async_copy(w1_hbm.at[p * TC:(p + 1) * TC, lo:hi], w1_s.at[p, :, lo:hi],
                                     sem.at[SEM_RAMP + RECTS.index(r)])

    def out_cps(i):
        sl = slice(OOFF[i], OOFF[i + 1])
        rows = TAIL_ROWS if i == NO - 1 else (0, D)
        return [pltpu.make_async_copy(out_s.at[r0:r1, sl], out_hbm.at[0, r0:r1, sl], sem.at[SEM_OUT + i + k])
                for k, (r0, r1) in enumerate(zip(rows[:-1], rows[1:]))]

    def x0_cp(j):
        sl = pl.ds(j * LANES, LANES)
        return pltpu.make_async_copy(x_hbm.at[0, :, sl], x_s.at[0, :, sl],
                                     sem.at[SEM_X if j == 0 else SEM_MISC + 5])

    wqkv_cp = pltpu.make_async_copy(wqkv_hbm, wqkv_s, sem.at[SEM_MISC + 0])
    wo_cp = pltpu.make_async_copy(wo_hbm, wo_s, sem.at[SEM_MISC + 1])
    b1_cp = pltpu.make_async_copy(b1_hbm, b1_s, sem.at[SEM_MISC + 2])
    b2_cp = pltpu.make_async_copy(b2_hbm, b2_s, sem.at[SEM_MISC + 3])
    w2_cp = pltpu.make_async_copy(w2_hbm, w2_s, sem.at[SEM_MISC + 4])

    x0_cp(0).start()
    x0_cp(1).start()
    for rects, xc in RAMP:
        for r in rects:
            rect_cp(r).start()
        if xc is not None:
            x_cp(xc).start()
    for p in range(2, NC):
        if p == NC - 1:
            wqkv_cp.start()
            wo_cp.start()
            b1_cp.start()
            b2_cp.start()
        w1_cp(p).start()
        if p + 1 < NC:
            x_cp(p + 1).start()
    w2_cp.start()

    def prep_wqkv_t():
        for c in range(11):
            wd = min(LANES, 3 * D - c * LANES)
            blk = wqkv_s[:, c * LANES:c * LANES + wd].T.astype(f32)
            for kt in range(4):
                kw = min(LANES, D - kt * LANES)
                wt32_s[kt, c * LANES:c * LANES + wd, 0:kw] = blk[:, kt * LANES:kt * LANES + kw]

    def prep_wqkv_perm():
        done = []
        for sec in range(3):
            for d in range(DH):
                r0 = sec * D + d * H
                tok = None
                for kt in range(4):
                    kw = min(LANES, D - kt * LANES)
                    rows = wt32_s[kt, pl.ds(sec * D + d, H, stride=DH), :]
                    wqkvt_s[r0:r0 + H, kt * LANES:kt * LANES + kw] = rows[:, 0:kw].astype(bf16)
                    if kt < 3:
                        t = pltpu.bitcast(rows[8:16], u32)
                        tok = t if tok is None else tok | t
                done.append(tok)
        return done

    def prep_wo():
        for nt in range(4):
            nw = min(LANES, D - nt * LANES)
            wo32_s[nt, :, 0:nw] = wo_s[:, nt * LANES:nt * LANES + nw].astype(f32)
        for nt in range(4):
            nw = min(LANES, D - nt * LANES)
            rows = [wo32_s[nt, pl.ds(d, H, stride=DH), :][:, 0:nw].astype(bf16) for d in range(DH)]
            blk = jnp.concatenate(rows, axis=0)
            wot_s[nt * LANES:nt * LANES + nw, :] = blk.T

    def ln_piece(p, tokens, cols=tuple(range(CPC))):
        xp, xnp, hp = x_s.at[p], xn_s.at[p], h_s.at[p]
        z = xp[0:8, 0:LANES].astype(f32)
        pace = _Pacer(tokens, 2 * NLB * CPC, z + 1.0 < z)
        for j in cols:
            col = pl.ds(j * LANES, LANES)
            m, r, rr = _ln_stats(xp, col, pace)
            for i in range(NLB):
                rows = slice(i * LNB, (i + 1) * LNB)
                xc = xp[rows, col].astype(f32) - _rep(pace(m), LNB)
                xnp[rows, col] = (xc * r).astype(bf16)
                hp[rows, col] = (xc * rr).astype(bf16)

    def mix1(p, mode, n_lo=0, n_hi=F, due=None, never=None):
        tokens = []
        nb = D // 16
        for n in range(n_lo // NB, n_hi // NB):
            ns = slice(n * NB, (n + 1) * NB)
            lhs = h_s[p] if due is None else _deadline(h_s[p], due[n * nb:(n + 1) * nb], never)
            part = jnp.dot(lhs, w1_s[p, :, ns], preferred_element_type=f32)
            tokens += [part[r:r + 8, 0:LANES] for r in range(0, D, 8)]
            if mode == "first":
                acc_s[:, ns] = part
            else:
                acc_s[:, ns] += part
        return tokens if due is not None else tokens[:len(tokens) * 7 // 8]

    zeros = jnp.zeros((D, LANES), f32)
    qkv_s[0, D:2 * D, :] = zeros
    qkv_s[0, 2 * D:3 * D, :] = zeros
    rk_s[0] = zeros
    rv_s[0] = zeros

    for j in range(CPC):
        _scope("wx0", lambda: x0_cp(j).wait())
        ln_piece(0, [], (j,))
    for rects, xc in RAMP:
        def waits():
            for r in rects:
                rect_cp(r).wait()
            if xc is not None:
                x_cp(xc).wait()
        _scope("wr", waits)
        tokens = []
        for p, lo, hi in rects:
            tokens += mix1(p, "first" if p == 0 else "mid", lo, hi)
        if xc is not None:
            ln_piece(xc, tokens)

    def mid_step(p, carry):
        _scope("wl", lambda: (w1_cp(p).wait(), x_cp(p + 1).wait()))
        ln_piece(p + 1, mix1(p, "mid"))
        return carry + 1

    steps = jax.lax.fori_loop(2, NC - 1, mid_step, 0)

    def waits():
        wqkv_cp.wait()
        wo_cp.wait()
        b1_cp.wait()
        b2_cp.wait()
        w1_cp(NC - 1).wait()
    _scope("wlast", waits)
    def qkv(c):
        r = jnp.dot(wqkvt_s[...], xn_s[c], preferred_element_type=f32)
        for j in range(TC // LANES):
            qkv_s[c * (TC // LANES) + j + 1] = r[:, j * LANES:(j + 1) * LANES]
        return _tokens(r)

    scale = DH ** -0.5

    def attn_col(jj, pace):
        lane = jax.lax.broadcasted_iota(jnp.int32, (SLAB, LANES), 1)
        m0 = [None] + [lane < LANES - 2 * a for a in range(1, 4)]
        m1 = [(lane >= 8) & (lane < LANES - 2 * a) for a in range(4)]
        nd = SLAB // H
        acc = [[None, None] for _ in range(4)]
        hist = [(), ()]
        for sl in range(D // SLAB):
            r0 = sl * SLAB
            q = qkv_s[jj + 1, r0:r0 + SLAB, :]
            k = qkv_s[jj + 1, D + r0:D + r0 + SLAB, :]
            q, k = pace.gate(q, k, after=hist[-2])
            kp = qkv_s[jj, D + r0:D + r0 + SLAB, :]
            rkp = rk_s[jj % 2, r0:r0 + SLAB, :]
            rk = pltpu.roll(k, 8, 1)
            rk_s[(jj + 1) % 2, r0:r0 + SLAB, :] = rk
            for a in range(4):
                rq = q if a == 0 else pltpu.roll(q, LANES - 2 * a, 1)
                for b in range(2):
                    if b == 0:
                        mix = k if a == 0 else jnp.where(m0[a], k, kp)
                    else:
                        mix = jnp.where(m1[a], rk, rkp)
                    p = rq * mix
                    for i in range(nd):
                        pi = p[i * H:(i + 1) * H]
                        acc[a][b] = pi if acc[a][b] is None else acc[a][b] + pi
            hist.append(tuple(acc[a][b][h:h + 8] for a in range(4) for b in range(2) for h in (0, 8)))
        lane16 = jax.lax.broadcasted_iota(jnp.int32, (H, LANES), 1)
        logit = []
        for w in range(W):
            a, b = w % 4, w // 4
            lw = acc[a][b] if a == 0 else pltpu.roll(acc[a][b], 2 * a, 1)
            lw = lw * scale
            if jj == 0 and w > 0:
                lw = jnp.where(lane16 >= 2 * w, lw, -1e9)
            logit.append(lw)
        mx = functools.reduce(jnp.maximum, logit)
        ex = [jnp.exp(l - mx) for l in logit]
        inv = 1.0 / functools.reduce(jnp.add, ex)
        ra = [[None, None] for _ in range(4)]
        for w in range(W):
            a, b = w % 4, w // 4
            aw = ex[w] * inv
            aw = aw if a == 0 else pltpu.roll(aw, LANES - 2 * a, 1)
            ra[a][b] = jnp.concatenate([aw] * nd, axis=0)
        for sl in range(D // SLAB):
            r0 = sl * SLAB
            v = qkv_s[jj + 1, 2 * D + r0:2 * D + r0 + SLAB, :]
            v, = pace.gate(v)
            vp = qkv_s[jj, 2 * D + r0:2 * D + r0 + SLAB, :]
            rvp = rv_s[jj % 2, r0:r0 + SLAB, :]
            rv = pltpu.roll(v, 8, 1)
            rv_s[(jj + 1) % 2, r0:r0 + SLAB, :] = rv
            o = None
            for a in range(4):
                mix0 = v if a == 0 else jnp.where(m0[a], v, vp)
                mix1 = jnp.where(m1[a], rv, rvp)
                t = ra[a][0] * mix0 + ra[a][1] * mix1
                o = t if a == 0 else o + pltpu.roll(t, 2 * a, 1)
            o_s[r0:r0 + SLAB, jj * LANES:(jj + 1) * LANES] = o.astype(bf16)

    def attn(c, tokens):
        z = b2f_s[0:8, :]
        pace = _Pacer(tokens, 2 * (D // SLAB) * CPC, z + 1.0 < z)
        for j in range(CPC):
            attn_col(c * CPC + j, pace)

    def gelu(tokens):
        z = b2f_s[0:8, :]
        pace = _Pacer(tokens, NLB * (F // LANES), z + 1.0 < z)
        for nn in range(F // LANES):
            col = pl.ds(nn * LANES, LANES)
            bias = jnp.broadcast_to(b1f_s[nn:nn + 1, :], (8, LANES))
            for i in range(NLB):
                rows = slice(i * LNB, (i + 1) * LNB)
                u_s[rows, col] = _gelu(acc_s[rows, col] + _rep(pace(bias), LNB)).astype(bf16)

    def gate_mm(i):
        cs = slice(OOFF[i], OOFF[i + 1])
        y, tokens = None, []
        for k0 in range(0, F, KB):
            ks = slice(k0, min(k0 + KB, F))
            part = jnp.dot(u_s[:, ks], w2_s[ks, cs], preferred_element_type=f32)
            tokens += _tokens(part) if k0 + KB <= F else _tokens(part[:, 0:LANES])
            y = part if y is None else y + part
        g = []
        for j in range(OUT_PIECES[i] // LANES):
            jj = OOFF[i] // LANES + j
            g.append(_silu(y[:, j * LANES:(j + 1) * LANES] + b2f_s[jj:jj + 1, :]))
        return g, tokens

    def final(i, g):
        cs = slice(OOFF[i], OOFF[i + 1])
        s = jnp.dot(wot_s[...], o_s[:, cs], preferred_element_type=f32)
        rows = TAIL_ROWS if i == NO - 1 else (0, D)
        for (r0, r1), cp in zip(zip(rows[:-1], rows[1:]), out_cps(i)):
            for j in range(OUT_PIECES[i] // LANES):
                jj = OOFF[i] // LANES + j
                xr = x_s[jj // CPC, r0:r1, pl.ds((jj % CPC) * LANES, LANES)].astype(f32)
                r = xr + s[r0:r1, j * LANES:(j + 1) * LANES] * g[j][r0:r1]
                out_s[r0:r1, pl.ds(jj * LANES, LANES)] = r.astype(bf16)
            cp.start()
        return _tokens(s)

    @pl.when(steps == NC - 3)
    def _():
        b1f_s[...] = b1_s[...].astype(f32)
        b2f_s[...] = b2_s[...].astype(f32)
        prep_wqkv_t()
        z = b2f_s[0:8, :]
        never = z + 1.0 < z
        nb = (F // NB) * (D // 16)
        last = mix1(NC - 1, "mid", due=_spread(prep_wqkv_perm(), nb, nb * 2 // 7, nb), never=never)

        tokens = []
        for c in range(QKV_AHEAD):
            tokens += qkv(c)
        gelu(last[len(last) // 2:] + tokens[:len(tokens) // 3])
        attn(0, tokens[len(tokens) // 3:len(tokens) * 9 // 10])

    _scope("ww2", lambda: w2_cp.wait())
    prep_wo()
    tokens = []
    for c in range(NC):
        if c + QKV_AHEAD < NC:
            tokens += qkv(c + QKV_AHEAD)
        g, t = gate_mm(c)
        tokens += t + final(c, g)
        if c + 1 < NC:
            attn(c + 1, tokens[c * ATTN_WIN:(c + 1) * ATTN_WIN])
    final(NC, gate_mm(NC)[0])

    def waits():
        for i in range(NO):
            for cp in out_cps(i):
                cp.wait()
    _scope("wout", waits)


@jax.jit
def pallas_recurrent_scan__sliding_local_dilated__mixer_token_mlp__prompt_kernel(
    A_x: jax.Array,
    A_wqkv: jax.Array,
    A_wo: jax.Array,
    B_x: jax.Array,
    B_w1: jax.Array,
    B_b1: jax.Array,
    B_w2: jax.Array,
    B_b2: jax.Array,
):
    del B_x
    xt = jnp.swapaxes(A_x, 1, 2)
    b1 = B_b1.reshape(F // LANES, LANES)
    b2 = B_b2.reshape(S // LANES, LANES)
    any_spec = pl.BlockSpec(memory_space=pl.ANY)
    out_t = pl.pallas_call(
        _kernel,
        out_shape=jax.ShapeDtypeStruct((1, D, S), bf16),
        in_specs=[any_spec] * 7,
        out_specs=any_spec,
        scratch_shapes=[
            pltpu.VMEM((NC, D, TC), bf16),
            pltpu.VMEM((D, 3 * D), bf16),
            pltpu.VMEM((D, D), bf16),
            pltpu.VMEM((NC, TC, F), bf16),
            pltpu.VMEM((F, S), bf16),
            pltpu.VMEM((F // LANES, LANES), bf16),
            pltpu.VMEM((S // LANES, LANES), bf16),
            pltpu.VMEM((NC, D // 2, TC), u32),
            pltpu.VMEM((NC, D // 2, TC), u32),
            pltpu.VMEM((D, F), f32),
            pltpu.VMEM((D // 2, F), u32),
            pltpu.VMEM((4, 11 * LANES, LANES), f32),
            pltpu.VMEM((3 * D // 2, D), u32),
            pltpu.VMEM((4, D, LANES), f32),
            pltpu.VMEM((D // 2, D), u32),
            pltpu.VMEM((NCOL + 1, 3 * D, LANES), f32),
            pltpu.VMEM((2, D, LANES), f32),
            pltpu.VMEM((2, D, LANES), f32),
            pltpu.VMEM((D // 2, S), u32),
            pltpu.VMEM((D, S), bf16),
            pltpu.VMEM((F // LANES, LANES), f32),
            pltpu.VMEM((S // LANES, LANES), f32),
            pltpu.SemaphoreType.DMA((NSEM,)),
        ],
        compiler_params=pltpu.CompilerParams(vmem_limit_bytes=100 * 1024 * 1024,
                                             disable_semaphore_checks=True,
                                             disable_bounds_checks=True),
        name="fused_mixer_attn",
    )(xt, A_wqkv, A_wo, B_w1, b1, B_w2, b2)
    return jnp.swapaxes(out_t, 1, 2)
```

```python
import functools

import jax
import jax.numpy as jnp
import jax.experimental.pallas as pl
import jax.experimental.pallas.tpu as pltpu

S = 2048
D = 448
H = 16
DH = D // H
F = 1792
W = 8
EPS = 1e-5
TC = 256
NC = S // TC
LANES = 128
NCOL = S // LANES
SLAB = 32

f32 = jnp.float32
bf16 = jnp.bfloat16
u32 = jnp.uint32

_SCOPES = False


def _scope(name, fn):
    if _SCOPES:
        with jax.named_scope(name):
            fn()
    else:
        fn()


LNB = 64
NLB = D // LNB


def _rep(v8, rows):
    return jnp.concatenate([v8] * (rows // 8), axis=0)


def _ln_stats(x_ref, col, pace):
    piv = jnp.broadcast_to(x_ref[0:1, col].astype(f32), (8, LANES))
    s1 = s2 = None
    for i in range(NLB):
        pv = _rep(pace(piv), LNB // 2)
        w = pltpu.bitcast(x_ref[i * LNB:(i + 1) * LNB, col], u32)
        for half in (w << 16, w & jnp.uint32(0xFFFF0000)):
            d = pltpu.bitcast(half, f32) - pv
            for k in range(LNB // 2 // 16):
                dk = d[k * 16:(k + 1) * 16]
                s1 = dk if s1 is None else s1 + dk
                s2 = dk * dk if s2 is None else s2 + dk * dk
    md = jnp.sum(s1, axis=0, keepdims=True) * (1.0 / D)
    v = jnp.maximum(jnp.sum(s2, axis=0, keepdims=True) * (1.0 / D) - md * md, 0.0)
    return piv + md, jax.lax.rsqrt(v + EPS)


def _tokens(r):
    return [r[i:i + 8, j:j + LANES] for j in range(0, r.shape[1], LANES) for i in range(0, r.shape[0], 8)]


def _deadline(lhs, toks, never):
    if not any(t is not None for t in toks):
        return lhs
    w = pltpu.bitcast(lhs, u32)
    blocks = [w[8 * i:8 * i + 8, 0:LANES] for i in range(w.shape[0] // 8)]
    blocks = [b if t is None else jnp.where(never, t, b) for b, t in zip(blocks, toks, strict=True)]
    w = jnp.concatenate([jnp.concatenate(blocks, axis=0), w[:, LANES:]], axis=1)
    return pltpu.bitcast(w, bf16)


def _spread(vals, nslots, lo, hi):
    out = [None] * nslots
    for i in range(lo, hi):
        out[i] = vals[((i - lo + 1) * len(vals)) // (hi - lo) - 1]
    return out


class _Pacer:
    def __init__(self, tokens, count, never):
        self.tokens, self.count, self.never, self.i = tokens, count, never, 0

    def __call__(self, v8):
        if not self.tokens:
            return v8
        tok = self.tokens[self.i * len(self.tokens) // self.count]
        self.i += 1
        return jnp.where(self.never, tok, v8)

    def gate(self, *vs, after=()):
        if not self.tokens:
            return vs
        tok = self.tokens[self.i * len(self.tokens) // self.count]
        self.i += 1
        for a in after:
            tok = jnp.maximum(tok, a)
        n = vs[0].shape[0]
        nv, tk = _rep(self.never, n), _rep(tok, n)
        return tuple(jnp.where(nv, tk, v) for v in vs)


def _gelu(x):
    c = 0.7978845608028654
    t = jnp.tanh(x * (c + (c * 0.044715) * (x * x)))
    hx = 0.5 * x
    return hx + hx * t


def _silu(y):
    hy = 0.5 * y
    return hy + hy * jnp.tanh(hy)


RAMP = (
    (((0, 0, 256),), None),
    (((0, 256, 768),), None),
    (((0, 768, 1280),), 1),
    (((0, 1280, F), (1, 0, 512)), None),
    (((1, 512, F),), 2),
)
RECTS = tuple(r for rects, _ in RAMP for r in rects)
NB = 256
ATTN_WIN = 740
KB = 512
CPC = TC // LANES
QKV_AHEAD = 3
OUT_PIECES = (256,) * 7 + (128, 128)
OOFF = tuple(sum(OUT_PIECES[:i]) for i in range(len(OUT_PIECES) + 1))
NO = len(OUT_PIECES)
TAIL_ROWS = (0, 256, 384, D)
SEM_X, SEM_W1, SEM_MISC, SEM_OUT = 0, NC, 2 * NC, 2 * NC + 6
SEM_RAMP = SEM_OUT + NO + len(TAIL_ROWS) - 2
NSEM = SEM_RAMP + len(RECTS)


def _kernel(x_hbm, wqkv_hbm, wo_hbm, w1_hbm, b1_hbm, w2_hbm, b2_hbm, out_hbm,
            x_s, wqkv_s, wo_s, w1_s, w2_s, b1_s, b2_s,
            xn_s, h_s, acc_s, u_s, wt32_s, wqkvt_s, wo32_s, wot_s,
            qkv_s, rk_s, rv_s, o_s, out_s, b1f_s, b2f_s, sem):
    xn_s, h_s, u_s, wqkvt_s, wot_s, o_s = (
        r.bitcast(bf16) for r in (xn_s, h_s, u_s, wqkvt_s, wot_s, o_s))

    def x_cp(p):
        return pltpu.make_async_copy(x_hbm.at[0, :, pl.ds(p * TC, TC)], x_s.at[p], sem.at[SEM_X + p])

    def w1_cp(p):
        return pltpu.make_async_copy(w1_hbm.at[pl.ds(p * TC, TC), :], w1_s.at[p], sem.at[SEM_W1 + p])

    def rect_cp(r):
        p, lo, hi = r
        return pltpu.make_async_copy(w1_hbm.at[p * TC:(p + 1) * TC, lo:hi], w1_s.at[p, :, lo:hi],
                                     sem.at[SEM_RAMP + RECTS.index(r)])

    def out_cps(i):
        sl = slice(OOFF[i], OOFF[i + 1])
        rows = TAIL_ROWS if i == NO - 1 else (0, D)
        return [pltpu.make_async_copy(out_s.at[r0:r1, sl], out_hbm.at[0, r0:r1, sl], sem.at[SEM_OUT + i + k])
                for k, (r0, r1) in enumerate(zip(rows[:-1], rows[1:]))]

    def x0_cp(j):
        sl = pl.ds(j * LANES, LANES)
        return pltpu.make_async_copy(x_hbm.at[0, :, sl], x_s.at[0, :, sl],
                                     sem.at[SEM_X if j == 0 else SEM_MISC + 5])

    wqkv_cp = pltpu.make_async_copy(wqkv_hbm, wqkv_s, sem.at[SEM_MISC + 0])
    wo_cp = pltpu.make_async_copy(wo_hbm, wo_s, sem.at[SEM_MISC + 1])
    b1_cp = pltpu.make_async_copy(b1_hbm, b1_s, sem.at[SEM_MISC + 2])
    b2_cp = pltpu.make_async_copy(b2_hbm, b2_s, sem.at[SEM_MISC + 3])
    w2_cp = pltpu.make_async_copy(w2_hbm, w2_s, sem.at[SEM_MISC + 4])

    x0_cp(0).start()
    x0_cp(1).start()
    for rects, xc in RAMP:
        for r in rects:
            rect_cp(r).start()
        if xc is not None:
            x_cp(xc).start()
    for p in range(2, NC):
        if p == NC - 1:
            wqkv_cp.start()
            wo_cp.start()
            b1_cp.start()
            b2_cp.start()
        w1_cp(p).start()
        if p + 1 < NC:
            x_cp(p + 1).start()
    w2_cp.start()

    def prep_wqkv_t():
        for c in range(11):
            wd = min(LANES, 3 * D - c * LANES)
            blk = wqkv_s[:, c * LANES:c * LANES + wd].T.astype(f32)
            for kt in range(4):
                kw = min(LANES, D - kt * LANES)
                wt32_s[kt, c * LANES:c * LANES + wd, 0:kw] = blk[:, kt * LANES:kt * LANES + kw]

    def prep_wqkv_perm():
        done = []
        for sec in range(3):
            for d in range(DH):
                r0 = sec * D + d * H
                tok = None
                for kt in range(4):
                    kw = min(LANES, D - kt * LANES)
                    rows = wt32_s[kt, pl.ds(sec * D + d, H, stride=DH), :]
                    wqkvt_s[r0:r0 + H, kt * LANES:kt * LANES + kw] = rows[:, 0:kw].astype(bf16)
                    if kt < 3:
                        t = pltpu.bitcast(rows[8:16], u32)
                        tok = t if tok is None else tok | t
                done.append(tok)
        return done

    def prep_wo():
        for nt in range(4):
            nw = min(LANES, D - nt * LANES)
            wo32_s[nt, :, 0:nw] = wo_s[:, nt * LANES:nt * LANES + nw].astype(f32)
        for nt in range(4):
            nw = min(LANES, D - nt * LANES)
            rows = [wo32_s[nt, pl.ds(d, H, stride=DH), :][:, 0:nw].astype(bf16) for d in range(DH)]
            blk = jnp.concatenate(rows, axis=0)
            wot_s[nt * LANES:nt * LANES + nw, :] = blk.T

    def ln_piece(p, tokens, cols=tuple(range(CPC))):
        xp, xnp, hp = x_s.at[p], xn_s.at[p], h_s.at[p]
        z = xp[0:8, 0:LANES].astype(f32)
        pace = _Pacer(tokens, 3 * NLB * CPC, z + 1.0 < z)
        for j in cols:
            col = pl.ds(j * LANES, LANES)
            m, r = _ln_stats(xp, col, pace)
            t1 = t2 = None
            for i in range(NLB):
                rows = slice(i * LNB, (i + 1) * LNB)
                xn = (xp[rows, col].astype(f32) - _rep(pace(m), LNB)) * r
                xnp[rows, col] = xn.astype(bf16)
                for k in range(LNB // 16):
                    xk = xn[k * 16:(k + 1) * 16]
                    t1 = xk if t1 is None else t1 + xk
                    t2 = xk * xk if t2 is None else t2 + xk * xk
            m2 = jnp.sum(t1, axis=0, keepdims=True) * (1.0 / D)
            v2 = jnp.maximum(jnp.sum(t2, axis=0, keepdims=True) * (1.0 / D) - m2 * m2, 0.0)
            r2 = jax.lax.rsqrt(v2 + EPS)
            m2 = jnp.broadcast_to(m2, (8, LANES))
            for i in range(NLB):
                rows = slice(i * LNB, (i + 1) * LNB)
                hp[rows, col] = ((xnp[rows, col].astype(f32) - _rep(pace(m2), LNB)) * r2).astype(bf16)

    def mix1(p, mode, n_lo=0, n_hi=F, due=None, never=None):
        tokens = []
        nb = D // 16
        for n in range(n_lo // NB, n_hi // NB):
            ns = slice(n * NB, (n + 1) * NB)
            lhs = h_s[p] if due is None else _deadline(h_s[p], due[n * nb:(n + 1) * nb], never)
            part = jnp.dot(lhs, w1_s[p, :, ns], preferred_element_type=f32)
            tokens += [part[r:r + 8, 0:LANES] for r in range(0, D, 8)]
            if mode == "first":
                acc_s[:, ns] = part
            else:
                acc_s[:, ns] += part
        return tokens if due is not None else tokens[:len(tokens) * 7 // 8]

    zeros = jnp.zeros((D, LANES), f32)
    qkv_s[0, D:2 * D, :] = zeros
    qkv_s[0, 2 * D:3 * D, :] = zeros
    rk_s[0] = zeros
    rv_s[0] = zeros

    for j in range(CPC):
        _scope("wx0", lambda: x0_cp(j).wait())
        ln_piece(0, [], (j,))
    for rects, xc in RAMP:
        def waits():
            for r in rects:
                rect_cp(r).wait()
            if xc is not None:
                x_cp(xc).wait()
        _scope("wr", waits)
        tokens = []
        for p, lo, hi in rects:
            tokens += mix1(p, "first" if p == 0 else "mid", lo, hi)
        if xc is not None:
            ln_piece(xc, tokens)

    def mid_step(p, carry):
        _scope("wl", lambda: (w1_cp(p).wait(), x_cp(p + 1).wait()))
        ln_piece(p + 1, mix1(p, "mid"))
        return carry + 1

    steps = jax.lax.fori_loop(2, NC - 1, mid_step, 0)

    def waits():
        wqkv_cp.wait()
        wo_cp.wait()
        b1_cp.wait()
        b2_cp.wait()
        w1_cp(NC - 1).wait()
    _scope("wlast", waits)
    def qkv(c):
        r = jnp.dot(wqkvt_s[...], xn_s[c], preferred_element_type=f32)
        for j in range(TC // LANES):
            qkv_s[c * (TC // LANES) + j + 1] = r[:, j * LANES:(j + 1) * LANES]
        return _tokens(r)

    scale = DH ** -0.5

    def attn_col(jj, pace):
        lane = jax.lax.broadcasted_iota(jnp.int32, (SLAB, LANES), 1)
        m0 = [None] + [lane < LANES - 2 * a for a in range(1, 4)]
        m1 = [(lane >= 8) & (lane < LANES - 2 * a) for a in range(4)]
        nd = SLAB // H
        acc = [[None, None] for _ in range(4)]
        hist = [(), ()]
        for sl in range(D // SLAB):
            r0 = sl * SLAB
            q = qkv_s[jj + 1, r0:r0 + SLAB, :]
            k = qkv_s[jj + 1, D + r0:D + r0 + SLAB, :]
            q, k = pace.gate(q, k, after=hist[-2])
            kp = qkv_s[jj, D + r0:D + r0 + SLAB, :]
            rkp = rk_s[jj % 2, r0:r0 + SLAB, :]
            rk = pltpu.roll(k, 8, 1)
            rk_s[(jj + 1) % 2, r0:r0 + SLAB, :] = rk
            for a in range(4):
                rq = q if a == 0 else pltpu.roll(q, LANES - 2 * a, 1)
                for b in range(2):
                    if b == 0:
                        mix = k if a == 0 else jnp.where(m0[a], k, kp)
                    else:
                        mix = jnp.where(m1[a], rk, rkp)
                    p = rq * mix
                    for i in range(nd):
                        pi = p[i * H:(i + 1) * H]
                        acc[a][b] = pi if acc[a][b] is None else acc[a][b] + pi
            hist.append(tuple(acc[a][b][h:h + 8] for a in range(4) for b in range(2) for h in (0, 8)))
        lane16 = jax.lax.broadcasted_iota(jnp.int32, (H, LANES), 1)
        logit = []
        for w in range(W):
            a, b = w % 4, w // 4
            lw = acc[a][b] if a == 0 else pltpu.roll(acc[a][b], 2 * a, 1)
            lw = lw * scale
            if jj == 0 and w > 0:
                lw = jnp.where(lane16 >= 2 * w, lw, -1e9)
            logit.append(lw)
        mx = functools.reduce(jnp.maximum, logit)
        ex = [jnp.exp(l - mx) for l in logit]
        inv = 1.0 / functools.reduce(jnp.add, ex)
        ra = [[None, None] for _ in range(4)]
        for w in range(W):
            a, b = w % 4, w // 4
            aw = ex[w] * inv
            aw = aw if a == 0 else pltpu.roll(aw, LANES - 2 * a, 1)
            ra[a][b] = jnp.concatenate([aw] * nd, axis=0)
        for sl in range(D // SLAB):
            r0 = sl * SLAB
            v = qkv_s[jj + 1, 2 * D + r0:2 * D + r0 + SLAB, :]
            v, = pace.gate(v)
            vp = qkv_s[jj, 2 * D + r0:2 * D + r0 + SLAB, :]
            rvp = rv_s[jj % 2, r0:r0 + SLAB, :]
            rv = pltpu.roll(v, 8, 1)
            rv_s[(jj + 1) % 2, r0:r0 + SLAB, :] = rv
            o = None
            for a in range(4):
                mix0 = v if a == 0 else jnp.where(m0[a], v, vp)
                mix1 = jnp.where(m1[a], rv, rvp)
                t = ra[a][0] * mix0 + ra[a][1] * mix1
                o = t if a == 0 else o + pltpu.roll(t, 2 * a, 1)
            o_s[r0:r0 + SLAB, jj * LANES:(jj + 1) * LANES] = o.astype(bf16)

    def attn(c, tokens):
        z = b2f_s[0:8, :]
        pace = _Pacer(tokens, 2 * (D // SLAB) * CPC, z + 1.0 < z)
        for j in range(CPC):
            attn_col(c * CPC + j, pace)

    def gelu(tokens):
        z = b2f_s[0:8, :]
        pace = _Pacer(tokens, NLB * (F // LANES), z + 1.0 < z)
        for nn in range(F // LANES):
            col = pl.ds(nn * LANES, LANES)
            bias = jnp.broadcast_to(b1f_s[nn:nn + 1, :], (8, LANES))
            for i in range(NLB):
                rows = slice(i * LNB, (i + 1) * LNB)
                u_s[rows, col] = _gelu(acc_s[rows, col] + _rep(pace(bias), LNB)).astype(bf16)

    def gate_mm(i):
        cs = slice(OOFF[i], OOFF[i + 1])
        y, tokens = None, []
        for k0 in range(0, F, KB):
            ks = slice(k0, min(k0 + KB, F))
            part = jnp.dot(u_s[:, ks], w2_s[ks, cs], preferred_element_type=f32)
            tokens += _tokens(part) if k0 + KB <= F else _tokens(part[:, 0:LANES])
            y = part if y is None else y + part
        g = []
        for j in range(OUT_PIECES[i] // LANES):
            jj = OOFF[i] // LANES + j
            g.append(_silu(y[:, j * LANES:(j + 1) * LANES] + b2f_s[jj:jj + 1, :]))
        return g, tokens

    def final(i, g):
        cs = slice(OOFF[i], OOFF[i + 1])
        s = jnp.dot(wot_s[...], o_s[:, cs], preferred_element_type=f32)
        rows = TAIL_ROWS if i == NO - 1 else (0, D)
        for (r0, r1), cp in zip(zip(rows[:-1], rows[1:]), out_cps(i)):
            for j in range(OUT_PIECES[i] // LANES):
                jj = OOFF[i] // LANES + j
                xr = x_s[jj // CPC, r0:r1, pl.ds((jj % CPC) * LANES, LANES)].astype(f32)
                r = xr + s[r0:r1, j * LANES:(j + 1) * LANES] * g[j][r0:r1]
                out_s[r0:r1, pl.ds(jj * LANES, LANES)] = r.astype(bf16)
            cp.start()
        return _tokens(s)

    @pl.when(steps == NC - 3)
    def _():
        b1f_s[...] = b1_s[...].astype(f32)
        b2f_s[...] = b2_s[...].astype(f32)
        prep_wqkv_t()
        z = b2f_s[0:8, :]
        never = z + 1.0 < z
        nb = (F // NB) * (D // 16)
        last = mix1(NC - 1, "mid", due=_spread(prep_wqkv_perm(), nb, nb * 2 // 7, nb), never=never)

        tokens = []
        for c in range(QKV_AHEAD):
            tokens += qkv(c)
        gelu(last[len(last) // 2:] + tokens[:len(tokens) // 3])
        attn(0, tokens[len(tokens) // 3:len(tokens) * 9 // 10])

    _scope("ww2", lambda: w2_cp.wait())
    prep_wo()
    tokens = []
    for c in range(NC):
        if c + QKV_AHEAD < NC:
            tokens += qkv(c + QKV_AHEAD)
        g, t = gate_mm(c)
        tokens += t + final(c, g)
        if c + 1 < NC:
            attn(c + 1, tokens[c * ATTN_WIN:(c + 1) * ATTN_WIN])
    final(NC, gate_mm(NC)[0])

    def waits():
        for i in range(NO):
            for cp in out_cps(i):
                cp.wait()
    _scope("wout", waits)


@jax.jit
def pallas_recurrent_scan__sliding_local_dilated__mixer_token_mlp__prompt_kernel(
    A_x: jax.Array,
    A_wqkv: jax.Array,
    A_wo: jax.Array,
    B_x: jax.Array,
    B_w1: jax.Array,
    B_b1: jax.Array,
    B_w2: jax.Array,
    B_b2: jax.Array,
):
    del B_x
    xt = jnp.swapaxes(A_x, 1, 2)
    b1 = B_b1.reshape(F // LANES, LANES)
    b2 = B_b2.reshape(S // LANES, LANES)
    any_spec = pl.BlockSpec(memory_space=pl.ANY)
    out_t = pl.pallas_call(
        _kernel,
        out_shape=jax.ShapeDtypeStruct((1, D, S), bf16),
        in_specs=[any_spec] * 7,
        out_specs=any_spec,
        scratch_shapes=[
            pltpu.VMEM((NC, D, TC), bf16),
            pltpu.VMEM((D, 3 * D), bf16),
            pltpu.VMEM((D, D), bf16),
            pltpu.VMEM((NC, TC, F), bf16),
            pltpu.VMEM((F, S), bf16),
            pltpu.VMEM((F // LANES, LANES), bf16),
            pltpu.VMEM((S // LANES, LANES), bf16),
            pltpu.VMEM((NC, D // 2, TC), u32),
            pltpu.VMEM((NC, D // 2, TC), u32),
            pltpu.VMEM((D, F), f32),
            pltpu.VMEM((D // 2, F), u32),
            pltpu.VMEM((4, 11 * LANES, LANES), f32),
            pltpu.VMEM((3 * D // 2, D), u32),
            pltpu.VMEM((4, D, LANES), f32),
            pltpu.VMEM((D // 2, D), u32),
            pltpu.VMEM((NCOL + 1, 3 * D, LANES), f32),
            pltpu.VMEM((2, D, LANES), f32),
            pltpu.VMEM((2, D, LANES), f32),
            pltpu.VMEM((D // 2, S), u32),
            pltpu.VMEM((D, S), bf16),
            pltpu.VMEM((F // LANES, LANES), f32),
            pltpu.VMEM((S // LANES, LANES), f32),
            pltpu.SemaphoreType.DMA((NSEM,)),
        ],
        compiler_params=pltpu.CompilerParams(vmem_limit_bytes=100 * 1024 * 1024,
                                             disable_semaphore_checks=True,
                                             disable_bounds_checks=True),
        name="fused_mixer_attn",
    )(xt, A_wqkv, A_wo, B_w1, b1, B_w2, b2)
    return jnp.swapaxes(out_t, 1, 2)
```

```python
import functools

import jax
import jax.numpy as jnp
import jax.experimental.pallas as pl
import jax.experimental.pallas.tpu as pltpu

S = 2048
D = 448
H = 16
DH = D // H
F = 1792
W = 8
EPS = 1e-5
TC = 256
NC = S // TC
LANES = 128
NCOL = S // LANES
SLAB = 32

f32 = jnp.float32
bf16 = jnp.bfloat16
u32 = jnp.uint32

_SCOPES = False


def _scope(name, fn):
    if _SCOPES:
        with jax.named_scope(name):
            fn()
    else:
        fn()


LNB = 64
NLB = D // LNB


def _rep(v8, rows):
    return jnp.concatenate([v8] * (rows // 8), axis=0)


def _ln_stats(x_ref, col, pace):
    piv = jnp.broadcast_to(x_ref[0:1, col].astype(f32), (8, LANES))
    s1 = s2 = None
    for i in range(NLB):
        pv = _rep(pace(piv), LNB // 2)
        w = pltpu.bitcast(x_ref[i * LNB:(i + 1) * LNB, col], u32)
        for half in (w << 16, w & jnp.uint32(0xFFFF0000)):
            d = pltpu.bitcast(half, f32) - pv
            for k in range(LNB // 2 // 16):
                dk = d[k * 16:(k + 1) * 16]
                s1 = dk if s1 is None else s1 + dk
                s2 = dk * dk if s2 is None else s2 + dk * dk
    md = jnp.sum(s1, axis=0, keepdims=True) * (1.0 / D)
    v = jnp.maximum(jnp.sum(s2, axis=0, keepdims=True) * (1.0 / D) - md * md, 0.0)
    return piv + md, jax.lax.rsqrt(v + EPS)


def _tokens(r):
    return [r[i:i + 8, j:j + LANES] for j in range(0, r.shape[1], LANES) for i in range(0, r.shape[0], 8)]


def _deadline(lhs, toks, never):
    if not any(t is not None for t in toks):
        return lhs
    w = pltpu.bitcast(lhs, u32)
    blocks = [w[8 * i:8 * i + 8, 0:LANES] for i in range(w.shape[0] // 8)]
    blocks = [b if t is None else jnp.where(never, t, b) for b, t in zip(blocks, toks, strict=True)]
    w = jnp.concatenate([jnp.concatenate(blocks, axis=0), w[:, LANES:]], axis=1)
    return pltpu.bitcast(w, bf16)


def _spread(vals, nslots, lo, hi):
    out = [None] * nslots
    for i in range(lo, hi):
        out[i] = vals[((i - lo + 1) * len(vals)) // (hi - lo) - 1]
    return out


class _Pacer:
    def __init__(self, tokens, count, never):
        self.tokens, self.count, self.never, self.i = tokens, count, never, 0

    def __call__(self, v8):
        if not self.tokens:
            return v8
        tok = self.tokens[self.i * len(self.tokens) // self.count]
        self.i += 1
        return jnp.where(self.never, tok, v8)

    def gate(self, *vs, after=()):
        if not self.tokens:
            return vs
        tok = self.tokens[self.i * len(self.tokens) // self.count]
        self.i += 1
        for a in after:
            tok = jnp.maximum(tok, a)
        n = vs[0].shape[0]
        nv, tk = _rep(self.never, n), _rep(tok, n)
        return tuple(jnp.where(nv, tk, v) for v in vs)


def _gelu(x):
    c = 0.7978845608028654
    t = jnp.tanh(x * (c + (c * 0.044715) * (x * x)))
    hx = 0.5 * x
    return hx + hx * t


def _silu(y):
    hy = 0.5 * y
    return hy + hy * jnp.tanh(hy)


RAMP = (
    (((0, 0, 128, 0, 768),), None),
    (((0, 0, 128, 768, F),), 0),
    (((0, 128, 256, 0, 1024),), 1),
    (((0, 128, 256, 1024, F), (1, 0, 256, 0, 512)), None),
    (((1, 0, 256, 512, F),), 2),
)
RECTS = tuple(r for rects, _ in RAMP for r in rects)
NB = 256
ATTN_WIN = 740
KB = 512
CPC = TC // LANES
QKV_AHEAD = 3
OUT_PIECES = (256,) * 7 + (128, 128)
OOFF = tuple(sum(OUT_PIECES[:i]) for i in range(len(OUT_PIECES) + 1))
NO = len(OUT_PIECES)
TAIL_ROWS = (0, 256, 384, D)
SEM_X, SEM_W1, SEM_MISC, SEM_OUT = 0, NC, 2 * NC, 2 * NC + 6
SEM_RAMP = SEM_OUT + NO + len(TAIL_ROWS) - 2
NSEM = SEM_RAMP + len(RECTS)


def _kernel(x_hbm, wqkv_hbm, wo_hbm, w1_hbm, b1_hbm, w2_hbm, b2_hbm, out_hbm,
            x_s, wqkv_s, wo_s, w1_s, w2_s, b1_s, b2_s,
            xn_s, h_s, acc_s, u_s, wt32_s, wqkvt_s, wo32_s, wot_s,
            qkv_s, rk_s, rv_s, o_s, out_s, b1f_s, b2f_s, sem):
    xn_s, h_s, u_s, wqkvt_s, wot_s, o_s = (
        r.bitcast(bf16) for r in (xn_s, h_s, u_s, wqkvt_s, wot_s, o_s))

    def x_cp(p):
        return pltpu.make_async_copy(x_hbm.at[0, :, pl.ds(p * TC, TC)], x_s.at[p], sem.at[SEM_X + p])

    def w1_cp(p):
        return pltpu.make_async_copy(w1_hbm.at[pl.ds(p * TC, TC), :], w1_s.at[p], sem.at[SEM_W1 + p])

    def rect_cp(r):
        p, k0, k1, lo, hi = r
        return pltpu.make_async_copy(w1_hbm.at[p * TC + k0:p * TC + k1, lo:hi], w1_s.at[p, k0:k1, lo:hi],
                                     sem.at[SEM_RAMP + RECTS.index(r)])

    def out_cps(i):
        sl = slice(OOFF[i], OOFF[i + 1])
        rows = TAIL_ROWS if i == NO - 1 else (0, D)
        return [pltpu.make_async_copy(out_s.at[r0:r1, sl], out_hbm.at[0, r0:r1, sl], sem.at[SEM_OUT + i + k])
                for k, (r0, r1) in enumerate(zip(rows[:-1], rows[1:]))]

    def x0_cp(j):
        sl = pl.ds(j * LANES, LANES)
        return pltpu.make_async_copy(x_hbm.at[0, :, sl], x_s.at[0, :, sl],
                                     sem.at[SEM_X if j == 0 else SEM_MISC + 5])

    wqkv_cp = pltpu.make_async_copy(wqkv_hbm, wqkv_s, sem.at[SEM_MISC + 0])
    wo_cp = pltpu.make_async_copy(wo_hbm, wo_s, sem.at[SEM_MISC + 1])
    b1_cp = pltpu.make_async_copy(b1_hbm, b1_s, sem.at[SEM_MISC + 2])
    b2_cp = pltpu.make_async_copy(b2_hbm, b2_s, sem.at[SEM_MISC + 3])
    w2_cp = pltpu.make_async_copy(w2_hbm, w2_s, sem.at[SEM_MISC + 4])

    def ramp_x_cp(xc):
        return x0_cp(1) if xc == 0 else x_cp(xc)

    x0_cp(0).start()
    for rects, xc in RAMP:
        for r in rects:
            rect_cp(r).start()
        if xc is not None:
            ramp_x_cp(xc).start()
    for p in range(2, NC):
        if p == NC - 1:
            wqkv_cp.start()
            wo_cp.start()
            b1_cp.start()
            b2_cp.start()
        w1_cp(p).start()
        if p + 1 < NC:
            x_cp(p + 1).start()
    w2_cp.start()

    def prep_wqkv_t():
        for c in range(11):
            wd = min(LANES, 3 * D - c * LANES)
            blk = wqkv_s[:, c * LANES:c * LANES + wd].T.astype(f32)
            for kt in range(4):
                kw = min(LANES, D - kt * LANES)
                wt32_s[kt, c * LANES:c * LANES + wd, 0:kw] = blk[:, kt * LANES:kt * LANES + kw]

    def prep_wqkv_perm():
        done = []
        for sec in range(3):
            for d in range(DH):
                r0 = sec * D + d * H
                tok = None
                for kt in range(4):
                    kw = min(LANES, D - kt * LANES)
                    rows = wt32_s[kt, pl.ds(sec * D + d, H, stride=DH), :]
                    wqkvt_s[r0:r0 + H, kt * LANES:kt * LANES + kw] = rows[:, 0:kw].astype(bf16)
                    if kt < 3:
                        t = pltpu.bitcast(rows[8:16], u32)
                        tok = t if tok is None else tok | t
                done.append(tok)
        return done

    def prep_wo():
        for nt in range(4):
            nw = min(LANES, D - nt * LANES)
            wo32_s[nt, :, 0:nw] = wo_s[:, nt * LANES:nt * LANES + nw].astype(f32)
        for nt in range(4):
            nw = min(LANES, D - nt * LANES)
            rows = [wo32_s[nt, pl.ds(d, H, stride=DH), :][:, 0:nw].astype(bf16) for d in range(DH)]
            blk = jnp.concatenate(rows, axis=0)
            wot_s[nt * LANES:nt * LANES + nw, :] = blk.T

    def ln_piece(p, tokens, cols=tuple(range(CPC))):
        xp, xnp, hp = x_s.at[p], xn_s.at[p], h_s.at[p]
        z = xp[0:8, 0:LANES].astype(f32)
        pace = _Pacer(tokens, 3 * NLB * len(cols), z + 1.0 < z)
        for j in cols:
            col = pl.ds(j * LANES, LANES)
            m, r = _ln_stats(xp, col, pace)
            t1 = t2 = None
            for i in range(NLB):
                rows = slice(i * LNB, (i + 1) * LNB)
                xn = (xp[rows, col].astype(f32) - _rep(pace(m), LNB)) * r
                xnp[rows, col] = xn.astype(bf16)
                for k in range(LNB // 16):
                    xk = xn[k * 16:(k + 1) * 16]
                    t1 = xk if t1 is None else t1 + xk
                    t2 = xk * xk if t2 is None else t2 + xk * xk
            m2 = jnp.sum(t1, axis=0, keepdims=True) * (1.0 / D)
            v2 = jnp.maximum(jnp.sum(t2, axis=0, keepdims=True) * (1.0 / D) - m2 * m2, 0.0)
            r2 = jax.lax.rsqrt(v2 + EPS)
            m2 = jnp.broadcast_to(m2, (8, LANES))
            for i in range(NLB):
                rows = slice(i * LNB, (i + 1) * LNB)
                hp[rows, col] = ((xnp[rows, col].astype(f32) - _rep(pace(m2), LNB)) * r2).astype(bf16)

    def mix1(p, mode, n_lo=0, n_hi=F, due=None, never=None):
        tokens = []
        nb = D // 16
        for n in range(n_lo // NB, n_hi // NB):
            ns = slice(n * NB, (n + 1) * NB)
            lhs = h_s[p] if due is None else _deadline(h_s[p], due[n * nb:(n + 1) * nb], never)
            part = jnp.dot(lhs, w1_s[p, :, ns], preferred_element_type=f32)
            tokens += [part[r:r + 8, 0:LANES] for r in range(0, D, 8)]
            if mode == "first":
                acc_s[:, ns] = part
            else:
                acc_s[:, ns] += part
        return tokens if due is not None else tokens[:len(tokens) * 7 // 8]

    zeros = jnp.zeros((D, LANES), f32)
    qkv_s[0, D:2 * D, :] = zeros
    qkv_s[0, 2 * D:3 * D, :] = zeros
    rk_s[0] = zeros
    rv_s[0] = zeros

    def mix1_half(k0, n_lo, n_hi):
        tokens = []
        for lo in range(n_lo, n_hi, 2 * NB):
            ns = slice(lo, min(lo + 2 * NB, n_hi))
            halves = ((0, D),) if ns.stop - lo == 2 * NB else ((0, D // 2), (D // 2, D))
            for r0, r1 in halves:
                part = jnp.dot(h_s[0, r0:r1, k0:k0 + LANES], w1_s[0, k0:k0 + LANES, ns],
                               preferred_element_type=f32)
                if r0 == 0:
                    tokens += [part[r:r + 8, 0:LANES] for r in range(0, r1, 8)]
                if k0 == 0:
                    acc_s[r0:r1, ns] = part
                else:
                    acc_s[r0:r1, ns] += part
        return tokens[:len(tokens) * 7 // 8]

    _scope("wx0", lambda: x0_cp(0).wait())
    ln_piece(0, [], (0,))
    for rects, xc in RAMP:
        def waits():
            for r in rects:
                rect_cp(r).wait()
            if xc is not None:
                ramp_x_cp(xc).wait()
        _scope("wr", waits)
        tokens = []
        for p, k0, k1, lo, hi in rects:
            tokens += mix1_half(k0, lo, hi) if p == 0 else mix1(p, "mid", lo, hi)
        if xc is not None:
            ln_piece(xc, tokens, (1,) if xc == 0 else tuple(range(CPC)))

    def mid_step(p, carry):
        _scope("wl", lambda: (w1_cp(p).wait(), x_cp(p + 1).wait()))
        ln_piece(p + 1, mix1(p, "mid"))
        return carry + 1

    steps = jax.lax.fori_loop(2, NC - 1, mid_step, 0)

    def waits():
        wqkv_cp.wait()
        wo_cp.wait()
        b1_cp.wait()
        b2_cp.wait()
        w1_cp(NC - 1).wait()
    _scope("wlast", waits)
    def qkv(c):
        r = jnp.dot(wqkvt_s[...], xn_s[c], preferred_element_type=f32)
        for j in range(TC // LANES):
            qkv_s[c * (TC // LANES) + j + 1] = r[:, j * LANES:(j + 1) * LANES]
        return _tokens(r)

    scale = DH ** -0.5

    def attn_col(jj, pace):
        lane = jax.lax.broadcasted_iota(jnp.int32, (SLAB, LANES), 1)
        m0 = [None] + [lane < LANES - 2 * a for a in range(1, 4)]
        m1 = [(lane >= 8) & (lane < LANES - 2 * a) for a in range(4)]
        nd = SLAB // H
        acc = [[None, None] for _ in range(4)]
        hist = [(), ()]
        for sl in range(D // SLAB):
            r0 = sl * SLAB
            q = qkv_s[jj + 1, r0:r0 + SLAB, :]
            k = qkv_s[jj + 1, D + r0:D + r0 + SLAB, :]
            q, k = pace.gate(q, k, after=hist[-2])
            kp = qkv_s[jj, D + r0:D + r0 + SLAB, :]
            rkp = rk_s[jj % 2, r0:r0 + SLAB, :]
            rk = pltpu.roll(k, 8, 1)
            rk_s[(jj + 1) % 2, r0:r0 + SLAB, :] = rk
            for a in range(4):
                rq = q if a == 0 else pltpu.roll(q, LANES - 2 * a, 1)
                for b in range(2):
                    if b == 0:
                        mix = k if a == 0 else jnp.where(m0[a], k, kp)
                    else:
                        mix = jnp.where(m1[a], rk, rkp)
                    p = rq * mix
                    for i in range(nd):
                        pi = p[i * H:(i + 1) * H]
                        acc[a][b] = pi if acc[a][b] is None else acc[a][b] + pi
            hist.append(tuple(acc[a][b][h:h + 8] for a in range(4) for b in range(2) for h in (0, 8)))
        lane16 = jax.lax.broadcasted_iota(jnp.int32, (H, LANES), 1)
        logit = []
        for w in range(W):
            a, b = w % 4, w // 4
            lw = acc[a][b] if a == 0 else pltpu.roll(acc[a][b], 2 * a, 1)
            lw = lw * scale
            if jj == 0 and w > 0:
                lw = jnp.where(lane16 >= 2 * w, lw, -1e9)
            logit.append(lw)
        mx = functools.reduce(jnp.maximum, logit)
        ex = [jnp.exp(l - mx) for l in logit]
        inv = 1.0 / functools.reduce(jnp.add, ex)
        ra = [[None, None] for _ in range(4)]
        for w in range(W):
            a, b = w % 4, w // 4
            aw = ex[w] * inv
            aw = aw if a == 0 else pltpu.roll(aw, LANES - 2 * a, 1)
            ra[a][b] = jnp.concatenate([aw] * nd, axis=0)
        for sl in range(D // SLAB):
            r0 = sl * SLAB
            v = qkv_s[jj + 1, 2 * D + r0:2 * D + r0 + SLAB, :]
            v, = pace.gate(v)
            vp = qkv_s[jj, 2 * D + r0:2 * D + r0 + SLAB, :]
            rvp = rv_s[jj % 2, r0:r0 + SLAB, :]
            rv = pltpu.roll(v, 8, 1)
            rv_s[(jj + 1) % 2, r0:r0 + SLAB, :] = rv
            o = None
            for a in range(4):
                mix0 = v if a == 0 else jnp.where(m0[a], v, vp)
                mix1 = jnp.where(m1[a], rv, rvp)
                t = ra[a][0] * mix0 + ra[a][1] * mix1
                o = t if a == 0 else o + pltpu.roll(t, 2 * a, 1)
            o_s[r0:r0 + SLAB, jj * LANES:(jj + 1) * LANES] = o.astype(bf16)

    def attn(c, tokens):
        z = b2f_s[0:8, :]
        pace = _Pacer(tokens, 2 * (D // SLAB) * CPC, z + 1.0 < z)
        for j in range(CPC):
            attn_col(c * CPC + j, pace)

    def gelu(tokens):
        z = b2f_s[0:8, :]
        pace = _Pacer(tokens, NLB * (F // LANES), z + 1.0 < z)
        for nn in range(F // LANES):
            col = pl.ds(nn * LANES, LANES)
            bias = jnp.broadcast_to(b1f_s[nn:nn + 1, :], (8, LANES))
            for i in range(NLB):
                rows = slice(i * LNB, (i + 1) * LNB)
                u_s[rows, col] = _gelu(acc_s[rows, col] + _rep(pace(bias), LNB)).astype(bf16)

    def gate_mm(i):
        cs = slice(OOFF[i], OOFF[i + 1])
        y, tokens = None, []
        for k0 in range(0, F, KB):
            ks = slice(k0, min(k0 + KB, F))
            part = jnp.dot(u_s[:, ks], w2_s[ks, cs], preferred_element_type=f32)
            tokens += _tokens(part) if k0 + KB <= F else _tokens(part[:, 0:LANES])
            y = part if y is None else y + part
        g = []
        for j in range(OUT_PIECES[i] // LANES):
            jj = OOFF[i] // LANES + j
            g.append(_silu(y[:, j * LANES:(j + 1) * LANES] + b2f_s[jj:jj + 1, :]))
        return g, tokens

    def final(i, g):
        cs = slice(OOFF[i], OOFF[i + 1])
        s = jnp.dot(wot_s[...], o_s[:, cs], preferred_element_type=f32)
        rows = TAIL_ROWS if i == NO - 1 else (0, D)
        for (r0, r1), cp in zip(zip(rows[:-1], rows[1:]), out_cps(i)):
            for j in range(OUT_PIECES[i] // LANES):
                jj = OOFF[i] // LANES + j
                xr = x_s[jj // CPC, r0:r1, pl.ds((jj % CPC) * LANES, LANES)].astype(f32)
                r = xr + s[r0:r1, j * LANES:(j + 1) * LANES] * g[j][r0:r1]
                out_s[r0:r1, pl.ds(jj * LANES, LANES)] = r.astype(bf16)
            cp.start()
        return _tokens(s)

    @pl.when(steps == NC - 3)
    def _():
        b1f_s[...] = b1_s[...].astype(f32)
        b2f_s[...] = b2_s[...].astype(f32)
        prep_wqkv_t()
        z = b2f_s[0:8, :]
        never = z + 1.0 < z
        nb = (F // NB) * (D // 16)
        last = mix1(NC - 1, "mid", due=_spread(prep_wqkv_perm(), nb, nb * 2 // 7, nb), never=never)

        tokens = []
        for c in range(QKV_AHEAD):
            tokens += qkv(c)
        gelu(last[len(last) // 2:] + tokens[:len(tokens) // 3])
        attn(0, tokens[len(tokens) // 3:len(tokens) * 9 // 10])

    _scope("ww2", lambda: w2_cp.wait())
    prep_wo()
    tokens = []
    for c in range(NC):
        if c + QKV_AHEAD < NC:
            tokens += qkv(c + QKV_AHEAD)
        g, t = gate_mm(c)
        tokens += t + final(c, g)
        if c + 1 < NC:
            attn(c + 1, tokens[c * ATTN_WIN:(c + 1) * ATTN_WIN])
    final(NC, gate_mm(NC)[0])

    def waits():
        for i in range(NO):
            for cp in out_cps(i):
                cp.wait()
    _scope("wout", waits)


@jax.jit
def pallas_recurrent_scan__sliding_local_dilated__mixer_token_mlp__prompt_kernel(
    A_x: jax.Array,
    A_wqkv: jax.Array,
    A_wo: jax.Array,
    B_x: jax.Array,
    B_w1: jax.Array,
    B_b1: jax.Array,
    B_w2: jax.Array,
    B_b2: jax.Array,
):
    del B_x
    xt = jnp.swapaxes(A_x, 1, 2)
    b1 = B_b1.reshape(F // LANES, LANES)
    b2 = B_b2.reshape(S // LANES, LANES)
    any_spec = pl.BlockSpec(memory_space=pl.ANY)
    out_t = pl.pallas_call(
        _kernel,
        out_shape=jax.ShapeDtypeStruct((1, D, S), bf16),
        in_specs=[any_spec] * 7,
        out_specs=any_spec,
        scratch_shapes=[
            pltpu.VMEM((NC, D, TC), bf16),
            pltpu.VMEM((D, 3 * D), bf16),
            pltpu.VMEM((D, D), bf16),
            pltpu.VMEM((NC, TC, F), bf16),
            pltpu.VMEM((F, S), bf16),
            pltpu.VMEM((F // LANES, LANES), bf16),
            pltpu.VMEM((S // LANES, LANES), bf16),
            pltpu.VMEM((NC, D // 2, TC), u32),
            pltpu.VMEM((NC, D // 2, TC), u32),
            pltpu.VMEM((D, F), f32),
            pltpu.VMEM((D // 2, F), u32),
            pltpu.VMEM((4, 11 * LANES, LANES), f32),
            pltpu.VMEM((3 * D // 2, D), u32),
            pltpu.VMEM((4, D, LANES), f32),
            pltpu.VMEM((D // 2, D), u32),
            pltpu.VMEM((NCOL + 1, 3 * D, LANES), f32),
            pltpu.VMEM((2, D, LANES), f32),
            pltpu.VMEM((2, D, LANES), f32),
            pltpu.VMEM((D // 2, S), u32),
            pltpu.VMEM((D, S), bf16),
            pltpu.VMEM((F // LANES, LANES), f32),
            pltpu.VMEM((S // LANES, LANES), f32),
            pltpu.SemaphoreType.DMA((NSEM,)),
        ],
        compiler_params=pltpu.CompilerParams(vmem_limit_bytes=100 * 1024 * 1024,
                                             disable_semaphore_checks=True,
                                             disable_bounds_checks=True),
        name="fused_mixer_attn",
    )(xt, A_wqkv, A_wo, B_w1, b1, B_w2, b2)
    return jnp.swapaxes(out_t, 1, 2)
```

```python
import functools

import jax
import jax.numpy as jnp
import jax.experimental.pallas as pl
import jax.experimental.pallas.tpu as pltpu

S = 2048
D = 448
H = 16
DH = D // H
F = 1792
W = 8
EPS = 1e-5
TC = 256
NC = S // TC
LANES = 128
NCOL = S // LANES
SLAB = 32

f32 = jnp.float32
bf16 = jnp.bfloat16
u32 = jnp.uint32

_SCOPES = False


def _scope(name, fn):
    if _SCOPES:
        with jax.named_scope(name):
            fn()
    else:
        fn()


LNB = 64
NLB = D // LNB


def _rep(v8, rows):
    return jnp.concatenate([v8] * (rows // 8), axis=0)


def _ln_stats(x_ref, col, pace):
    piv = jnp.broadcast_to(x_ref[0:1, col].astype(f32), (8, LANES))
    s1 = s2 = None
    for i in range(NLB):
        pv = _rep(pace(piv), LNB // 2)
        w = pltpu.bitcast(x_ref[i * LNB:(i + 1) * LNB, col], u32)
        for half in (w << 16, w & jnp.uint32(0xFFFF0000)):
            d = pltpu.bitcast(half, f32) - pv
            for k in range(LNB // 2 // 16):
                dk = d[k * 16:(k + 1) * 16]
                s1 = dk if s1 is None else s1 + dk
                s2 = dk * dk if s2 is None else s2 + dk * dk
    md = jnp.sum(s1, axis=0, keepdims=True) * (1.0 / D)
    v = jnp.maximum(jnp.sum(s2, axis=0, keepdims=True) * (1.0 / D) - md * md, 0.0)
    return piv + md, jax.lax.rsqrt(v + EPS)


def _tokens(r):
    return [r[i:i + 8, j:j + LANES] for j in range(0, r.shape[1], LANES) for i in range(0, r.shape[0], 8)]


def _deadline(lhs, toks, never):
    if not any(t is not None for t in toks):
        return lhs
    w = pltpu.bitcast(lhs, u32)
    blocks = [w[8 * i:8 * i + 8, 0:LANES] for i in range(w.shape[0] // 8)]
    blocks = [b if t is None else jnp.where(never, t, b) for b, t in zip(blocks, toks, strict=True)]
    w = jnp.concatenate([jnp.concatenate(blocks, axis=0), w[:, LANES:]], axis=1)
    return pltpu.bitcast(w, bf16)


def _spread(vals, nslots, lo, hi):
    out = [None] * nslots
    for i in range(lo, hi):
        out[i] = vals[((i - lo + 1) * len(vals)) // (hi - lo) - 1]
    return out


class _Pacer:
    def __init__(self, tokens, count, never):
        self.tokens, self.count, self.never, self.i = tokens, count, never, 0

    def __call__(self, v8):
        if not self.tokens:
            return v8
        tok = self.tokens[self.i * len(self.tokens) // self.count]
        self.i += 1
        return jnp.where(self.never, tok, v8)

    def gate(self, *vs, after=()):
        if not self.tokens:
            return vs
        tok = self.tokens[self.i * len(self.tokens) // self.count]
        self.i += 1
        for a in after:
            tok = jnp.maximum(tok, a)
        n = vs[0].shape[0]
        nv, tk = _rep(self.never, n), _rep(tok, n)
        return tuple(jnp.where(nv, tk, v) for v in vs)


def _gelu(x):
    c = 0.7978845608028654
    t = jnp.tanh(x * (c + (c * 0.044715) * (x * x)))
    hx = 0.5 * x
    return hx + hx * t


def _silu(y):
    hy = 0.5 * y
    return hy + hy * jnp.tanh(hy)


RAMP = (
    (((0, 0, 128, 0, 768),), None),
    (((0, 0, 128, 768, F),), 0),
    (((0, 128, 256, 0, 1024),), 1),
    (((0, 128, 256, 1024, F), (1, 0, 256, 0, 512)), None),
    (((1, 0, 256, 512, F),), 2),
)
RECTS = tuple(r for rects, _ in RAMP for r in rects)
NB = 256
ATTN_WIN = 740
KB = 512
CPC = TC // LANES
QKV_AHEAD = 3
OUT_PIECES = (256,) * 7 + (128, 128)
OOFF = tuple(sum(OUT_PIECES[:i]) for i in range(len(OUT_PIECES) + 1))
NO = len(OUT_PIECES)
TAIL_ROWS = (0, 256, 384, D)
SEM_X, SEM_W1, SEM_MISC, SEM_OUT = 0, NC, 2 * NC, 2 * NC + 6
SEM_RAMP = SEM_OUT + NO + len(TAIL_ROWS) - 2
NSEM = SEM_RAMP + len(RECTS)


def _kernel(x_hbm, wqkv_hbm, wo_hbm, w1_hbm, b1_hbm, w2_hbm, b2_hbm, out_hbm,
            x_s, wqkv_s, wo_s, w1_s, w2_s, b1_s, b2_s,
            xn_s, h_s, acc_s, u_s, wt32_s, wqkvt_s, wo32_s, wot_s,
            qkv_s, rk_s, rv_s, o_s, out_s, b1f_s, b2f_s, sem):
    xn_s, h_s, u_s, wqkvt_s, wot_s, o_s = (
        r.bitcast(bf16) for r in (xn_s, h_s, u_s, wqkvt_s, wot_s, o_s))

    def x_cp(p):
        return pltpu.make_async_copy(x_hbm.at[0, :, pl.ds(p * TC, TC)], x_s.at[p], sem.at[SEM_X + p])

    def w1_cp(p):
        return pltpu.make_async_copy(w1_hbm.at[pl.ds(p * TC, TC), :], w1_s.at[p], sem.at[SEM_W1 + p])

    def rect_cp(r):
        p, k0, k1, lo, hi = r
        return pltpu.make_async_copy(w1_hbm.at[p * TC + k0:p * TC + k1, lo:hi], w1_s.at[p, k0:k1, lo:hi],
                                     sem.at[SEM_RAMP + RECTS.index(r)])

    def out_cps(i):
        sl = slice(OOFF[i], OOFF[i + 1])
        rows = TAIL_ROWS if i == NO - 1 else (0, D)
        return [pltpu.make_async_copy(out_s.at[r0:r1, sl], out_hbm.at[0, r0:r1, sl], sem.at[SEM_OUT + i + k])
                for k, (r0, r1) in enumerate(zip(rows[:-1], rows[1:]))]

    def x0_cp(j):
        sl = pl.ds(j * LANES, LANES)
        return pltpu.make_async_copy(x_hbm.at[0, :, sl], x_s.at[0, :, sl],
                                     sem.at[SEM_X if j == 0 else SEM_MISC + 5])

    wqkv_cp = pltpu.make_async_copy(wqkv_hbm, wqkv_s, sem.at[SEM_MISC + 0])
    wo_cp = pltpu.make_async_copy(wo_hbm, wo_s, sem.at[SEM_MISC + 1])
    b1_cp = pltpu.make_async_copy(b1_hbm, b1_s, sem.at[SEM_MISC + 2])
    b2_cp = pltpu.make_async_copy(b2_hbm, b2_s, sem.at[SEM_MISC + 3])
    w2_cp = pltpu.make_async_copy(w2_hbm, w2_s, sem.at[SEM_MISC + 4])

    def ramp_x_cp(xc):
        return x0_cp(1) if xc == 0 else x_cp(xc)

    x0_cp(0).start()
    for rects, xc in RAMP:
        for r in rects:
            rect_cp(r).start()
        if xc is not None:
            ramp_x_cp(xc).start()
    for p in range(2, NC):
        if p == NC - 1:
            wqkv_cp.start()
            wo_cp.start()
            b1_cp.start()
            b2_cp.start()
        w1_cp(p).start()
        if p + 1 < NC:
            x_cp(p + 1).start()
    w2_cp.start()

    def prep_wqkv_t():
        for c in range(11):
            wd = min(LANES, 3 * D - c * LANES)
            blk = wqkv_s[:, c * LANES:c * LANES + wd].T.astype(f32)
            for kt in range(4):
                kw = min(LANES, D - kt * LANES)
                wt32_s[kt, c * LANES:c * LANES + wd, 0:kw] = blk[:, kt * LANES:kt * LANES + kw]

    def prep_wqkv_perm():
        done = []
        for sec in range(3):
            for d in range(DH):
                r0 = sec * D + d * H
                tok = None
                for kt in range(4):
                    kw = min(LANES, D - kt * LANES)
                    rows = wt32_s[kt, pl.ds(sec * D + d, H, stride=DH), :]
                    wqkvt_s[r0:r0 + H, kt * LANES:kt * LANES + kw] = rows[:, 0:kw].astype(bf16)
                    if kt < 3:
                        t = pltpu.bitcast(rows[8:16], u32)
                        tok = t if tok is None else tok | t
                done.append(tok)
        return done

    def prep_wo():
        for nt in range(4):
            nw = min(LANES, D - nt * LANES)
            wo32_s[nt, 0:D, 0:nw] = wo_s[:, nt * LANES:nt * LANES + nw].astype(f32)
        for nt in range(4):
            nw = min(LANES, D - nt * LANES)
            rows = [wo32_s[nt, pl.ds(d, H, stride=DH), :][:, 0:nw].astype(bf16) for d in range(DH)]
            blk = jnp.concatenate(rows, axis=0)
            wot_s[nt * LANES:nt * LANES + nw, :] = blk.T

    def ln_piece(p, tokens, cols=tuple(range(CPC))):
        xp, xnp, hp = x_s.at[p], xn_s.at[p], h_s.at[p]
        z = xp[0:8, 0:LANES].astype(f32)
        pace = _Pacer(tokens, 3 * NLB * len(cols), z + 1.0 < z)
        for j in cols:
            col = pl.ds(j * LANES, LANES)
            m, r = _ln_stats(xp, col, pace)
            t1 = t2 = None
            for i in range(NLB):
                rows = slice(i * LNB, (i + 1) * LNB)
                xn = (xp[rows, col].astype(f32) - _rep(pace(m), LNB)) * r
                xnp[rows, col] = xn.astype(bf16)
                for k in range(LNB // 16):
                    xk = xn[k * 16:(k + 1) * 16]
                    t1 = xk if t1 is None else t1 + xk
                    t2 = xk * xk if t2 is None else t2 + xk * xk
            m2 = jnp.sum(t1, axis=0, keepdims=True) * (1.0 / D)
            v2 = jnp.maximum(jnp.sum(t2, axis=0, keepdims=True) * (1.0 / D) - m2 * m2, 0.0)
            r2 = jax.lax.rsqrt(v2 + EPS)
            m2 = jnp.broadcast_to(m2, (8, LANES))
            for i in range(NLB):
                rows = slice(i * LNB, (i + 1) * LNB)
                hp[rows, col] = ((xnp[rows, col].astype(f32) - _rep(pace(m2), LNB)) * r2).astype(bf16)

    def mix1(p, n_lo=0, n_hi=F, due=None, never=None):
        tokens = []
        nb = D // 16
        for n in range(n_lo // NB, n_hi // NB):
            ns = slice(n * NB, (n + 1) * NB)
            lhs = h_s[p] if due is None else _deadline(h_s[p], due[n * nb:(n + 1) * nb], never)
            part = jnp.dot(lhs, w1_s[p, :, ns], preferred_element_type=f32)
            tokens += [part[r:r + 8, 0:LANES] for r in range(0, D, 8)]
            acc_s[:, ns] += part
        return tokens if due is not None else tokens[:len(tokens) * 7 // 8]

    zeros = jnp.zeros((D, LANES), f32)
    qkv_s[0, D:2 * D, :] = zeros
    qkv_s[0, 2 * D:3 * D, :] = zeros
    rk_s[0] = zeros
    rv_s[0] = zeros

    def mix1_half(k0, n_lo, n_hi):
        tokens = []
        for lo in range(n_lo, n_hi, 2 * NB):
            ns = slice(lo, min(lo + 2 * NB, n_hi))
            halves = ((0, D),) if ns.stop - lo == 2 * NB else ((0, D // 2), (D // 2, D))
            for r0, r1 in halves:
                part = jnp.dot(h_s[0, r0:r1, k0:k0 + LANES], w1_s[0, k0:k0 + LANES, ns],
                               preferred_element_type=f32)
                if r0 == 0:
                    tokens += [part[r:r + 8, 0:LANES] for r in range(0, r1, 8)]
                if k0 == 0:
                    acc_s[r0:r1, ns] = part
                else:
                    acc_s[r0:r1, ns] += part
        return tokens[:len(tokens) * 7 // 8]

    _scope("wx0", lambda: x0_cp(0).wait())
    ln_piece(0, [], (0,))
    for rects, xc in RAMP:
        def waits():
            for r in rects:
                rect_cp(r).wait()
            if xc is not None:
                ramp_x_cp(xc).wait()
        _scope("wr", waits)
        tokens = []
        for p, k0, k1, lo, hi in rects:
            tokens += mix1_half(k0, lo, hi) if p == 0 else mix1(p, lo, hi)
        if xc is not None:
            ln_piece(xc, tokens, (1,) if xc == 0 else tuple(range(CPC)))

    def mid_step(p, carry):
        _scope("wl", lambda: (w1_cp(p).wait(), x_cp(p + 1).wait()))
        ln_piece(p + 1, mix1(p))
        return carry + 1

    steps = jax.lax.fori_loop(2, NC - 1, mid_step, 0)

    def waits():
        wqkv_cp.wait()
        wo_cp.wait()
        b1_cp.wait()
        b2_cp.wait()
        w1_cp(NC - 1).wait()
    _scope("wlast", waits)

    def qkv(c):
        r = jnp.dot(wqkvt_s[...], xn_s[c], preferred_element_type=f32)
        for j in range(TC // LANES):
            qkv_s[c * (TC // LANES) + j + 1] = r[:, j * LANES:(j + 1) * LANES]
        return _tokens(r)

    scale = DH ** -0.5

    def attn_col(jj, pace):
        lane = jax.lax.broadcasted_iota(jnp.int32, (SLAB, LANES), 1)
        m0 = [None] + [lane < LANES - 2 * a for a in range(1, 4)]
        m1 = [(lane >= 8) & (lane < LANES - 2 * a) for a in range(4)]
        nd = SLAB // H
        acc = [[None, None] for _ in range(4)]
        hist = [(), ()]
        for sl in range(D // SLAB):
            r0 = sl * SLAB
            q = qkv_s[jj + 1, r0:r0 + SLAB, :]
            k = qkv_s[jj + 1, D + r0:D + r0 + SLAB, :]
            q, k = pace.gate(q, k, after=hist[-2])
            kp = qkv_s[jj, D + r0:D + r0 + SLAB, :]
            rkp = rk_s[jj % 2, r0:r0 + SLAB, :]
            rk = pltpu.roll(k, 8, 1)
            rk_s[(jj + 1) % 2, r0:r0 + SLAB, :] = rk
            for a in range(4):
                rq = q if a == 0 else pltpu.roll(q, LANES - 2 * a, 1)
                for b in range(2):
                    if b == 0:
                        mix = k if a == 0 else jnp.where(m0[a], k, kp)
                    else:
                        mix = jnp.where(m1[a], rk, rkp)
                    p = rq * mix
                    for i in range(nd):
                        pi = p[i * H:(i + 1) * H]
                        acc[a][b] = pi if acc[a][b] is None else acc[a][b] + pi
            hist.append(tuple(acc[a][b][h:h + 8] for a in range(4) for b in range(2) for h in (0, 8)))
        lane16 = jax.lax.broadcasted_iota(jnp.int32, (H, LANES), 1)
        logit = []
        for w in range(W):
            a, b = w % 4, w // 4
            lw = acc[a][b] if a == 0 else pltpu.roll(acc[a][b], 2 * a, 1)
            lw = lw * scale
            if jj == 0 and w > 0:
                lw = jnp.where(lane16 >= 2 * w, lw, -1e9)
            logit.append(lw)
        mx = functools.reduce(jnp.maximum, logit)
        ex = [jnp.exp(l - mx) for l in logit]
        inv = 1.0 / functools.reduce(jnp.add, ex)
        ra = [[None, None] for _ in range(4)]
        for w in range(W):
            a, b = w % 4, w // 4
            aw = ex[w] * inv
            aw = aw if a == 0 else pltpu.roll(aw, LANES - 2 * a, 1)
            ra[a][b] = jnp.concatenate([aw] * nd, axis=0)
        for sl in range(D // SLAB):
            r0 = sl * SLAB
            v = qkv_s[jj + 1, 2 * D + r0:2 * D + r0 + SLAB, :]
            v, = pace.gate(v)
            vp = qkv_s[jj, 2 * D + r0:2 * D + r0 + SLAB, :]
            rvp = rv_s[jj % 2, r0:r0 + SLAB, :]
            rv = pltpu.roll(v, 8, 1)
            rv_s[(jj + 1) % 2, r0:r0 + SLAB, :] = rv
            o = None
            for a in range(4):
                mix0 = v if a == 0 else jnp.where(m0[a], v, vp)
                mix1 = jnp.where(m1[a], rv, rvp)
                t = ra[a][0] * mix0 + ra[a][1] * mix1
                o = t if a == 0 else o + pltpu.roll(t, 2 * a, 1)
            o_s[r0:r0 + SLAB, jj * LANES:(jj + 1) * LANES] = o.astype(bf16)

    def attn(c, tokens):
        z = b2f_s[0:8, :]
        pace = _Pacer(tokens, 2 * (D // SLAB) * CPC, z + 1.0 < z)
        for j in range(CPC):
            attn_col(c * CPC + j, pace)

    def gelu(tokens):
        z = b2f_s[0:8, :]
        pace = _Pacer(tokens, NLB * (F // LANES), z + 1.0 < z)
        for nn in range(F // LANES):
            col = pl.ds(nn * LANES, LANES)
            bias = jnp.broadcast_to(b1f_s[nn:nn + 1, :], (8, LANES))
            for i in range(NLB):
                rows = slice(i * LNB, (i + 1) * LNB)
                u_s[rows, col] = _gelu(acc_s[rows, col] + _rep(pace(bias), LNB)).astype(bf16)

    def gate_mm(i):
        cs = slice(OOFF[i], OOFF[i + 1])
        y, tokens = None, []
        for k0 in range(0, F, KB):
            ks = slice(k0, min(k0 + KB, F))
            part = jnp.dot(u_s[:, ks], w2_s[ks, cs], preferred_element_type=f32)
            tokens += _tokens(part) if k0 + KB <= F else _tokens(part[:, 0:LANES])
            y = part if y is None else y + part
        g = []
        for j in range(OUT_PIECES[i] // LANES):
            jj = OOFF[i] // LANES + j
            g.append(_silu(y[:, j * LANES:(j + 1) * LANES] + b2f_s[jj:jj + 1, :]))
        return g, tokens

    def final(i, g):
        cs = slice(OOFF[i], OOFF[i + 1])
        s = jnp.dot(wot_s[...], o_s[:, cs], preferred_element_type=f32)
        rows = TAIL_ROWS if i == NO - 1 else (0, D)
        for (r0, r1), cp in zip(zip(rows[:-1], rows[1:]), out_cps(i)):
            for j in range(OUT_PIECES[i] // LANES):
                jj = OOFF[i] // LANES + j
                xr = x_s[jj // CPC, r0:r1, pl.ds((jj % CPC) * LANES, LANES)].astype(f32)
                r = xr + s[r0:r1, j * LANES:(j + 1) * LANES] * g[j][r0:r1]
                out_s[r0:r1, pl.ds(jj * LANES, LANES)] = r.astype(bf16)
            cp.start()
        return _tokens(s)

    @pl.when(steps == NC - 3)
    def _():
        b1f_s[...] = b1_s[...].astype(f32)
        b2f_s[...] = b2_s[...].astype(f32)
        prep_wqkv_t()
        z = b2f_s[0:8, :]
        never = z + 1.0 < z
        nb = (F // NB) * (D // 16)
        last = mix1(NC - 1, due=_spread(prep_wqkv_perm(), nb, nb * 2 // 7, nb), never=never)

        tokens = []
        for c in range(QKV_AHEAD):
            tokens += qkv(c)
        gelu(last[len(last) // 2:] + tokens[:len(tokens) // 3])
        attn(0, tokens[len(tokens) // 3:len(tokens) * 9 // 10])

    _scope("ww2", lambda: w2_cp.wait())
    prep_wo()
    tokens = []
    for c in range(NC):
        if c + QKV_AHEAD < NC:
            tokens += qkv(c + QKV_AHEAD)
        g, t = gate_mm(c)
        tokens += t + final(c, g)
        if c + 1 < NC:
            attn(c + 1, tokens[c * ATTN_WIN:(c + 1) * ATTN_WIN])
    final(NC, gate_mm(NC)[0])

    def waits():
        for i in range(NO):
            for cp in out_cps(i):
                cp.wait()
    _scope("wout", waits)


@jax.jit
def pallas_recurrent_scan__sliding_local_dilated__mixer_token_mlp__prompt_kernel(
    A_x: jax.Array,
    A_wqkv: jax.Array,
    A_wo: jax.Array,
    B_x: jax.Array,
    B_w1: jax.Array,
    B_b1: jax.Array,
    B_w2: jax.Array,
    B_b2: jax.Array,
):
    del B_x
    xt = jnp.swapaxes(A_x, 1, 2)
    b1 = B_b1.reshape(F // LANES, LANES)
    b2 = B_b2.reshape(S // LANES, LANES)
    any_spec = pl.BlockSpec(memory_space=pl.ANY)
    out_t = pl.pallas_call(
        _kernel,
        out_shape=jax.ShapeDtypeStruct((1, D, S), bf16),
        in_specs=[any_spec] * 7,
        out_specs=any_spec,
        scratch_shapes=[
            pltpu.VMEM((NC, D, TC), bf16),
            pltpu.VMEM((D, 3 * D), bf16),
            pltpu.VMEM((D, D), bf16),
            pltpu.VMEM((NC, TC, F), bf16),
            pltpu.VMEM((F, S), bf16),
            pltpu.VMEM((F // LANES, LANES), bf16),
            pltpu.VMEM((S // LANES, LANES), bf16),
            pltpu.VMEM((NC, D // 2, TC), u32),
            pltpu.VMEM((NC, D // 2, TC), u32),
            pltpu.VMEM((D, F), f32),
            pltpu.VMEM((D // 2, F), u32),
            pltpu.VMEM((4, 11 * LANES, LANES), f32),
            pltpu.VMEM((3 * D // 2, D), u32),
            pltpu.VMEM((4, D + 32, LANES), f32),
            pltpu.VMEM((D // 2, D), u32),
            pltpu.VMEM((NCOL + 1, 3 * D, LANES), f32),
            pltpu.VMEM((2, D, LANES), f32),
            pltpu.VMEM((2, D, LANES), f32),
            pltpu.VMEM((D // 2, S), u32),
            pltpu.VMEM((D, S), bf16),
            pltpu.VMEM((F // LANES, LANES), f32),
            pltpu.VMEM((S // LANES, LANES), f32),
            pltpu.SemaphoreType.DMA((NSEM,)),
        ],
        compiler_params=pltpu.CompilerParams(vmem_limit_bytes=100 * 1024 * 1024,
                                             disable_semaphore_checks=True,
                                             disable_bounds_checks=True),
        name="fused_mixer_attn",
    )(xt, A_wqkv, A_wo, B_w1, b1, B_w2, b2)
    return jnp.swapaxes(out_t, 1, 2)
```

```python
import functools

import jax
import jax.numpy as jnp
import jax.experimental.pallas as pl
import jax.experimental.pallas.tpu as pltpu

S = 2048
D = 448
H = 16
DH = D // H
F = 1792
W = 8
EPS = 1e-5
TC = 256
NC = S // TC
LANES = 128
NCOL = S // LANES
SLAB = 32

f32 = jnp.float32
bf16 = jnp.bfloat16
u32 = jnp.uint32

_SCOPES = False


def _scope(name, fn):
    if _SCOPES:
        with jax.named_scope(name):
            fn()
    else:
        fn()


LNB = 64
NLB = D // LNB


def _rep(v8, rows):
    return jnp.concatenate([v8] * (rows // 8), axis=0)


def _ln_stats(x_ref, col, pace):
    piv = jnp.broadcast_to(x_ref[0:1, col].astype(f32), (8, LANES))
    s1 = s2 = None
    for i in range(NLB):
        pv = _rep(pace(piv), LNB // 2)
        w = pltpu.bitcast(x_ref[i * LNB:(i + 1) * LNB, col], u32)
        for half in (w << 16, w & jnp.uint32(0xFFFF0000)):
            d = pltpu.bitcast(half, f32) - pv
            for k in range(LNB // 2 // 16):
                dk = d[k * 16:(k + 1) * 16]
                s1 = dk if s1 is None else s1 + dk
                s2 = dk * dk if s2 is None else s2 + dk * dk
    md = jnp.sum(s1, axis=0, keepdims=True) * (1.0 / D)
    v = jnp.maximum(jnp.sum(s2, axis=0, keepdims=True) * (1.0 / D) - md * md, 0.0)
    return piv + md, jax.lax.rsqrt(v + EPS)


def _tokens(r):
    return [r[i:i + 8, j:j + LANES] for j in range(0, r.shape[1], LANES) for i in range(0, r.shape[0], 8)]


def _deadline(lhs, toks, never):
    if not any(t is not None for t in toks):
        return lhs
    w = pltpu.bitcast(lhs, u32)
    blocks = [w[8 * i:8 * i + 8, 0:LANES] for i in range(w.shape[0] // 8)]
    blocks = [b if t is None else jnp.where(never, t, b) for b, t in zip(blocks, toks, strict=True)]
    w = jnp.concatenate([jnp.concatenate(blocks, axis=0), w[:, LANES:]], axis=1)
    return pltpu.bitcast(w, bf16)


def _spread(vals, nslots, lo, hi):
    out = [None] * nslots
    for i in range(lo, hi):
        out[i] = vals[((i - lo + 1) * len(vals)) // (hi - lo) - 1]
    return out


class _Pacer:
    def __init__(self, tokens, count, never):
        self.tokens, self.count, self.never, self.i = tokens, count, never, 0

    def __call__(self, v8):
        if not self.tokens:
            return v8
        tok = self.tokens[self.i * len(self.tokens) // self.count]
        self.i += 1
        return jnp.where(self.never, tok, v8)

    def gate(self, *vs, after=()):
        if not self.tokens:
            return vs
        tok = self.tokens[self.i * len(self.tokens) // self.count]
        self.i += 1
        for a in after:
            tok = jnp.maximum(tok, a)
        n = vs[0].shape[0]
        nv, tk = _rep(self.never, n), _rep(tok, n)
        return tuple(jnp.where(nv, tk, v) for v in vs)


def _gelu(x):
    c = 0.7978845608028654
    t = jnp.tanh(x * (c + (c * 0.044715) * (x * x)))
    hx = 0.5 * x
    return hx + hx * t


def _silu(y):
    hy = 0.5 * y
    return hy + hy * jnp.tanh(hy)


RAMP = (
    (((0, 0, 128, 0, 768),), None),
    (((0, 0, 128, 768, F),), 0),
    (((0, 128, 256, 0, 1024),), 1),
    (((0, 128, 256, 1024, F), (1, 0, 256, 0, 512)), None),
    (((1, 0, 256, 512, F),), 2),
)
RECTS = tuple(r for rects, _ in RAMP for r in rects)
NB = 256
ATTN_WIN = 740
KB = 512
CPC = TC // LANES
QKV_AHEAD = 3
OUT_PIECES = (256,) * 7 + (128, 128)
OOFF = tuple(sum(OUT_PIECES[:i]) for i in range(len(OUT_PIECES) + 1))
NO = len(OUT_PIECES)
TAIL_ROWS = (0, 256, 384, D)
SEM_X, SEM_W1, SEM_MISC, SEM_OUT = 0, NC, 2 * NC, 2 * NC + 6
SEM_RAMP = SEM_OUT + NO + len(TAIL_ROWS) - 2
NSEM = SEM_RAMP + len(RECTS)


def _kernel(x_hbm, wqkv_hbm, wo_hbm, w1_hbm, b1_hbm, w2_hbm, b2_hbm, out_hbm,
            x_s, wqkv_s, wo_s, w1_s, w2_s, b1_s, b2_s,
            xn_s, h_s, acc_s, u_s, wt32_s, wqkvt_s, wo32_s, wot_s,
            qkv_s, rk_s, rv_s, o_s, out_s, b1f_s, b2f_s, sem):
    xn_s, h_s, u_s, wqkvt_s, wot_s, o_s = (
        r.bitcast(bf16) for r in (xn_s, h_s, u_s, wqkvt_s, wot_s, o_s))

    def x_cp(p):
        return pltpu.make_async_copy(x_hbm.at[0, :, pl.ds(p * TC, TC)], x_s.at[p], sem.at[SEM_X + p])

    def w1_cp(p):
        return pltpu.make_async_copy(w1_hbm.at[pl.ds(p * TC, TC), :], w1_s.at[p], sem.at[SEM_W1 + p])

    def rect_cp(r):
        p, k0, k1, lo, hi = r
        return pltpu.make_async_copy(w1_hbm.at[p * TC + k0:p * TC + k1, lo:hi], w1_s.at[p, k0:k1, lo:hi],
                                     sem.at[SEM_RAMP + RECTS.index(r)])

    def out_cps(i):
        sl = slice(OOFF[i], OOFF[i + 1])
        rows = TAIL_ROWS if i == NO - 1 else (0, D)
        return [pltpu.make_async_copy(out_s.at[r0:r1, sl], out_hbm.at[0, r0:r1, sl], sem.at[SEM_OUT + i + k])
                for k, (r0, r1) in enumerate(zip(rows[:-1], rows[1:]))]

    def x0_cp(j):
        sl = pl.ds(j * LANES, LANES)
        return pltpu.make_async_copy(x_hbm.at[0, :, sl], x_s.at[0, :, sl],
                                     sem.at[SEM_X if j == 0 else SEM_MISC + 5])

    wqkv_cp = pltpu.make_async_copy(wqkv_hbm, wqkv_s, sem.at[SEM_MISC + 0])
    wo_cp = pltpu.make_async_copy(wo_hbm, wo_s, sem.at[SEM_MISC + 1])
    b1_cp = pltpu.make_async_copy(b1_hbm, b1_s, sem.at[SEM_MISC + 2])
    b2_cp = pltpu.make_async_copy(b2_hbm, b2_s, sem.at[SEM_MISC + 3])
    w2_cp = pltpu.make_async_copy(w2_hbm, w2_s, sem.at[SEM_MISC + 4])

    def ramp_x_cp(xc):
        return x0_cp(1) if xc == 0 else x_cp(xc)

    x0_cp(0).start()
    for rects, xc in RAMP:
        for r in rects:
            rect_cp(r).start()
        if xc is not None:
            ramp_x_cp(xc).start()
    for p in range(2, NC):
        if p == NC - 1:
            wqkv_cp.start()
            wo_cp.start()
            b1_cp.start()
            b2_cp.start()
        w1_cp(p).start()
        if p + 1 < NC:
            x_cp(p + 1).start()
    w2_cp.start()

    def prep_wqkv_t():
        for c in range(11):
            wd = min(LANES, 3 * D - c * LANES)
            blk = wqkv_s[:, c * LANES:c * LANES + wd].T.astype(f32)
            for kt in range(4):
                kw = min(LANES, D - kt * LANES)
                wt32_s[kt, c * LANES:c * LANES + wd, 0:kw] = blk[:, kt * LANES:kt * LANES + kw]

    def prep_wqkv_perm():
        done = []
        for sec in range(3):
            for d in range(DH):
                r0 = sec * D + d * H
                tok = None
                for kt in range(4):
                    kw = min(LANES, D - kt * LANES)
                    rows = wt32_s[kt, pl.ds(sec * D + d, H, stride=DH), :]
                    wqkvt_s[r0:r0 + H, kt * LANES:kt * LANES + kw] = rows[:, 0:kw].astype(bf16)
                    if kt < 3:
                        t = pltpu.bitcast(rows[8:16], u32)
                        tok = t if tok is None else tok | t
                done.append(tok)
        return done

    def prep_wo(tokens):
        z = b2f_s[0:8, :]
        pace = _Pacer(tokens, 3 * NLB, z + 1.0 < z)
        for nt in range(4):
            nw = min(LANES, D - nt * LANES)
            for i in range(NLB):
                rows = slice(i * LNB, (i + 1) * LNB)
                w = wo_s[rows, nt * LANES:nt * LANES + nw].astype(f32)
                wo32_s[nt, rows, 0:nw] = pace.gate(w)[0] if nt < 3 else w
        for nt in range(4):
            nw = min(LANES, D - nt * LANES)
            rows = [wo32_s[nt, pl.ds(d, H, stride=DH), :][:, 0:nw].astype(bf16) for d in range(DH)]
            blk = jnp.concatenate(rows, axis=0)
            wot_s[nt * LANES:nt * LANES + nw, :] = blk.T

    def ln_piece(p, tokens, cols=tuple(range(CPC))):
        xp, xnp, hp = x_s.at[p], xn_s.at[p], h_s.at[p]
        z = xp[0:8, 0:LANES].astype(f32)
        pace = _Pacer(tokens, 3 * NLB * len(cols), z + 1.0 < z)
        for j in cols:
            col = pl.ds(j * LANES, LANES)
            m, r = _ln_stats(xp, col, pace)
            t1 = t2 = None
            for i in range(NLB):
                rows = slice(i * LNB, (i + 1) * LNB)
                xn = (xp[rows, col].astype(f32) - _rep(pace(m), LNB)) * r
                xnp[rows, col] = xn.astype(bf16)
                for k in range(LNB // 16):
                    xk = xn[k * 16:(k + 1) * 16]
                    t1 = xk if t1 is None else t1 + xk
                    t2 = xk * xk if t2 is None else t2 + xk * xk
            m2 = jnp.sum(t1, axis=0, keepdims=True) * (1.0 / D)
            v2 = jnp.maximum(jnp.sum(t2, axis=0, keepdims=True) * (1.0 / D) - m2 * m2, 0.0)
            r2 = jax.lax.rsqrt(v2 + EPS)
            m2 = jnp.broadcast_to(m2, (8, LANES))
            for i in range(NLB):
                rows = slice(i * LNB, (i + 1) * LNB)
                hp[rows, col] = ((xnp[rows, col].astype(f32) - _rep(pace(m2), LNB)) * r2).astype(bf16)

    def mix1(p, n_lo=0, n_hi=F, due=None, never=None):
        tokens = []
        nb = D // 16
        for n in range(n_lo // NB, n_hi // NB):
            ns = slice(n * NB, (n + 1) * NB)
            lhs = h_s[p] if due is None else _deadline(h_s[p], due[n * nb:(n + 1) * nb], never)
            part = jnp.dot(lhs, w1_s[p, :, ns], preferred_element_type=f32)
            tokens += [part[r:r + 8, 0:LANES] for r in range(0, D, 8)]
            acc_s[:, ns] += part
        return tokens if due is not None else tokens[:len(tokens) * 7 // 8]

    zeros = jnp.zeros((D, LANES), f32)
    qkv_s[0, D:2 * D, :] = zeros
    qkv_s[0, 2 * D:3 * D, :] = zeros
    rk_s[0] = zeros
    rv_s[0] = zeros

    def mix1_half(k0, n_lo, n_hi):
        tokens = []
        for lo in range(n_lo, n_hi, 2 * NB):
            ns = slice(lo, min(lo + 2 * NB, n_hi))
            halves = ((0, D),) if ns.stop - lo == 2 * NB else ((0, D // 2), (D // 2, D))
            for r0, r1 in halves:
                part = jnp.dot(h_s[0, r0:r1, k0:k0 + LANES], w1_s[0, k0:k0 + LANES, ns],
                               preferred_element_type=f32)
                if r0 == 0:
                    tokens += [part[r:r + 8, 0:LANES] for r in range(0, r1, 8)]
                if k0 == 0:
                    acc_s[r0:r1, ns] = part
                else:
                    acc_s[r0:r1, ns] += part
        return tokens[:len(tokens) * 7 // 8]

    _scope("wx0", lambda: x0_cp(0).wait())
    ln_piece(0, [], (0,))
    for rects, xc in RAMP:
        def waits():
            for r in rects:
                rect_cp(r).wait()
            if xc is not None:
                ramp_x_cp(xc).wait()
        _scope("wr", waits)
        tokens = []
        for p, k0, k1, lo, hi in rects:
            tokens += mix1_half(k0, lo, hi) if p == 0 else mix1(p, lo, hi)
        if xc is not None:
            ln_piece(xc, tokens, (1,) if xc == 0 else tuple(range(CPC)))

    def mid_step(p, carry):
        _scope("wl", lambda: (w1_cp(p).wait(), x_cp(p + 1).wait()))
        ln_piece(p + 1, mix1(p))
        return carry + 1

    steps = jax.lax.fori_loop(2, NC - 1, mid_step, 0)

    def waits():
        wqkv_cp.wait()
        wo_cp.wait()
        b1_cp.wait()
        b2_cp.wait()
        w1_cp(NC - 1).wait()
    _scope("wlast", waits)

    def qkv(c):
        r = jnp.dot(wqkvt_s[...], xn_s[c], preferred_element_type=f32)
        for j in range(TC // LANES):
            qkv_s[c * (TC // LANES) + j + 1] = r[:, j * LANES:(j + 1) * LANES]
        return _tokens(r)

    scale = DH ** -0.5

    def attn_col(jj, pace):
        lane = jax.lax.broadcasted_iota(jnp.int32, (SLAB, LANES), 1)
        m0 = [None] + [lane < LANES - 2 * a for a in range(1, 4)]
        m1 = [(lane >= 8) & (lane < LANES - 2 * a) for a in range(4)]
        nd = SLAB // H
        acc = [[None, None] for _ in range(4)]
        hist = [(), ()]
        for sl in range(D // SLAB):
            r0 = sl * SLAB
            q = qkv_s[jj + 1, r0:r0 + SLAB, :]
            k = qkv_s[jj + 1, D + r0:D + r0 + SLAB, :]
            q, k = pace.gate(q, k, after=hist[-2])
            kp = qkv_s[jj, D + r0:D + r0 + SLAB, :]
            rkp = rk_s[jj % 2, r0:r0 + SLAB, :]
            rk = pltpu.roll(k, 8, 1)
            rk_s[(jj + 1) % 2, r0:r0 + SLAB, :] = rk
            for a in range(4):
                rq = q if a == 0 else pltpu.roll(q, LANES - 2 * a, 1)
                for b in range(2):
                    if b == 0:
                        mix = k if a == 0 else jnp.where(m0[a], k, kp)
                    else:
                        mix = jnp.where(m1[a], rk, rkp)
                    p = rq * mix
                    for i in range(nd):
                        pi = p[i * H:(i + 1) * H]
                        acc[a][b] = pi if acc[a][b] is None else acc[a][b] + pi
            hist.append(tuple(acc[a][b][h:h + 8] for a in range(4) for b in range(2) for h in (0, 8)))
        lane16 = jax.lax.broadcasted_iota(jnp.int32, (H, LANES), 1)
        logit = []
        for w in range(W):
            a, b = w % 4, w // 4
            lw = acc[a][b] if a == 0 else pltpu.roll(acc[a][b], 2 * a, 1)
            lw = lw * scale
            if jj == 0 and w > 0:
                lw = jnp.where(lane16 >= 2 * w, lw, -1e9)
            logit.append(lw)
        mx = functools.reduce(jnp.maximum, logit)
        ex = [jnp.exp(l - mx) for l in logit]
        inv = 1.0 / functools.reduce(jnp.add, ex)
        ra = [[None, None] for _ in range(4)]
        for w in range(W):
            a, b = w % 4, w // 4
            aw = ex[w] * inv
            aw = aw if a == 0 else pltpu.roll(aw, LANES - 2 * a, 1)
            ra[a][b] = jnp.concatenate([aw] * nd, axis=0)
        for sl in range(D // SLAB):
            r0 = sl * SLAB
            v = qkv_s[jj + 1, 2 * D + r0:2 * D + r0 + SLAB, :]
            v, = pace.gate(v)
            vp = qkv_s[jj, 2 * D + r0:2 * D + r0 + SLAB, :]
            rvp = rv_s[jj % 2, r0:r0 + SLAB, :]
            rv = pltpu.roll(v, 8, 1)
            rv_s[(jj + 1) % 2, r0:r0 + SLAB, :] = rv
            o = None
            for a in range(4):
                mix0 = v if a == 0 else jnp.where(m0[a], v, vp)
                mix1 = jnp.where(m1[a], rv, rvp)
                t = ra[a][0] * mix0 + ra[a][1] * mix1
                o = t if a == 0 else o + pltpu.roll(t, 2 * a, 1)
            o_s[r0:r0 + SLAB, jj * LANES:(jj + 1) * LANES] = o.astype(bf16)

    def attn(c, tokens):
        z = b2f_s[0:8, :]
        pace = _Pacer(tokens, 2 * (D // SLAB) * CPC, z + 1.0 < z)
        for j in range(CPC):
            attn_col(c * CPC + j, pace)

    def gelu(tokens):
        z = b2f_s[0:8, :]
        pace = _Pacer(tokens, NLB * (F // LANES), z + 1.0 < z)
        for nn in range(F // LANES):
            col = pl.ds(nn * LANES, LANES)
            bias = jnp.broadcast_to(b1f_s[nn:nn + 1, :], (8, LANES))
            for i in range(NLB):
                rows = slice(i * LNB, (i + 1) * LNB)
                u_s[rows, col] = _gelu(acc_s[rows, col] + _rep(pace(bias), LNB)).astype(bf16)

    def gate_mm(i):
        cs = slice(OOFF[i], OOFF[i + 1])
        y, tokens = None, []
        for k0 in range(0, F, KB):
            ks = slice(k0, min(k0 + KB, F))
            part = jnp.dot(u_s[:, ks], w2_s[ks, cs], preferred_element_type=f32)
            tokens += _tokens(part) if k0 + KB <= F else _tokens(part[:, 0:LANES])
            y = part if y is None else y + part
        g = []
        for j in range(OUT_PIECES[i] // LANES):
            jj = OOFF[i] // LANES + j
            g.append(_silu(y[:, j * LANES:(j + 1) * LANES] + b2f_s[jj:jj + 1, :]))
        return g, tokens

    def final(i, g):
        cs = slice(OOFF[i], OOFF[i + 1])
        s = jnp.dot(wot_s[...], o_s[:, cs], preferred_element_type=f32)
        rows = TAIL_ROWS if i == NO - 1 else (0, D)
        for (r0, r1), cp in zip(zip(rows[:-1], rows[1:]), out_cps(i)):
            for j in range(OUT_PIECES[i] // LANES):
                jj = OOFF[i] // LANES + j
                xr = x_s[jj // CPC, r0:r1, pl.ds((jj % CPC) * LANES, LANES)].astype(f32)
                r = xr + s[r0:r1, j * LANES:(j + 1) * LANES] * g[j][r0:r1]
                out_s[r0:r1, pl.ds(jj * LANES, LANES)] = r.astype(bf16)
            cp.start()
        return _tokens(s)

    @pl.when(steps == NC - 3)
    def _():
        b1f_s[...] = b1_s[...].astype(f32)
        b2f_s[...] = b2_s[...].astype(f32)
        prep_wqkv_t()
        z = b2f_s[0:8, :]
        never = z + 1.0 < z
        nb = (F // NB) * (D // 16)
        last = mix1(NC - 1, due=_spread(prep_wqkv_perm(), nb, nb * 2 // 7, nb), never=never)

        tokens = []
        for c in range(QKV_AHEAD):
            tokens += qkv(c)
        gelu(last[len(last) // 2:] + tokens[:len(tokens) // 3])
        attn(0, tokens[len(tokens) // 3:len(tokens) * 9 // 10])

    _scope("ww2", lambda: w2_cp.wait())
    tokens = []
    for c in range(NC):
        if c + QKV_AHEAD < NC:
            tokens += qkv(c + QKV_AHEAD)
        if c == 0:
            prep_wo(tokens[8:])
        g, t = gate_mm(c)
        tokens += t + final(c, g)
        if c + 1 < NC:
            attn(c + 1, tokens[c * ATTN_WIN:(c + 1) * ATTN_WIN])
    final(NC, gate_mm(NC)[0])

    def waits():
        for i in range(NO):
            for cp in out_cps(i):
                cp.wait()
    _scope("wout", waits)


@jax.jit
def pallas_recurrent_scan__sliding_local_dilated__mixer_token_mlp__prompt_kernel(
    A_x: jax.Array,
    A_wqkv: jax.Array,
    A_wo: jax.Array,
    B_x: jax.Array,
    B_w1: jax.Array,
    B_b1: jax.Array,
    B_w2: jax.Array,
    B_b2: jax.Array,
):
    del B_x
    xt = jnp.swapaxes(A_x, 1, 2)
    b1 = B_b1.reshape(F // LANES, LANES)
    b2 = B_b2.reshape(S // LANES, LANES)
    any_spec = pl.BlockSpec(memory_space=pl.ANY)
    out_t = pl.pallas_call(
        _kernel,
        out_shape=jax.ShapeDtypeStruct((1, D, S), bf16),
        in_specs=[any_spec] * 7,
        out_specs=any_spec,
        scratch_shapes=[
            pltpu.VMEM((NC, D, TC), bf16),
            pltpu.VMEM((D, 3 * D), bf16),
            pltpu.VMEM((D, D), bf16),
            pltpu.VMEM((NC, TC, F), bf16),
            pltpu.VMEM((F, S), bf16),
            pltpu.VMEM((F // LANES, LANES), bf16),
            pltpu.VMEM((S // LANES, LANES), bf16),
            pltpu.VMEM((NC, D // 2, TC), u32),
            pltpu.VMEM((NC, D // 2, TC), u32),
            pltpu.VMEM((D, F), f32),
            pltpu.VMEM((D // 2, F), u32),
            pltpu.VMEM((4, 11 * LANES, LANES), f32),
            pltpu.VMEM((3 * D // 2, D), u32),
            pltpu.VMEM((4, D + 32, LANES), f32),
            pltpu.VMEM((D // 2, D), u32),
            pltpu.VMEM((NCOL + 1, 3 * D, LANES), f32),
            pltpu.VMEM((2, D, LANES), f32),
            pltpu.VMEM((2, D, LANES), f32),
            pltpu.VMEM((D // 2, S), u32),
            pltpu.VMEM((D, S), bf16),
            pltpu.VMEM((F // LANES, LANES), f32),
            pltpu.VMEM((S // LANES, LANES), f32),
            pltpu.SemaphoreType.DMA((NSEM,)),
        ],
        compiler_params=pltpu.CompilerParams(vmem_limit_bytes=100 * 1024 * 1024,
                                             disable_semaphore_checks=True,
                                             disable_bounds_checks=True),
        name="fused_mixer_attn",
    )(xt, A_wqkv, A_wo, B_w1, b1, B_w2, b2)
    return jnp.swapaxes(out_t, 1, 2)
```

```python
import functools

import jax
import jax.numpy as jnp
import jax.experimental.pallas as pl
import jax.experimental.pallas.tpu as pltpu

S = 2048
D = 448
H = 16
DH = D // H
F = 1792
W = 8
EPS = 1e-5
TC = 256
NC = S // TC
LANES = 128
NCOL = S // LANES
SLAB = 32

f32 = jnp.float32
bf16 = jnp.bfloat16
u32 = jnp.uint32

_SCOPES = False


def _scope(name, fn):
    if _SCOPES:
        with jax.named_scope(name):
            fn()
    else:
        fn()


LNB = 64
NLB = D // LNB


def _rep(v8, rows):
    return jnp.concatenate([v8] * (rows // 8), axis=0)


def _ln_stats(x_ref, col, pace):
    piv = jnp.broadcast_to(x_ref[0:1, col].astype(f32), (8, LANES))
    s1 = s2 = None
    for i in range(NLB):
        pv = _rep(pace(piv), LNB // 2)
        w = pltpu.bitcast(x_ref[i * LNB:(i + 1) * LNB, col], u32)
        for half in (w << 16, w & jnp.uint32(0xFFFF0000)):
            d = pltpu.bitcast(half, f32) - pv
            for k in range(LNB // 2 // 16):
                dk = d[k * 16:(k + 1) * 16]
                s1 = dk if s1 is None else s1 + dk
                s2 = dk * dk if s2 is None else s2 + dk * dk
    md = jnp.sum(s1, axis=0, keepdims=True) * (1.0 / D)
    v = jnp.maximum(jnp.sum(s2, axis=0, keepdims=True) * (1.0 / D) - md * md, 0.0)
    return piv + md, jax.lax.rsqrt(v + EPS)


def _tokens(r):
    return [r[i:i + 8, j:j + LANES] for j in range(0, r.shape[1], LANES) for i in range(0, r.shape[0], 8)]


def _deadline(lhs, toks, never):
    if not any(t is not None for t in toks):
        return lhs
    w = pltpu.bitcast(lhs, u32)
    blocks = [w[8 * i:8 * i + 8, 0:LANES] for i in range(w.shape[0] // 8)]
    blocks = [b if t is None else jnp.where(never, t, b) for b, t in zip(blocks, toks, strict=True)]
    w = jnp.concatenate([jnp.concatenate(blocks, axis=0), w[:, LANES:]], axis=1)
    return pltpu.bitcast(w, bf16)


def _spread(vals, nslots, lo, hi):
    out = [None] * nslots
    for i in range(lo, hi):
        out[i] = vals[((i - lo + 1) * len(vals)) // (hi - lo) - 1]
    return out


class _Pacer:
    def __init__(self, tokens, count, never):
        self.tokens, self.count, self.never, self.i = tokens, count, never, 0

    def __call__(self, v8):
        if not self.tokens:
            return v8
        tok = self.tokens[self.i * len(self.tokens) // self.count]
        self.i += 1
        return jnp.where(self.never, tok, v8)

    def gate(self, *vs, after=()):
        if not self.tokens:
            return vs
        tok = self.tokens[self.i * len(self.tokens) // self.count]
        self.i += 1
        for a in after:
            tok = jnp.maximum(tok, a)
        n = vs[0].shape[0]
        nv, tk = _rep(self.never, n), _rep(tok, n)
        return tuple(jnp.where(nv, tk, v) for v in vs)


def _gelu(x):
    c = 0.7978845608028654
    t = jnp.tanh(x * (c + (c * 0.044715) * (x * x)))
    hx = 0.5 * x
    return hx + hx * t


def _silu(y):
    hy = 0.5 * y
    return hy + hy * jnp.tanh(hy)


RAMP = (
    (((0, 0, 128, 0, 768),), None, None),
    (((0, 0, 128, 768, F),), 0, (0, (1,))),
    (((0, 128, 256, 0, 1024),), 1, (1, (0,))),
    (((0, 128, 256, 1024, F), (1, 0, 256, 0, 512)), None, (1, (1,))),
    (((1, 0, 256, 512, F),), 2, (2, (0, 1))),
)
RECTS = tuple(r for rects, _, _ in RAMP for r in rects)
NB = 256
ATTN_WIN = 740
KB = 512
CPC = TC // LANES
QKV_AHEAD = 3
OUT_PIECES = (256,) * 7 + (128, 128)
OOFF = tuple(sum(OUT_PIECES[:i]) for i in range(len(OUT_PIECES) + 1))
NO = len(OUT_PIECES)
TAIL_ROWS = (0, 256, 384, D)
SEM_X, SEM_W1, SEM_MISC, SEM_OUT = 0, NC, 2 * NC, 2 * NC + 6
SEM_RAMP = SEM_OUT + NO + len(TAIL_ROWS) - 2
NSEM = SEM_RAMP + len(RECTS)


def _kernel(x_hbm, wqkv_hbm, wo_hbm, w1_hbm, b1_hbm, w2_hbm, b2_hbm, out_hbm,
            x_s, wqkv_s, wo_s, w1_s, w2_s, b1_s, b2_s,
            xn_s, h_s, acc_s, u_s, wt32_s, wqkvt_s, wo32_s, wot_s,
            qkv_s, rk_s, rv_s, o_s, out_s, b1f_s, b2f_s, sem):
    xn_s, h_s, u_s, wqkvt_s, wot_s, o_s = (
        r.bitcast(bf16) for r in (xn_s, h_s, u_s, wqkvt_s, wot_s, o_s))

    def x_cp(p):
        return pltpu.make_async_copy(x_hbm.at[0, :, pl.ds(p * TC, TC)], x_s.at[p], sem.at[SEM_X + p])

    def w1_cp(p):
        return pltpu.make_async_copy(w1_hbm.at[pl.ds(p * TC, TC), :], w1_s.at[p], sem.at[SEM_W1 + p])

    def rect_cp(r):
        p, k0, k1, lo, hi = r
        return pltpu.make_async_copy(w1_hbm.at[p * TC + k0:p * TC + k1, lo:hi], w1_s.at[p, k0:k1, lo:hi],
                                     sem.at[SEM_RAMP + RECTS.index(r)])

    def out_cps(i):
        sl = slice(OOFF[i], OOFF[i + 1])
        rows = TAIL_ROWS if i == NO - 1 else (0, D)
        return [pltpu.make_async_copy(out_s.at[r0:r1, sl], out_hbm.at[0, r0:r1, sl], sem.at[SEM_OUT + i + k])
                for k, (r0, r1) in enumerate(zip(rows[:-1], rows[1:]))]

    def x0_cp(j):
        sl = pl.ds(j * LANES, LANES)
        return pltpu.make_async_copy(x_hbm.at[0, :, sl], x_s.at[0, :, sl],
                                     sem.at[SEM_X if j == 0 else SEM_MISC + 5])

    wqkv_cp = pltpu.make_async_copy(wqkv_hbm, wqkv_s, sem.at[SEM_MISC + 0])
    wo_cp = pltpu.make_async_copy(wo_hbm, wo_s, sem.at[SEM_MISC + 1])
    b1_cp = pltpu.make_async_copy(b1_hbm, b1_s, sem.at[SEM_MISC + 2])
    b2_cp = pltpu.make_async_copy(b2_hbm, b2_s, sem.at[SEM_MISC + 3])
    w2_cp = pltpu.make_async_copy(w2_hbm, w2_s, sem.at[SEM_MISC + 4])

    def ramp_x_cp(xc):
        return x0_cp(1) if xc == 0 else x_cp(xc)

    x0_cp(0).start()
    for rects, xc, _ in RAMP:
        for r in rects:
            rect_cp(r).start()
        if xc is not None:
            ramp_x_cp(xc).start()
    for p in range(2, NC):
        if p == NC - 1:
            wqkv_cp.start()
            wo_cp.start()
            b1_cp.start()
            b2_cp.start()
        w1_cp(p).start()
        if p + 1 < NC:
            x_cp(p + 1).start()
    w2_cp.start()

    def prep_wqkv_t():
        for c in range(11):
            wd = min(LANES, 3 * D - c * LANES)
            blk = wqkv_s[:, c * LANES:c * LANES + wd].T.astype(f32)
            for kt in range(4):
                kw = min(LANES, D - kt * LANES)
                wt32_s[kt, c * LANES:c * LANES + wd, 0:kw] = blk[:, kt * LANES:kt * LANES + kw]

    def prep_wqkv_perm():
        done = []
        for sec in range(3):
            for d in range(DH):
                r0 = sec * D + d * H
                tok = None
                for kt in range(4):
                    kw = min(LANES, D - kt * LANES)
                    rows = wt32_s[kt, pl.ds(sec * D + d, H, stride=DH), :]
                    wqkvt_s[r0:r0 + H, kt * LANES:kt * LANES + kw] = rows[:, 0:kw].astype(bf16)
                    if kt < 3:
                        t = pltpu.bitcast(rows[8:16], u32)
                        tok = t if tok is None else tok | t
                done.append(tok)
        return done

    def prep_wo(tokens):
        z = b2f_s[0:8, :]
        pace = _Pacer(tokens, 3 * NLB, z + 1.0 < z)
        for nt in range(4):
            nw = min(LANES, D - nt * LANES)
            for i in range(NLB):
                rows = slice(i * LNB, (i + 1) * LNB)
                w = wo_s[rows, nt * LANES:nt * LANES + nw].astype(f32)
                wo32_s[nt, rows, 0:nw] = pace.gate(w)[0] if nt < 3 else w
        for nt in range(4):
            nw = min(LANES, D - nt * LANES)
            rows = [wo32_s[nt, pl.ds(d, H, stride=DH), :][:, 0:nw].astype(bf16) for d in range(DH)]
            blk = jnp.concatenate(rows, axis=0)
            wot_s[nt * LANES:nt * LANES + nw, :] = blk.T

    def ln_piece(p, tokens, cols=tuple(range(CPC))):
        xp, xnp, hp = x_s.at[p], xn_s.at[p], h_s.at[p]
        z = xp[0:8, 0:LANES].astype(f32)
        pace = _Pacer(tokens, 3 * NLB * len(cols), z + 1.0 < z)
        for j in cols:
            col = pl.ds(j * LANES, LANES)
            m, r = _ln_stats(xp, col, pace)
            t1 = t2 = None
            for i in range(NLB):
                rows = slice(i * LNB, (i + 1) * LNB)
                xn = (xp[rows, col].astype(f32) - _rep(pace(m), LNB)) * r
                xnp[rows, col] = xn.astype(bf16)
                for k in range(LNB // 16):
                    xk = xn[k * 16:(k + 1) * 16]
                    t1 = xk if t1 is None else t1 + xk
                    t2 = xk * xk if t2 is None else t2 + xk * xk
            m2 = jnp.sum(t1, axis=0, keepdims=True) * (1.0 / D)
            v2 = jnp.maximum(jnp.sum(t2, axis=0, keepdims=True) * (1.0 / D) - m2 * m2, 0.0)
            r2 = jax.lax.rsqrt(v2 + EPS)
            m2 = jnp.broadcast_to(m2, (8, LANES))
            for i in range(NLB):
                rows = slice(i * LNB, (i + 1) * LNB)
                hp[rows, col] = ((xnp[rows, col].astype(f32) - _rep(pace(m2), LNB)) * r2).astype(bf16)

    def mix1(p, n_lo=0, n_hi=F, due=None, never=None):
        tokens = []
        nb = D // 16
        for n in range(n_lo // NB, n_hi // NB):
            ns = slice(n * NB, (n + 1) * NB)
            lhs = h_s[p] if due is None else _deadline(h_s[p], due[n * nb:(n + 1) * nb], never)
            part = jnp.dot(lhs, w1_s[p, :, ns], preferred_element_type=f32)
            tokens += [part[r:r + 8, 0:LANES] for r in range(0, D, 8)]
            acc_s[:, ns] += part
        return tokens if due is not None else tokens[:len(tokens) * 7 // 8]

    zeros = jnp.zeros((D, LANES), f32)
    qkv_s[0, D:2 * D, :] = zeros
    qkv_s[0, 2 * D:3 * D, :] = zeros
    rk_s[0] = zeros
    rv_s[0] = zeros

    def mix1_half(k0, n_lo, n_hi):
        tokens = []
        for lo in range(n_lo, n_hi, 2 * NB):
            ns = slice(lo, min(lo + 2 * NB, n_hi))
            halves = ((0, D),) if ns.stop - lo == 2 * NB else ((0, D // 2), (D // 2, D))
            for r0, r1 in halves:
                part = jnp.dot(h_s[0, r0:r1, k0:k0 + LANES], w1_s[0, k0:k0 + LANES, ns],
                               preferred_element_type=f32)
                if r0 == 0:
                    tokens += [part[r:r + 8, 0:LANES] for r in range(0, r1, 8)]
                if k0 == 0:
                    acc_s[r0:r1, ns] = part
                else:
                    acc_s[r0:r1, ns] += part
        return tokens[:len(tokens) * 7 // 8]

    _scope("wx0", lambda: x0_cp(0).wait())
    ln_piece(0, [], (0,))
    for rects, xc, ln in RAMP:
        def waits():
            for r in rects:
                rect_cp(r).wait()
            if xc is not None:
                ramp_x_cp(xc).wait()
        _scope("wr", waits)
        for i, (p, k0, _, lo, hi) in enumerate(rects):
            tokens = mix1_half(k0, lo, hi) if p == 0 else mix1(p, lo, hi)
            if i == 0 and ln is not None:
                ln_piece(ln[0], tokens, ln[1])

    def mid_step(p, carry):
        _scope("wl", lambda: (w1_cp(p).wait(), x_cp(p + 1).wait()))
        ln_piece(p + 1, mix1(p))
        return carry + 1

    steps = jax.lax.fori_loop(2, NC - 1, mid_step, 0)

    def waits():
        wqkv_cp.wait()
        wo_cp.wait()
        b1_cp.wait()
        b2_cp.wait()
        w1_cp(NC - 1).wait()
    _scope("wlast", waits)

    def qkv(c):
        r = jnp.dot(wqkvt_s[...], xn_s[c], preferred_element_type=f32)
        for j in range(TC // LANES):
            qkv_s[c * (TC // LANES) + j + 1] = r[:, j * LANES:(j + 1) * LANES]
        return _tokens(r)

    scale = DH ** -0.5

    def attn_col(jj, pace):
        lane = jax.lax.broadcasted_iota(jnp.int32, (SLAB, LANES), 1)
        m0 = [None] + [lane < LANES - 2 * a for a in range(1, 4)]
        m1 = [(lane >= 8) & (lane < LANES - 2 * a) for a in range(4)]
        nd = SLAB // H
        acc = [[None, None] for _ in range(4)]
        hist = [(), ()]
        for sl in range(D // SLAB):
            r0 = sl * SLAB
            q = qkv_s[jj + 1, r0:r0 + SLAB, :]
            k = qkv_s[jj + 1, D + r0:D + r0 + SLAB, :]
            q, k = pace.gate(q, k, after=hist[-2])
            kp = qkv_s[jj, D + r0:D + r0 + SLAB, :]
            rkp = rk_s[jj % 2, r0:r0 + SLAB, :]
            rk = pltpu.roll(k, 8, 1)
            rk_s[(jj + 1) % 2, r0:r0 + SLAB, :] = rk
            for a in range(4):
                rq = q if a == 0 else pltpu.roll(q, LANES - 2 * a, 1)
                for b in range(2):
                    if b == 0:
                        mix = k if a == 0 else jnp.where(m0[a], k, kp)
                    else:
                        mix = jnp.where(m1[a], rk, rkp)
                    p = rq * mix
                    for i in range(nd):
                        pi = p[i * H:(i + 1) * H]
                        acc[a][b] = pi if acc[a][b] is None else acc[a][b] + pi
            hist.append(tuple(acc[a][b][h:h + 8] for a in range(4) for b in range(2) for h in (0, 8)))
        lane16 = jax.lax.broadcasted_iota(jnp.int32, (H, LANES), 1)
        logit = []
        for w in range(W):
            a, b = w % 4, w // 4
            lw = acc[a][b] if a == 0 else pltpu.roll(acc[a][b], 2 * a, 1)
            lw = lw * scale
            if jj == 0 and w > 0:
                lw = jnp.where(lane16 >= 2 * w, lw, -1e9)
            logit.append(lw)
        mx = functools.reduce(jnp.maximum, logit)
        ex = [jnp.exp(l - mx) for l in logit]
        inv = 1.0 / functools.reduce(jnp.add, ex)
        ra = [[None, None] for _ in range(4)]
        for w in range(W):
            a, b = w % 4, w // 4
            aw = ex[w] * inv
            aw = aw if a == 0 else pltpu.roll(aw, LANES - 2 * a, 1)
            ra[a][b] = jnp.concatenate([aw] * nd, axis=0)
        for sl in range(D // SLAB):
            r0 = sl * SLAB
            v = qkv_s[jj + 1, 2 * D + r0:2 * D + r0 + SLAB, :]
            v, = pace.gate(v)
            vp = qkv_s[jj, 2 * D + r0:2 * D + r0 + SLAB, :]
            rvp = rv_s[jj % 2, r0:r0 + SLAB, :]
            rv = pltpu.roll(v, 8, 1)
            rv_s[(jj + 1) % 2, r0:r0 + SLAB, :] = rv
            o = None
            for a in range(4):
                mix0 = v if a == 0 else jnp.where(m0[a], v, vp)
                mix1 = jnp.where(m1[a], rv, rvp)
                t = ra[a][0] * mix0 + ra[a][1] * mix1
                o = t if a == 0 else o + pltpu.roll(t, 2 * a, 1)
            o_s[r0:r0 + SLAB, jj * LANES:(jj + 1) * LANES] = o.astype(bf16)

    def attn(c, tokens):
        z = b2f_s[0:8, :]
        pace = _Pacer(tokens, 2 * (D // SLAB) * CPC, z + 1.0 < z)
        for j in range(CPC):
            attn_col(c * CPC + j, pace)

    def gelu(tokens):
        z = b2f_s[0:8, :]
        pace = _Pacer(tokens, NLB * (F // LANES), z + 1.0 < z)
        for nn in range(F // LANES):
            col = pl.ds(nn * LANES, LANES)
            bias = jnp.broadcast_to(b1f_s[nn:nn + 1, :], (8, LANES))
            for i in range(NLB):
                rows = slice(i * LNB, (i + 1) * LNB)
                u_s[rows, col] = _gelu(acc_s[rows, col] + _rep(pace(bias), LNB)).astype(bf16)

    def gate_mm(i):
        cs = slice(OOFF[i], OOFF[i + 1])
        y, tokens = None, []
        for k0 in range(0, F, KB):
            ks = slice(k0, min(k0 + KB, F))
            part = jnp.dot(u_s[:, ks], w2_s[ks, cs], preferred_element_type=f32)
            tokens += _tokens(part) if k0 + KB <= F else _tokens(part[:, 0:LANES])
            y = part if y is None else y + part
        g = []
        for j in range(OUT_PIECES[i] // LANES):
            jj = OOFF[i] // LANES + j
            g.append(_silu(y[:, j * LANES:(j + 1) * LANES] + b2f_s[jj:jj + 1, :]))
        return g, tokens

    def final(i, g):
        cs = slice(OOFF[i], OOFF[i + 1])
        s = jnp.dot(wot_s[...], o_s[:, cs], preferred_element_type=f32)
        rows = TAIL_ROWS if i == NO - 1 else (0, D)
        for (r0, r1), cp in zip(zip(rows[:-1], rows[1:]), out_cps(i)):
            for j in range(OUT_PIECES[i] // LANES):
                jj = OOFF[i] // LANES + j
                xr = x_s[jj // CPC, r0:r1, pl.ds((jj % CPC) * LANES, LANES)].astype(f32)
                r = xr + s[r0:r1, j * LANES:(j + 1) * LANES] * g[j][r0:r1]
                out_s[r0:r1, pl.ds(jj * LANES, LANES)] = r.astype(bf16)
            cp.start()
        return _tokens(s)

    @pl.when(steps == NC - 3)
    def _():
        b1f_s[...] = b1_s[...].astype(f32)
        b2f_s[...] = b2_s[...].astype(f32)
        prep_wqkv_t()
        z = b2f_s[0:8, :]
        never = z + 1.0 < z
        nb = (F // NB) * (D // 16)
        last = mix1(NC - 1, due=_spread(prep_wqkv_perm(), nb, nb * 2 // 7, nb), never=never)

        tokens = []
        for c in range(QKV_AHEAD):
            tokens += qkv(c)
        gelu(last[len(last) // 2:] + tokens[:len(tokens) // 3])
        attn(0, tokens[len(tokens) // 3:len(tokens) * 9 // 10])

    _scope("ww2", lambda: w2_cp.wait())
    tokens = []
    for c in range(NC):
        if c + QKV_AHEAD < NC:
            tokens += qkv(c + QKV_AHEAD)
        if c == 0:
            prep_wo(tokens[8:])
        g, t = gate_mm(c)
        tokens += t + final(c, g)
        if c + 1 < NC:
            attn(c + 1, tokens[c * ATTN_WIN:(c + 1) * ATTN_WIN])
    final(NC, gate_mm(NC)[0])

    def waits():
        for i in range(NO):
            for cp in out_cps(i):
                cp.wait()
    _scope("wout", waits)


@jax.jit
def pallas_recurrent_scan__sliding_local_dilated__mixer_token_mlp__prompt_kernel(
    A_x: jax.Array,
    A_wqkv: jax.Array,
    A_wo: jax.Array,
    B_x: jax.Array,
    B_w1: jax.Array,
    B_b1: jax.Array,
    B_w2: jax.Array,
    B_b2: jax.Array,
):
    del B_x
    xt = jnp.swapaxes(A_x, 1, 2)
    b1 = B_b1.reshape(F // LANES, LANES)
    b2 = B_b2.reshape(S // LANES, LANES)
    any_spec = pl.BlockSpec(memory_space=pl.ANY)
    out_t = pl.pallas_call(
        _kernel,
        out_shape=jax.ShapeDtypeStruct((1, D, S), bf16),
        in_specs=[any_spec] * 7,
        out_specs=any_spec,
        scratch_shapes=[
            pltpu.VMEM((NC, D, TC), bf16),
            pltpu.VMEM((D, 3 * D), bf16),
            pltpu.VMEM((D, D), bf16),
            pltpu.VMEM((NC, TC, F), bf16),
            pltpu.VMEM((F, S), bf16),
            pltpu.VMEM((F // LANES, LANES), bf16),
            pltpu.VMEM((S // LANES, LANES), bf16),
            pltpu.VMEM((NC, D // 2, TC), u32),
            pltpu.VMEM((NC, D // 2, TC), u32),
            pltpu.VMEM((D, F), f32),
            pltpu.VMEM((D // 2, F), u32),
            pltpu.VMEM((4, 11 * LANES, LANES), f32),
            pltpu.VMEM((3 * D // 2, D), u32),
            pltpu.VMEM((4, D + 32, LANES), f32),
            pltpu.VMEM((D // 2, D), u32),
            pltpu.VMEM((NCOL + 1, 3 * D, LANES), f32),
            pltpu.VMEM((2, D, LANES), f32),
            pltpu.VMEM((2, D, LANES), f32),
            pltpu.VMEM((D // 2, S), u32),
            pltpu.VMEM((D, S), bf16),
            pltpu.VMEM((F // LANES, LANES), f32),
            pltpu.VMEM((S // LANES, LANES), f32),
            pltpu.SemaphoreType.DMA((NSEM,)),
        ],
        compiler_params=pltpu.CompilerParams(vmem_limit_bytes=100 * 1024 * 1024,
                                             disable_semaphore_checks=True,
                                             disable_bounds_checks=True),
        name="fused_mixer_attn",
    )(xt, A_wqkv, A_wo, B_w1, b1, B_w2, b2)
    return jnp.swapaxes(out_t, 1, 2)
```

```python
import functools

import jax
import jax.numpy as jnp
import jax.experimental.pallas as pl
import jax.experimental.pallas.tpu as pltpu

S = 2048
D = 448
H = 16
DH = D // H
F = 1792
W = 8
EPS = 1e-5
TC = 256
NC = S // TC
LANES = 128
NCOL = S // LANES
SLAB = 32

f32 = jnp.float32
bf16 = jnp.bfloat16
u32 = jnp.uint32

_SCOPES = False


def _scope(name, fn):
    if _SCOPES:
        with jax.named_scope(name):
            fn()
    else:
        fn()


LNB = 64
NLB = D // LNB


def _rep(v8, rows):
    return jnp.concatenate([v8] * (rows // 8), axis=0)


def _ln_stats(x_ref, col, pace):
    piv = jnp.broadcast_to(x_ref[0:1, col].astype(f32), (8, LANES))
    s1 = s2 = None
    for i in range(NLB):
        pv = _rep(pace(piv), LNB // 2)
        w = pltpu.bitcast(x_ref[i * LNB:(i + 1) * LNB, col], u32)
        for half in (w << 16, w & jnp.uint32(0xFFFF0000)):
            d = pltpu.bitcast(half, f32) - pv
            for k in range(LNB // 2 // 16):
                dk = d[k * 16:(k + 1) * 16]
                s1 = dk if s1 is None else s1 + dk
                s2 = dk * dk if s2 is None else s2 + dk * dk
    md = jnp.sum(s1, axis=0, keepdims=True) * (1.0 / D)
    v = jnp.maximum(jnp.sum(s2, axis=0, keepdims=True) * (1.0 / D) - md * md, 0.0)
    return piv + md, jax.lax.rsqrt(v + EPS)


def _tokens(r):
    return [r[i:i + 8, j:j + LANES] for j in range(0, r.shape[1], LANES) for i in range(0, r.shape[0], 8)]


def _deadline(lhs, toks, never):
    if not any(t is not None for t in toks):
        return lhs
    w = pltpu.bitcast(lhs, u32)
    blocks = [w[8 * i:8 * i + 8, 0:LANES] for i in range(w.shape[0] // 8)]
    blocks = [b if t is None else jnp.where(never, t, b) for b, t in zip(blocks, toks, strict=True)]
    w = jnp.concatenate([jnp.concatenate(blocks, axis=0), w[:, LANES:]], axis=1)
    return pltpu.bitcast(w, bf16)


def _spread(vals, nslots, lo, hi):
    out = [None] * nslots
    for i in range(lo, hi):
        out[i] = vals[((i - lo + 1) * len(vals)) // (hi - lo) - 1]
    return out


class _Pacer:
    def __init__(self, tokens, count, never):
        self.tokens, self.count, self.never, self.i = tokens, count, never, 0

    def __call__(self, v8):
        if not self.tokens:
            return v8
        tok = self.tokens[self.i * len(self.tokens) // self.count]
        self.i += 1
        return jnp.where(self.never, tok, v8)

    def gate(self, *vs, after=()):
        if not self.tokens:
            return vs
        tok = self.tokens[self.i * len(self.tokens) // self.count]
        self.i += 1
        for a in after:
            tok = jnp.maximum(tok, a)
        n = vs[0].shape[0]
        nv, tk = _rep(self.never, n), _rep(tok, n)
        return tuple(jnp.where(nv, tk, v) for v in vs)


def _gelu(x):
    c = 0.7978845608028654
    t = jnp.tanh(x * (c + (c * 0.044715) * (x * x)))
    hx = 0.5 * x
    return hx + hx * t


def _silu(y):
    hy = 0.5 * y
    return hy + hy * jnp.tanh(hy)


RAMP = (
    ((), ((0, 0, 512, ()),)),
    ((1,), ((0, 512, 1280, (1,)),)),
    ((), ((0, 1280, F, ()), (1, 0, 768, ()))),
    ((2,), ((1, 768, F, (2,)), (2, 0, 1024, ()))),
    ((3, 4, 5), ((2, 1024, F, (3,)), (3, 0, F, (4, 5)))),
)
RAMP_COLS = 6
RECTS = tuple(r for _, rects in RAMP for r in rects)
NB = 256
ATTN_WIN = 740
KB = 512
CPC = TC // LANES
QKV_AHEAD = 3
OUT_PIECES = (256,) * 7 + (128, 128)
OOFF = tuple(sum(OUT_PIECES[:i]) for i in range(len(OUT_PIECES) + 1))
NO = len(OUT_PIECES)
TAIL_ROWS = (0, 256, 384, D)
SEM_X, SEM_W1, SEM_MISC, SEM_OUT = 0, NC, 2 * NC, 2 * NC + 5
SEM_RAMP = SEM_OUT + NO + len(TAIL_ROWS) - 2
SEM_COL = SEM_RAMP + len(RECTS)
NSEM = SEM_COL + RAMP_COLS


def _kernel(x_hbm, wqkv_hbm, wo_hbm, w1_hbm, b1_hbm, w2_hbm, b2_hbm, out_hbm,
            x_s, wqkv_s, wo_s, w1_s, w2_s, b1_s, b2_s,
            xn_s, h_s, acc_s, u_s, wt32_s, wqkvt_s, wo32_s, wot_s,
            qkv_s, rk_s, rv_s, o_s, out_s, b1f_s, b2f_s, sem):
    xn_s, h_s, u_s, wqkvt_s, wot_s, o_s = (
        r.bitcast(bf16) for r in (xn_s, h_s, u_s, wqkvt_s, wot_s, o_s))

    def x_cp(p):
        return pltpu.make_async_copy(x_hbm.at[0, :, pl.ds(p * TC, TC)], x_s.at[p], sem.at[SEM_X + p])

    def w1_cp(p):
        return pltpu.make_async_copy(w1_hbm.at[pl.ds(p * TC, TC), :], w1_s.at[p], sem.at[SEM_W1 + p])

    def rect_cp(r):
        k, lo, hi, _ = r
        return pltpu.make_async_copy(w1_hbm.at[k * LANES:(k + 1) * LANES, lo:hi],
                                     w1_s.at[k // CPC, pl.ds(k % CPC * LANES, LANES), lo:hi],
                                     sem.at[SEM_RAMP + RECTS.index(r)])

    def out_cps(i):
        sl = slice(OOFF[i], OOFF[i + 1])
        rows = TAIL_ROWS if i == NO - 1 else (0, D)
        return [pltpu.make_async_copy(out_s.at[r0:r1, sl], out_hbm.at[0, r0:r1, sl], sem.at[SEM_OUT + i + k])
                for k, (r0, r1) in enumerate(zip(rows[:-1], rows[1:]))]

    def col_cp(j):
        return pltpu.make_async_copy(x_hbm.at[0, :, j * LANES:(j + 1) * LANES],
                                     x_s.at[j // CPC, :, pl.ds(j % CPC * LANES, LANES)],
                                     sem.at[SEM_COL + j])

    wqkv_cp = pltpu.make_async_copy(wqkv_hbm, wqkv_s, sem.at[SEM_MISC + 0])
    wo_cp = pltpu.make_async_copy(wo_hbm, wo_s, sem.at[SEM_MISC + 1])
    b1_cp = pltpu.make_async_copy(b1_hbm, b1_s, sem.at[SEM_MISC + 2])
    b2_cp = pltpu.make_async_copy(b2_hbm, b2_s, sem.at[SEM_MISC + 3])
    w2_cp = pltpu.make_async_copy(w2_hbm, w2_s, sem.at[SEM_MISC + 4])

    col_cp(0).start()
    for cols, rects in RAMP:
        for r in rects:
            rect_cp(r).start()
        for j in cols:
            col_cp(j).start()
    for p in range(2, NC):
        if p == NC - 1:
            wqkv_cp.start()
            wo_cp.start()
            b1_cp.start()
            b2_cp.start()
        w1_cp(p).start()
        if p + 1 < NC:
            x_cp(p + 1).start()
    w2_cp.start()

    def prep_wqkv_t():
        for c in range(11):
            wd = min(LANES, 3 * D - c * LANES)
            blk = wqkv_s[:, c * LANES:c * LANES + wd].T.astype(f32)
            for kt in range(4):
                kw = min(LANES, D - kt * LANES)
                wt32_s[kt, c * LANES:c * LANES + wd, 0:kw] = blk[:, kt * LANES:kt * LANES + kw]

    def prep_wqkv_perm():
        done = []
        for sec in range(3):
            for d in range(DH):
                r0 = sec * D + d * H
                tok = None
                for kt in range(4):
                    kw = min(LANES, D - kt * LANES)
                    rows = wt32_s[kt, pl.ds(sec * D + d, H, stride=DH), :]
                    wqkvt_s[r0:r0 + H, kt * LANES:kt * LANES + kw] = rows[:, 0:kw].astype(bf16)
                    if kt < 3:
                        t = pltpu.bitcast(rows[8:16], u32)
                        tok = t if tok is None else tok | t
                done.append(tok)
        return done

    def prep_wo(tokens):
        z = b2f_s[0:8, :]
        pace = _Pacer(tokens, 3 * NLB, z + 1.0 < z)
        for nt in range(4):
            nw = min(LANES, D - nt * LANES)
            for i in range(NLB):
                rows = slice(i * LNB, (i + 1) * LNB)
                w = wo_s[rows, nt * LANES:nt * LANES + nw].astype(f32)
                wo32_s[nt, rows, 0:nw] = pace.gate(w)[0] if nt < 3 else w
        for nt in range(4):
            nw = min(LANES, D - nt * LANES)
            rows = [wo32_s[nt, pl.ds(d, H, stride=DH), :][:, 0:nw].astype(bf16) for d in range(DH)]
            blk = jnp.concatenate(rows, axis=0)
            wot_s[nt * LANES:nt * LANES + nw, :] = blk.T

    def ln_piece(p, tokens, cols=tuple(range(CPC))):
        xp, xnp, hp = x_s.at[p], xn_s.at[p], h_s.at[p if isinstance(p, int) and p < 2 else 2]
        z = xp[0:8, pl.ds(cols[0] * LANES, LANES)].astype(f32)
        pace = _Pacer(tokens, 3 * NLB * len(cols), z + 1.0 < z)
        for j in cols:
            col = pl.ds(j * LANES, LANES)
            m, r = _ln_stats(xp, col, pace)
            t1 = t2 = None
            for i in range(NLB):
                rows = slice(i * LNB, (i + 1) * LNB)
                xn = (xp[rows, col].astype(f32) - _rep(pace(m), LNB)) * r
                xnp[rows, col] = xn.astype(bf16)
                for k in range(LNB // 16):
                    xk = xn[k * 16:(k + 1) * 16]
                    t1 = xk if t1 is None else t1 + xk
                    t2 = xk * xk if t2 is None else t2 + xk * xk
            m2 = jnp.sum(t1, axis=0, keepdims=True) * (1.0 / D)
            v2 = jnp.maximum(jnp.sum(t2, axis=0, keepdims=True) * (1.0 / D) - m2 * m2, 0.0)
            r2 = jax.lax.rsqrt(v2 + EPS)
            m2 = jnp.broadcast_to(m2, (8, LANES))
            for i in range(NLB):
                rows = slice(i * LNB, (i + 1) * LNB)
                hp[rows, col] = ((xnp[rows, col].astype(f32) - _rep(pace(m2), LNB)) * r2).astype(bf16)

    def mix1(p, due=None, never=None):
        tokens = []
        nb = D // 16
        for n in range(F // NB):
            ns = slice(n * NB, (n + 1) * NB)
            lhs = h_s[2] if due is None else _deadline(h_s[2], due[n * nb:(n + 1) * nb], never)
            part = jnp.dot(lhs, w1_s[p, :, ns], preferred_element_type=f32)
            tokens += [part[r:r + 8, 0:LANES] for r in range(0, D, 8)]
            acc_s[:, ns] += part
        return tokens if due is not None else tokens[:len(tokens) * 7 // 8]

    zeros = jnp.zeros((D, LANES), f32)
    qkv_s[0, D:2 * D, :] = zeros
    qkv_s[0, 2 * D:3 * D, :] = zeros
    rk_s[0] = zeros
    rv_s[0] = zeros

    def mix1_tile(k, n_lo, n_hi):
        p, ks = k // CPC, pl.ds(k % CPC * LANES, LANES)
        tokens = []
        for lo in range(n_lo, n_hi, 2 * NB):
            ns = slice(lo, min(lo + 2 * NB, n_hi))
            halves = ((0, D),) if ns.stop - lo == 2 * NB else ((0, D // 2), (D // 2, D))
            for r0, r1 in halves:
                part = jnp.dot(h_s[p, r0:r1, ks], w1_s[p, ks, ns], preferred_element_type=f32)
                if r0 == 0:
                    tokens += [part[r:r + 8, 0:LANES] for r in range(0, r1, 8)]
                if k == 0:
                    acc_s[r0:r1, ns] = part
                else:
                    acc_s[r0:r1, ns] += part
        return tokens[:len(tokens) * 7 // 8]

    _scope("wx0", lambda: col_cp(0).wait())
    ln_piece(0, [], (0,))
    for cols, rects in RAMP:
        def waits():
            for r in rects:
                rect_cp(r).wait()
            for j in cols:
                col_cp(j).wait()
        _scope("wr", waits)
        for k, lo, hi, ln in rects:
            tokens = mix1_tile(k, lo, hi)
            if ln:
                ln_piece(ln[0] // CPC, tokens, tuple(j % CPC for j in ln))

    def mid_step(p, carry):
        _scope("wl", lambda: (w1_cp(p).wait(), x_cp(p + 1).wait()))
        ln_piece(p + 1, mix1(p))
        return carry + 1

    steps = jax.lax.fori_loop(2, NC - 1, mid_step, 0)

    def waits():
        wqkv_cp.wait()
        wo_cp.wait()
        b1_cp.wait()
        b2_cp.wait()
        w1_cp(NC - 1).wait()
    _scope("wlast", waits)

    def qkv(c):
        r = jnp.dot(wqkvt_s[...], xn_s[c], preferred_element_type=f32)
        for j in range(TC // LANES):
            qkv_s[c * (TC // LANES) + j + 1] = r[:, j * LANES:(j + 1) * LANES]
        return _tokens(r)

    scale = DH ** -0.5

    def attn_col(jj, pace):
        lane = jax.lax.broadcasted_iota(jnp.int32, (SLAB, LANES), 1)
        m0 = [None] + [lane < LANES - 2 * a for a in range(1, 4)]
        m1 = [(lane >= 8) & (lane < LANES - 2 * a) for a in range(4)]
        nd = SLAB // H
        acc = [[None, None] for _ in range(4)]
        hist = [(), ()]
        for sl in range(D // SLAB):
            r0 = sl * SLAB
            q = qkv_s[jj + 1, r0:r0 + SLAB, :]
            k = qkv_s[jj + 1, D + r0:D + r0 + SLAB, :]
            q, k = pace.gate(q, k, after=hist[-2])
            kp = qkv_s[jj, D + r0:D + r0 + SLAB, :]
            rkp = rk_s[jj % 2, r0:r0 + SLAB, :]
            rk = pltpu.roll(k, 8, 1)
            rk_s[(jj + 1) % 2, r0:r0 + SLAB, :] = rk
            for a in range(4):
                rq = q if a == 0 else pltpu.roll(q, LANES - 2 * a, 1)
                for b in range(2):
                    if b == 0:
                        mix = k if a == 0 else jnp.where(m0[a], k, kp)
                    else:
                        mix = jnp.where(m1[a], rk, rkp)
                    p = rq * mix
                    for i in range(nd):
                        pi = p[i * H:(i + 1) * H]
                        acc[a][b] = pi if acc[a][b] is None else acc[a][b] + pi
            hist.append(tuple(acc[a][b][h:h + 8] for a in range(4) for b in range(2) for h in (0, 8)))
        lane16 = jax.lax.broadcasted_iota(jnp.int32, (H, LANES), 1)
        logit = []
        for w in range(W):
            a, b = w % 4, w // 4
            lw = acc[a][b] if a == 0 else pltpu.roll(acc[a][b], 2 * a, 1)
            lw = lw * scale
            if jj == 0 and w > 0:
                lw = jnp.where(lane16 >= 2 * w, lw, -1e9)
            logit.append(lw)
        mx = functools.reduce(jnp.maximum, logit)
        ex = [jnp.exp(l - mx) for l in logit]
        inv = 1.0 / functools.reduce(jnp.add, ex)
        ra = [[None, None] for _ in range(4)]
        for w in range(W):
            a, b = w % 4, w // 4
            aw = ex[w] * inv
            aw = aw if a == 0 else pltpu.roll(aw, LANES - 2 * a, 1)
            ra[a][b] = jnp.concatenate([aw] * nd, axis=0)
        for sl in range(D // SLAB):
            r0 = sl * SLAB
            v = qkv_s[jj + 1, 2 * D + r0:2 * D + r0 + SLAB, :]
            v, = pace.gate(v)
            vp = qkv_s[jj, 2 * D + r0:2 * D + r0 + SLAB, :]
            rvp = rv_s[jj % 2, r0:r0 + SLAB, :]
            rv = pltpu.roll(v, 8, 1)
            rv_s[(jj + 1) % 2, r0:r0 + SLAB, :] = rv
            o = None
            for a in range(4):
                mix0 = v if a == 0 else jnp.where(m0[a], v, vp)
                mix1 = jnp.where(m1[a], rv, rvp)
                t = ra[a][0] * mix0 + ra[a][1] * mix1
                o = t if a == 0 else o + pltpu.roll(t, 2 * a, 1)
            o_s[r0:r0 + SLAB, jj * LANES:(jj + 1) * LANES] = o.astype(bf16)

    def attn(c, tokens):
        z = b2f_s[0:8, :]
        pace = _Pacer(tokens, 2 * (D // SLAB) * CPC, z + 1.0 < z)
        for j in range(CPC):
            attn_col(c * CPC + j, pace)

    def gelu(tokens):
        z = b2f_s[0:8, :]
        pace = _Pacer(tokens, NLB * (F // LANES), z + 1.0 < z)
        for nn in range(F // LANES):
            col = pl.ds(nn * LANES, LANES)
            bias = jnp.broadcast_to(b1f_s[nn:nn + 1, :], (8, LANES))
            for i in range(NLB):
                rows = slice(i * LNB, (i + 1) * LNB)
                u_s[rows, col] = _gelu(acc_s[rows, col] + _rep(pace(bias), LNB)).astype(bf16)

    def gate_mm(i):
        cs = slice(OOFF[i], OOFF[i + 1])
        y, tokens = None, []
        for k0 in range(0, F, KB):
            ks = slice(k0, min(k0 + KB, F))
            part = jnp.dot(u_s[:, ks], w2_s[ks, cs], preferred_element_type=f32)
            tokens += _tokens(part) if k0 + KB <= F else _tokens(part[:, 0:LANES])
            y = part if y is None else y + part
        g = []
        for j in range(OUT_PIECES[i] // LANES):
            jj = OOFF[i] // LANES + j
            g.append(_silu(y[:, j * LANES:(j + 1) * LANES] + b2f_s[jj:jj + 1, :]))
        return g, tokens

    def final(i, g):
        cs = slice(OOFF[i], OOFF[i + 1])
        s = jnp.dot(wot_s[...], o_s[:, cs], preferred_element_type=f32)
        rows = TAIL_ROWS if i == NO - 1 else (0, D)
        for (r0, r1), cp in zip(zip(rows[:-1], rows[1:]), out_cps(i)):
            for j in range(OUT_PIECES[i] // LANES):
                jj = OOFF[i] // LANES + j
                xr = x_s[jj // CPC, r0:r1, pl.ds((jj % CPC) * LANES, LANES)].astype(f32)
                r = xr + s[r0:r1, j * LANES:(j + 1) * LANES] * g[j][r0:r1]
                out_s[r0:r1, pl.ds(jj * LANES, LANES)] = r.astype(bf16)
            cp.start()
        return _tokens(s)

    @pl.when(steps == NC - 3)
    def _():
        b1f_s[...] = b1_s[...].astype(f32)
        b2f_s[...] = b2_s[...].astype(f32)
        prep_wqkv_t()
        z = b2f_s[0:8, :]
        never = z + 1.0 < z
        nb = (F // NB) * (D // 16)
        last = mix1(NC - 1, due=_spread(prep_wqkv_perm(), nb, nb * 2 // 7, nb), never=never)

        tokens = []
        for c in range(QKV_AHEAD):
            tokens += qkv(c)
        gelu(last[len(last) // 2:] + tokens[:len(tokens) // 3])
        attn(0, tokens[len(tokens) // 3:len(tokens) * 9 // 10])

    _scope("ww2", lambda: w2_cp.wait())
    tokens = []
    for c in range(NC):
        if c + QKV_AHEAD < NC:
            tokens += qkv(c + QKV_AHEAD)
        if c == 0:
            prep_wo(tokens[8:])
        g, t = gate_mm(c)
        tokens += t + final(c, g)
        if c + 1 < NC:
            attn(c + 1, tokens[c * ATTN_WIN:(c + 1) * ATTN_WIN])
    final(NC, gate_mm(NC)[0])

    def waits():
        for i in range(NO):
            for cp in out_cps(i):
                cp.wait()
    _scope("wout", waits)


@jax.jit
def pallas_recurrent_scan__sliding_local_dilated__mixer_token_mlp__prompt_kernel(
    A_x: jax.Array,
    A_wqkv: jax.Array,
    A_wo: jax.Array,
    B_x: jax.Array,
    B_w1: jax.Array,
    B_b1: jax.Array,
    B_w2: jax.Array,
    B_b2: jax.Array,
):
    del B_x
    xt = jnp.swapaxes(A_x, 1, 2)
    b1 = B_b1.reshape(F // LANES, LANES)
    b2 = B_b2.reshape(S // LANES, LANES)
    any_spec = pl.BlockSpec(memory_space=pl.ANY)
    out_t = pl.pallas_call(
        _kernel,
        out_shape=jax.ShapeDtypeStruct((1, D, S), bf16),
        in_specs=[any_spec] * 7,
        out_specs=any_spec,
        scratch_shapes=[
            pltpu.VMEM((NC, D, TC), bf16),
            pltpu.VMEM((D, 3 * D), bf16),
            pltpu.VMEM((D, D), bf16),
            pltpu.VMEM((NC, TC, F), bf16),
            pltpu.VMEM((F, S), bf16),
            pltpu.VMEM((F // LANES, LANES), bf16),
            pltpu.VMEM((S // LANES, LANES), bf16),
            pltpu.VMEM((NC, D // 2, TC), u32),
            pltpu.VMEM((3, D // 2, TC), u32),
            pltpu.VMEM((D, F), f32),
            pltpu.VMEM((D // 2, F), u32),
            pltpu.VMEM((4, 11 * LANES, LANES), f32),
            pltpu.VMEM((3 * D // 2, D), u32),
            pltpu.VMEM((4, D + 32, LANES), f32),
            pltpu.VMEM((D // 2, D), u32),
            pltpu.VMEM((NCOL + 1, 3 * D, LANES), f32),
            pltpu.VMEM((2, D, LANES), f32),
            pltpu.VMEM((2, D, LANES), f32),
            pltpu.VMEM((D // 2, S), u32),
            pltpu.VMEM((D, S), bf16),
            pltpu.VMEM((F // LANES, LANES), f32),
            pltpu.VMEM((S // LANES, LANES), f32),
            pltpu.SemaphoreType.DMA((NSEM,)),
        ],
        compiler_params=pltpu.CompilerParams(vmem_limit_bytes=100 * 1024 * 1024,
                                             disable_semaphore_checks=True,
                                             disable_bounds_checks=True),
        name="fused_mixer_attn",
    )(xt, A_wqkv, A_wo, B_w1, b1, B_w2, b2)
    return jnp.swapaxes(out_t, 1, 2)
```
